```python
import jax
import jax.numpy as jnp

def _softmax(x, axis=-1):
    return jax.nn.softmax(x, axis=axis)

def _gelu(x):
    return jax.nn.gelu(x, approximate=True)

def _silu(x):
    return jax.nn.silu(x)

def _sigmoid(x):
    return jax.nn.sigmoid(x)

def _layernorm(x, axis=-1, eps=1e-05):
    m = jnp.mean(x, axis=axis, keepdims=True)
    v = jnp.var(x, axis=axis, keepdims=True)
    return (x - m) / jnp.sqrt(v + eps)

def _scatter_add(tgt, idx, src, axis=0):
    return tgt.at[idx].add(src)

def _segment_sum(src, seg, n):
    return jax.ops.segment_sum(src, seg, n)

class _Rng:

    def __init__(self, key):
        self._k = key

    def _next(self):
        self._k, sub = jax.random.split(self._k)
        return sub

    def normal(self, shape):
        return jax.random.normal(self._next(), shape, dtype=jnp.bfloat16)

    def randint(self, lo, hi, shape):
        return jax.random.randint(self._next(), shape, lo, hi, dtype=jnp.int32)

    def uniform(self, shape, lo=0.0, hi=1.0):
        return jax.random.uniform(self._next(), shape, jnp.bfloat16, lo, hi)

    def permutation(self, n):
        return jax.random.permutation(self._next(), n)
kernel_name = 'parallel_sum__memory_aug_recurrent_mem_tr__moe_arch_mod__prompt'

def setup_inputs():
    _rng = _Rng(jax.random.key(int.from_bytes(__import__("os").urandom(4), "little")))
    _w = lambda a: (lambda t: t.astype(jnp.bfloat16) if jnp.issubdtype(t.dtype, jnp.floating) else t)(jnp.asarray(a))

    def _A_setup():
        B, S, Dm = (1, 2048, 1024)
        H, Dh = (32, 128)
        M, seg = (8, 32)
        seg = min(seg, S)
        S = S // seg * seg
        return {'x': _w((lambda *s: _rng.normal(s) * 0.05)(B, S, Dm)), 'mem0': _w((lambda *s: _rng.normal(s) * 0.05)(B, M, Dm)), 'Wq': _w((lambda *s: _rng.normal(s) * 0.05)(Dm, H, Dh) * Dm ** (-0.5)), 'Wk': _w((lambda *s: _rng.normal(s) * 0.05)(Dm, H, Dh) * Dm ** (-0.5)), 'Wv': _w((lambda *s: _rng.normal(s) * 0.05)(Dm, H, Dh) * Dm ** (-0.5)), 'Wo': _w((lambda *s: _rng.normal(s) * 0.05)(H, Dh, Dm) * (H * Dh) ** (-0.5)), 'seg_len': seg}
    _A_in = _A_setup()

    def _B_setup():
        B, S, D, F, C = (1, 2048, 1024, 3584, 2)
        return {'x': _w((lambda *s: _rng.normal(s) * 0.05)(B, S, D)), 'w_r': _w((lambda *s: _rng.normal(s) * 0.05)(D)), 'w_gate': _w((lambda *s: _rng.normal(s) * 0.05)(D, F)), 'w_up': _w((lambda *s: _rng.normal(s) * 0.05)(D, F)), 'w_down': _w((lambda *s: _rng.normal(s) * 0.05)(F, D))}
    _B_in = _B_setup()
    return {'A_x': _A_in['x'], 'A_mem0': _A_in['mem0'], 'A_Wq': _A_in['Wq'], 'A_Wk': _A_in['Wk'], 'A_Wv': _A_in['Wv'], 'A_Wo': _A_in['Wo'], 'A_seg_len': _A_in['seg_len'], 'B_x': _B_in['x'], 'B_w_r': _B_in['w_r'], 'B_w_gate': _B_in['w_gate'], 'B_w_up': _B_in['w_up'], 'B_w_down': _B_in['w_down']}

def reference(A_x, A_mem0, A_Wq, A_Wk, A_Wv, A_Wo, A_seg_len, B_x, B_w_r, B_w_gate, B_w_up, B_w_down):

    def _A_ref(x, mem0, Wq, Wk, Wv, Wo, seg_len):
        B, S, Dm = x.shape
        H, Dh = (Wq.shape[1], Wq.shape[2])
        M = mem0.shape[1]
        scale = Dh ** (-0.5)
        n_seg = S // seg_len
        L = M + seg_len
        idx = jnp.arange(L)
        mask = (idx[:, None] < M) | (idx[:, None] >= idx[None, :])
        mem = mem0
        outs = []
        for s in range(n_seg):
            xs = x[:, s * seg_len:(s + 1) * seg_len, :].copy()
            h = jnp.concatenate([mem, xs], axis=1)
            q = jnp.einsum('btd,dhe->bhte', h, Wq)
            k = jnp.einsum('btd,dhe->bhte', h, Wk)
            v = jnp.einsum('btd,dhe->bhte', h, Wv)
            scores = jnp.einsum('bhqe,bhke->bhqk', q, k) * scale
            scores = jnp.where(mask[None, None], scores, -1000000000.0)
            p = _softmax(scores, axis=-1)
            o = jnp.einsum('bhqk,bhke->bhqe', p, v)
            o = jnp.einsum('bhte,hed->btd', o, Wo)
            mem = o[:, :M, :].copy()
            outs.append(o[:, M:, :])
        return jnp.concatenate(outs, axis=1)

    def _B_ref(x, w_r, w_gate, w_up, w_down):
        B, S, D = x.shape
        C = 2
        r = x @ w_r
        idx = jnp.argsort(-r, axis=-1)[:, :C]
        idx_e = jnp.repeat(idx.reshape(B, C, 1), D, axis=2)
        x_sel = jnp.take_along_axis(x, idx_e, axis=1)
        g = _silu(x_sel @ w_gate)
        u = x_sel @ w_up
        y = g * u @ w_down
        r_sel = _sigmoid(jnp.take_along_axis(r, idx, axis=1))
        y = y * r_sel.reshape(B, C, 1)
        b_off = (jnp.arange(B) * S).reshape(B, 1)
        flat_idx = (idx + b_off).reshape(B * C)
        zero = (x * 0.0).reshape(B * S, D)
        upd = _scatter_add(zero, flat_idx, y.reshape(B * C, D), axis=0)
        return x + upd.reshape(B, S, D)
    x = A_x
    xn = _layernorm(x, axis=-1)
    return x + _A_ref(xn, A_mem0, A_Wq, A_Wk, A_Wv, A_Wo, A_seg_len) + _B_ref(xn, B_w_r, B_w_gate, B_w_up, B_w_down)
```

```python
import functools

import jax
import jax.numpy as jnp
from jax import lax
import jax.experimental.pallas as pl
import jax.experimental.pallas.tpu as pltpu

F32 = jnp.float32
BF16 = jnp.bfloat16
U32 = jnp.uint32

S = 2048
D = 1024
H = 32
E = 128
M = 8
SEG = 32
NSEG = S // SEG
FF = 3584
NP = H // 2
L2 = 2 * (M + SEG)

PRE = 512
TPS = 24
NS = 17
NO = 17
NE = PRE // SEG
NST = 6
NCH = 3 * NP
NOC = 4
KC = H * E // NOC
PPC = NP // NOC
XCH = 512

EPS = 1e-05
SCALE = float(E) ** -0.5


def _rb(v):
    return v.astype(BF16).astype(F32)


def _layernorm_rows(xb, wr):
    xf = xb.astype(F32)
    mean = jnp.sum(xf, axis=-1, keepdims=True) * (1.0 / D)
    xc = xf - mean
    var = jnp.sum(xc * xc, axis=-1, keepdims=True) * (1.0 / D)
    den = _rb(jnp.sqrt(_rb(_rb(var) + EPS)))
    d = _rb(xf - _rb(mean))
    xn = (d * (1.0 / den)).astype(BF16)
    r = _rb(jnp.sum(xn.astype(F32) * wr, axis=-1, keepdims=True))
    return xn, r


def _kernel(x_hbm, mem0_hbm, wq_hbm, wk_hbm, wv_hbm, wo_hbm, wr_hbm, wg_hbm, wu_hbm, wd_hbm,
            out_hbm,
            x_v, xn_v, l_v, ring, o_v0, o_v1, o_v2, o_v3, wqkv, wo_v, stage, wg_v, wu_v, wd_v, r_v, wr_v, fill_v,
            sem_x, sem_s, sem_st, sem_w, sem_o):
    o_vs = (o_v0, o_v1, o_v2, o_v3)
    w32 = [w.bitcast(U32) for w in (wq_hbm, wk_hbm, wv_hbm)]

    def x_copy(c):
        return pltpu.make_async_copy(x_hbm.at[pl.ds(c * XCH, XCH)], x_v.at[pl.ds(c * XCH, XCH)],
                                     sem_x.at[c])

    def st_copy(t, p, slot, dp):
        return pltpu.make_async_copy(w32[t].at[:, dp, p, 0, :], stage.at[slot, dp],
                                     sem_st.at[slot, dp])

    def st_start(c):
        slot = lax.rem(c, NST)
        p = lax.div(c, 3)
        t = lax.rem(c, 3)
        for tt in range(3):
            @pl.when(t == tt)
            def _():
                st_copy(tt, p, slot, 0).start()
                st_copy(tt, p, slot, 1).start()

    def st_wait(c):
        slot = lax.rem(c, NST)
        st_copy(0, 0, slot, 0).wait()
        st_copy(0, 0, slot, 1).wait()

    mem0_copy = pltpu.make_async_copy(mem0_hbm, l_v.at[pl.ds(0, M)], sem_s.at[0])
    wr_copy = pltpu.make_async_copy(wr_hbm, wr_v, sem_s.at[1])
    wo_copy = pltpu.make_async_copy(wo_hbm.bitcast(U32), wo_v, sem_w.at[0])
    wg_copy = pltpu.make_async_copy(wg_hbm.bitcast(U32), wg_v, sem_w.at[1])
    wu_copy = pltpu.make_async_copy(wu_hbm.bitcast(U32), wu_v, sem_w.at[2])
    wd_copy = pltpu.make_async_copy(wd_hbm.bitcast(U32), wd_v, sem_w.at[3])

    wr_copy.start()
    x_copy(0).start()
    for c in range(2):
        st_copy(c % 3, c // 3, c, 0).start()
        st_copy(c % 3, c // 3, c, 1).start()
    x_copy(1).start()
    for c in range(2, NST):
        st_copy(c % 3, c // 3, c, 0).start()
        st_copy(c % 3, c // 3, c, 1).start()
    mem0_copy.start()
    x_copy(2).start()
    x_copy(3).start()
    wo_copy.start()

    row = lax.broadcasted_iota(jnp.int32, (L2, L2), 0)
    col = lax.broadcasted_iota(jnp.int32, (L2, L2), 1)
    rl = jnp.where(row >= L2 // 2, row - L2 // 2, row)
    cl = jnp.where(col >= L2 // 2, col - L2 // 2, col)
    same = (row >= L2 // 2) == (col >= L2 // 2)
    keep = (rl < M) | (rl >= cl)
    fill_v[...] = jnp.where(same, jnp.where(keep, 0.0, -1000000000.0), -jnp.inf).astype(F32)

    wr_copy.wait()
    x_copy(0).wait()

    def ln0(i, c):
        r0 = pl.multiple_of(i * 32, 32)
        xn, r = _layernorm_rows(x_v[pl.ds(r0, 32), :], wr_v[...].astype(F32))
        xn_v[pl.ds(r0, 32), :] = xn
        r_v[pl.ds(r0, 32), :] = r
        return c

    lax.fori_loop(0, PRE // 32, ln0, 0)

    def relayout(c):
        slot = lax.rem(c, NST)
        for j in range(D // 2 // 64):
            a = stage[slot, 0, j * 64:(j + 1) * 64, :]
            b = stage[slot, 1, j * 64:(j + 1) * 64, :]
            wqkv[c, j * 64:(j + 1) * 64, 0:E] = (a & jnp.uint32(0xFFFF)) | (b << 16)
            wqkv[c, j * 64:(j + 1) * 64, E:2 * E] = (a >> 16) | (b & jnp.uint32(0xFFFF0000))

    st_wait(0)
    relayout(0)
    st_start(NST)
    x_copy(1).wait()

    def pro(c, carry):
        @pl.when(c == 16)
        def _():
            x_copy(2).wait()

        @pl.when(c == 32)
        def _():
            x_copy(3).wait()

        cn = jnp.minimum(c + 1, NCH - 1)

        @pl.when(c + 1 < NCH)
        def _():
            st_wait(c + 1)

        p = lax.div(c, 3)
        t = lax.rem(c, 3)
        for rb in range(PRE // 128):
            w = pltpu.bitcast(wqkv[c], BF16)
            y = jnp.dot(xn_v[rb * 128:(rb + 1) * 128, :], w, preferred_element_type=F32)
            y = y.astype(BF16)
            for sg in range(4):
                for hh in range(2):
                    ring[rb * 4 + sg, t, p, hh * 40 + M:hh * 40 + 40, :] = (
                        y[sg * 32:(sg + 1) * 32, hh * E:(hh + 1) * E])
        r0 = pl.multiple_of(PRE + c * 32, 32)
        xn, r = _layernorm_rows(x_v[pl.ds(r0, 32), :], wr_v[...].astype(F32))
        xn_v[pl.ds(r0, 32), :] = xn
        r_v[pl.ds(r0, 32), :] = r
        for j in range(4):
            g = c * 4 + j
            lr = pl.multiple_of(lax.div(g, 3) * 32 + M + lax.rem(g, 3) * 8, 8)
            l_v[pl.ds(lr, 8), :] = xn[j * 8:(j + 1) * 8, :]
        relayout(cn)

        @pl.when(c + 1 + NST < NCH)
        def _():
            st_start(c + 1 + NST)

        return carry

    lax.fori_loop(0, NCH, pro, 0)

    wg_copy.start()
    wu_copy.start()
    wd_copy.start()
    mem0_copy.wait()
    wo_copy.wait()

    def step(s, carry):
        slot = lax.rem(s, NS)
        oslot = lax.rem(s, NO)
        lhs = l_v[pl.ds(pl.multiple_of(s * 32, 32), 32), :]
        qdst = []
        for j in range(3):
            t0 = PRE + s * TPS + 8 * j
            qdst.append((lax.rem(lax.div(t0, SEG), NS), M + lax.rem(t0, SEG)))
        odst = []
        for j in range(4):
            g = 4 * s + j
            r_ring = lax.rem(lax.div(g, 3), NO) * 32 + M + lax.rem(g, 3) * 8
            r_epi = (NO + s - (NSEG - NE)) * 32 + 8 * j
            odst.append(pl.multiple_of(jnp.where(s < NSEG - NE, r_ring, r_epi), 8))
        orow = pl.multiple_of(oslot * 32, 32)

        def qkv(p):
            for t in range(3):
                w = pltpu.bitcast(wqkv[3 * p + t], BF16)
                y = jnp.dot(lhs, w, preferred_element_type=F32).astype(BF16)
                for hh in range(2):
                    yc = y[:, hh * E:(hh + 1) * E]
                    ring[slot, t, p, hh * 40:hh * 40 + M, :] = yc[0:M]
                    for j in range(3):
                        qs, qr = qdst[j]
                        ring[qs, t, p, pl.ds(pl.multiple_of(hh * 40 + qr, 8), 8), :] = (
                            yc[M + 8 * j:M + 8 * j + 8])

        def attn_a(q, k):
            sc = lax.dot_general(q, k, (((1,), (1,)), ((), ())), preferred_element_type=F32)
            fill = fill_v[...]
            sc = jnp.where(fill == 0.0, sc * SCALE, fill)
            mx = jnp.max(sc, axis=-1, keepdims=True)
            e = jnp.exp(sc - mx)
            den = jnp.sum(e, axis=-1, keepdims=True)
            return e.astype(BF16), pl.reciprocal(den, approx=True)

        def attn_b(p, e, inv, v):
            o = jnp.dot(e, v, preferred_element_type=F32)
            o = (o * inv).astype(BF16)
            oc = o_vs[p // PPC]
            for hh in range(2):
                cs = (2 * (p % PPC) + hh) * E
                oc[pl.ds(orow, M), cs:cs + E] = o[hh * 40:hh * 40 + M]
                for j in range(4):
                    oc[pl.ds(odst[j], 8), cs:cs + E] = o[hh * 40 + M + 8 * j:hh * 40 + M + 8 * j + 8]

        def wo_chunk(c):
            a = o_vs[c][pl.ds(orow, 32), :]
            w = pltpu.bitcast(wo_v[c * KC // 2:(c + 1) * KC // 2, :], BF16)
            return jnp.dot(a, w, preferred_element_type=F32)

        pe = {}
        for p in range(NP):
            if p >= 1:
                q, k = ring[slot, 0, p - 1], ring[slot, 1, p - 1]
            if p >= 2:
                v = ring[slot, 2, p - 2]
            qkv(p)
            if p >= 1:
                pe[p - 1] = attn_a(q, k)
            if p >= 2:
                attn_b(p - 2, *pe.pop(p - 2), v)
        q, k = ring[slot, 0, NP - 1], ring[slot, 1, NP - 1]
        v14, v15 = ring[slot, 2, NP - 2], ring[slot, 2, NP - 1]
        acc = wo_chunk(0)
        pe[NP - 1] = attn_a(q, k)
        attn_b(NP - 2, *pe.pop(NP - 2), v14)
        acc = acc + wo_chunk(1)
        attn_b(NP - 1, *pe.pop(NP - 1), v15)
        acc = acc + wo_chunk(2)
        acc = acc + wo_chunk(3)
        l_v[pl.ds(pl.multiple_of(s * 32 + 32, 32), M), :] = acc[0:M].astype(BF16)
        r0 = pl.multiple_of(s * TPS, 8)
        x_v[pl.ds(r0, TPS), :] = (x_v[pl.ds(r0, TPS), :].astype(F32)
                                  + xn_v[pl.ds(r0, TPS), :].astype(F32)
                                  + acc[M:]).astype(BF16)
        return carry

    lax.fori_loop(0, NSEG, step, 0)

    r = r_v[...]
    idx = lax.broadcasted_iota(jnp.int32, (S, 1), 0).astype(F32)
    m1 = jnp.max(r, axis=0, keepdims=True)
    i1 = jnp.min(jnp.where(r == m1, idx, float(S - 1)), axis=0, keepdims=True)
    r2 = jnp.where(idx == i1, -jnp.inf, r)
    m2 = jnp.max(r2, axis=0, keepdims=True)
    i2 = jnp.min(jnp.where((r2 == m2) & (idx != i1), idx, float(S - 1)), axis=0, keepdims=True)
    sel = []
    for iv in (i1, i2):
        i = jnp.clip(jnp.max(iv).astype(jnp.int32), 0, S - 1)
        sel.append((pl.multiple_of(lax.div(i, 8) * 8, 8), lax.rem(i, 8), i))
    row8 = lax.broadcasted_iota(jnp.int32, (8, D), 0)
    rows = []
    for base, off, _ in sel:
        blk = xn_v[pl.ds(base, 8), :].astype(F32)
        rows.append(jnp.sum(jnp.where(row8 == off, blk, 0.0), axis=0, keepdims=True))
    row16 = lax.broadcasted_iota(jnp.int32, (16, D), 0)
    xs = jnp.where(row16 == 0, rows[0], jnp.where(row16 == 1, rows[1], 0.0)).astype(BF16)
    wg_copy.wait()
    wu_copy.wait()
    wd_copy.wait()
    gp = _rb(jnp.dot(xs, pltpu.bitcast(wg_v[...], BF16), preferred_element_type=F32))
    up = _rb(jnp.dot(xs, pltpu.bitcast(wu_v[...], BF16), preferred_element_type=F32))
    g = _rb(gp * (1.0 / (1.0 + jnp.exp(-gp))))
    hm = (g * up).astype(BF16)
    y = _rb(jnp.dot(hm, pltpu.bitcast(wd_v[...], BF16), preferred_element_type=F32))
    for n, ((base, off, i), mv) in enumerate(zip(sel, (m1, m2))):
        gate = _rb(1.0 / (1.0 + jnp.exp(-mv)))
        upd = _rb(y[n:n + 1, :] * gate)
        done = i < S - PRE
        hit = row8 == off
        x_v[pl.ds(base, 8), :] = (x_v[pl.ds(base, 8), :].astype(F32)
                                  + jnp.where(hit & done, upd, 0.0)).astype(BF16)
        xn_v[pl.ds(base, 8), :] = (xn_v[pl.ds(base, 8), :].astype(F32)
                                   + jnp.where(hit & jnp.logical_not(done), upd, 0.0)).astype(BF16)

    def out_copy(r0, n, k):
        return pltpu.make_async_copy(x_v.at[pl.ds(r0, n)], out_hbm.at[pl.ds(r0, n)], sem_o.at[k])

    out_copy(0, S - PRE, 0).start()

    def epi(b, carry):
        ar = pl.ds(pl.multiple_of(NO * 32 + b * 128, 32), 128)
        a = jnp.concatenate([oc[ar, :] for oc in o_vs], axis=1)
        acc = jnp.dot(a, pltpu.bitcast(wo_v[...], BF16), preferred_element_type=F32)
        r0 = pl.multiple_of(S - PRE + b * 128, 128)
        x_v[pl.ds(r0, 128), :] = (x_v[pl.ds(r0, 128), :].astype(F32)
                                  + xn_v[pl.ds(r0, 128), :].astype(F32) + acc).astype(BF16)
        out_copy(r0, 128, 1 + b).start()
        return carry

    lax.fori_loop(0, PRE // 128, epi, 0)
    out_copy(0, S - PRE, 0).wait()
    for b in range(PRE // 128):
        out_copy(S - PRE + b * 128, 128, 1 + b).wait()


@jax.jit
def pallas_parallel_sum__memory_aug_recurrent_mem_tr__moe_arch_mod__prompt_kernel(
    A_x: jax.Array,
    A_mem0: jax.Array,
    A_Wq: jax.Array,
    A_Wk: jax.Array,
    A_Wv: jax.Array,
    A_Wo: jax.Array,
    A_seg_len: jax.Array,
    B_x: jax.Array,
    B_w_r: jax.Array,
    B_w_gate: jax.Array,
    B_w_up: jax.Array,
    B_w_down: jax.Array,
):
    del A_seg_len, B_x
    assert A_x.shape == (1, S, D) and A_Wq.shape == (D, H, E) and A_mem0.shape == (1, M, D)
    wshape = (D // 2, 2, NP, 2, E)
    any_spec = pl.BlockSpec(memory_space=pl.ANY)
    out = pl.pallas_call(
        _kernel,
        out_shape=jax.ShapeDtypeStruct((S, D), BF16),
        in_specs=[any_spec] * 10,
        out_specs=any_spec,
        scratch_shapes=[
            pltpu.VMEM((S, D), BF16),
            pltpu.VMEM((S, D), BF16),
            pltpu.VMEM((S + 32, D), BF16),
            pltpu.VMEM((NS, 3, NP, L2, E), BF16),
            *[pltpu.VMEM(((NO + NE) * 32, KC), BF16)] * NOC,
            pltpu.VMEM((NCH, D // 2, 2 * E), U32),
            pltpu.VMEM((H * E // 2, D), U32),
            pltpu.VMEM((NST, 2, D // 2, E), U32),
            pltpu.VMEM((D // 2, FF), U32),
            pltpu.VMEM((D // 2, FF), U32),
            pltpu.VMEM((FF // 2, D), U32),
            pltpu.VMEM((S, 1), F32),
            pltpu.VMEM((1, D), BF16),
            pltpu.VMEM((L2, L2), F32),
            pltpu.SemaphoreType.DMA((S // XCH,)),
            pltpu.SemaphoreType.DMA((2,)),
            pltpu.SemaphoreType.DMA((NST, 2)),
            pltpu.SemaphoreType.DMA((4,)),
            pltpu.SemaphoreType.DMA((1 + PRE // 128,)),
        ],
        compiler_params=pltpu.CompilerParams(vmem_limit_bytes=120 * 1024 * 1024),
    )(
        A_x.reshape(S, D),
        A_mem0.reshape(M, D),
        A_Wq.reshape(wshape),
        A_Wk.reshape(wshape),
        A_Wv.reshape(wshape),
        A_Wo.reshape(H * E, D),
        B_w_r.reshape(1, D),
        B_w_gate,
        B_w_up,
        B_w_down,
    )
    return out.reshape(1, S, D)
```

```python
import functools
import os

import jax
import jax.numpy as jnp
from jax import lax
import jax.experimental.pallas as pl
import jax.experimental.pallas.tpu as pltpu

OPT = dict(kv.split('=') for kv in os.environ.get('KOPT', '').split(',') if kv)


def opt(k, d):
    return int(OPT.get(k, d))


class _NoScope:
    def __enter__(self):
        return self

    def __exit__(self, *a):
        return False


def scope(name):
    return jax.named_scope(name) if opt('scopes', 0) else _NoScope()


F32 = jnp.float32
BF16 = jnp.bfloat16
U32 = jnp.uint32

S = 2048
D = 1024
H = 32
E = 128
M = 8
SEG = 32
NSEG = S // SEG
FF = 3584
NP = H // 2
L2 = 2 * (M + SEG)

PRE = 512
TPS = 24
NS = 17
NO = 17
NE = PRE // SEG
NST = 2
NCH = 3 * NP
NOC = opt('noc', 8)
KC = H * E // NOC
PPC = NP // NOC
XA = 128
XBR = (S - PRE) // NP
WOP = (H * E // 2) // NP

EPS = 1e-05
SCALE = float(E) ** -0.5


def _rb(v):
    return v.astype(BF16).astype(F32)


def _layernorm_rows(xb, wr):
    xf = xb.astype(F32)
    mean = jnp.sum(xf, axis=-1, keepdims=True) * (1.0 / D)
    xc = xf - mean
    var = jnp.sum(xc * xc, axis=-1, keepdims=True) * (1.0 / D)
    den = _rb(jnp.sqrt(_rb(_rb(var) + EPS)))
    d = _rb(xf - _rb(mean))
    xn = (d * (1.0 / den)).astype(BF16)
    r = _rb(jnp.sum(xn.astype(F32) * wr, axis=-1, keepdims=True))
    return xn, r


def _scatter_scores(acc, r, g0):
    lane = lax.broadcasted_iota(jnp.int32, acc.shape, 1)
    for j in range(r.shape[0] // 8):
        acc = jnp.where(lane == g0 + j, r[j * 8:(j + 1) * 8, :], acc)
    return acc


def _kernel(x_hbm, mem0_hbm, wq_hbm, wk_hbm, wv_hbm, wo_hbm, wr_hbm, wg_hbm, wu_hbm, wd_hbm,
            out_hbm,
            x_v, xn_v, xp_v, l_v, ring, wqkv, wo_v, stage, wc0, wc1, wc2, wg_v, wu_v, wd_v, wr_v, fill_v,
            sem_xa, sem_xb, sem_s, sem_st, sem_wo, sem_w, sem_o, *o_vs):
    w32 = [w.bitcast(U32) for w in (wq_hbm, wk_hbm, wv_hbm)]
    wo32 = wo_hbm.bitcast(U32)
    wcur = (wc0, wc1, wc2)

    def xa_copy(c):
        return pltpu.make_async_copy(x_hbm.at[pl.ds(c * XA, XA)], x_v.at[pl.ds(c * XA, XA)],
                                     sem_xa.at[c])

    xc_copy = pltpu.make_async_copy(x_hbm.at[pl.ds(PRE, TPS)], x_v.at[pl.ds(PRE, TPS)], sem_s.at[2])

    def xb_copy(i):
        r0 = pl.multiple_of(PRE + i * XBR, 32)
        return pltpu.make_async_copy(x_hbm.at[pl.ds(r0, XBR)], x_v.at[pl.ds(r0, XBR)], sem_xb)

    def st_copy(t, p, slot, k, dp):
        return pltpu.make_async_copy(w32[t].at[:, dp, p, 0, :], stage.at[slot, k, dp],
                                     sem_st.at[slot, k, dp])

    def grp_copies(g):
        slot = lax.rem(g, NST)
        cps = []
        for k, (t, p) in enumerate(((1, g), (2, g), (0, g + 1))):
            p = jnp.minimum(p, NP - 1)
            cps += [st_copy(t, p, slot, k, 0), st_copy(t, p, slot, k, 1)]
        return cps

    def wo_copy(i):
        r0 = pl.multiple_of(i * WOP, 8)
        return pltpu.make_async_copy(wo32.at[pl.ds(r0, WOP)], wo_v.at[pl.ds(r0, WOP)], sem_wo)

    mem0_copy = pltpu.make_async_copy(mem0_hbm, l_v.at[pl.ds(0, M)], sem_s.at[0])
    wr_copy = pltpu.make_async_copy(wr_hbm, wr_v, sem_s.at[1])
    first_copies = [st_copy(0, 0, NST, 0, 0), st_copy(0, 0, NST, 0, 1)]
    wg_copy = pltpu.make_async_copy(wg_hbm.bitcast(U32), wg_v, sem_w.at[0])
    wu_copy = pltpu.make_async_copy(wu_hbm.bitcast(U32), wu_v, sem_w.at[1])
    wd_copy = pltpu.make_async_copy(wd_hbm.bitcast(U32), wd_v, sem_w.at[2])

    xa_copy(0).start()
    wr_copy.start()
    for c in range(1, PRE // XA):
        xa_copy(c).start()
    xc_copy.start()
    for cp in first_copies:
        cp.start()
    for cp in grp_copies(0):
        cp.start()
    mem0_copy.start()

    row = lax.broadcasted_iota(jnp.int32, (L2, L2), 0)
    col = lax.broadcasted_iota(jnp.int32, (L2, L2), 1)
    rl = jnp.where(row >= L2 // 2, row - L2 // 2, row)
    cl = jnp.where(col >= L2 // 2, col - L2 // 2, col)
    same = (row >= L2 // 2) == (col >= L2 // 2)
    keep = (rl < M) | (rl >= cl)
    fill_v[...] = jnp.where(same, jnp.where(keep, 0.0, -1000000000.0), -jnp.inf).astype(F32)

    with scope('wait_wr'):
        wr_copy.wait()
        if opt('w0', 0):
            xa_copy(0).wait()
            xa_copy(0).start()

    def ln0(i, racc):
        xa_copy(i).wait()
        for j in range(XA // 32):
            r0 = pl.multiple_of(i * XA + j * 32, 32)
            xn, r = _layernorm_rows(x_v[pl.ds(r0, 32), :], wr_v[...].astype(F32))
            xn_v[pl.ds(r0, 32), :] = xn
            xp_v[pl.ds(r0, 32), :] = xn
            racc = _scatter_scores(racc, r, i * (XA // 8) + j * 4)
        return racc

    with scope('ln0'):
        racc = lax.fori_loop(0, PRE // XA, ln0, jnp.zeros((8, S // 8), F32))

    def ln_step(i, racc):
        ic = jnp.minimum(i, NSEG - 1)
        r0 = pl.multiple_of(PRE + ic * TPS, 8)
        xn, r = _layernorm_rows(x_v[pl.ds(r0, TPS), :], wr_v[...].astype(F32))
        xn_v[pl.ds(r0, TPS), :] = xn
        l_v[pl.ds(pl.multiple_of(i * 32 + M, 8), TPS), :] = xn
        return _scatter_scores(racc, r, PRE // 8 + ic * (TPS // 8))

    with scope('ln_s0'):
        xc_copy.wait()
        racc = ln_step(0, racc)

    def relayout(slot, k, c, dst):
        for j in range(D // 2 // 64):
            a = stage[slot, k, 0, j * 64:(j + 1) * 64, :]
            b = stage[slot, k, 1, j * 64:(j + 1) * 64, :]
            ev = (a & jnp.uint32(0xFFFF)) | (b << 16)
            od = (a >> 16) | (b & jnp.uint32(0xFFFF0000))
            dst[j * 64:(j + 1) * 64, 0:E] = ev
            dst[j * 64:(j + 1) * 64, E:2 * E] = od
            wqkv[c, j * 64:(j + 1) * 64, 0:E] = ev
            wqkv[c, j * 64:(j + 1) * 64, E:2 * E] = od

    with scope('pre_pro'):
        for cp in first_copies:
            cp.wait()
        relayout(NST, 0, 0, wc0)

    MB = opt('promb', 128)

    def pro(p, carry):
        for cp in grp_copies(p):
            cp.wait()
        for cp in grp_copies(p + 1):
            cp.start()
        wo_copy(p).start()
        xb_copy(p).start()

        slot = lax.rem(p, NST)
        for t in range(3):
            relayout(slot, t, 3 * p + t + 1, wcur[(t + 1) % 3])
            for rb in range(PRE // MB):
                w = pltpu.bitcast(wcur[t][...], BF16)
                y = jnp.dot(xp_v[rb * MB:(rb + 1) * MB, :], w, preferred_element_type=F32)
                y = y.astype(BF16)
                for sg in range(MB // 32):
                    for hh in range(2):
                        ring[rb * (MB // 32) + sg, t, p, hh * 40 + M:hh * 40 + 40, :] = (
                            y[sg * 32:(sg + 1) * 32, hh * E:(hh + 1) * E])
        return carry

    xb_all = pltpu.make_async_copy(x_hbm.at[pl.ds(PRE, S - PRE)], x_v.at[pl.ds(PRE, S - PRE)], sem_xb)
    with scope('pro'):
        lax.fori_loop(0, NP, pro, 0)

    for cp in grp_copies(NP):
        cp.wait()
    xb_all.wait()
    wg_copy.start()
    wu_copy.start()
    wd_copy.start()
    mem0_copy.wait()
    pltpu.make_async_copy(wo32, wo_v, sem_wo).wait()

    def step(s, racc):
        slot = lax.rem(s, NS)
        oslot = lax.rem(s, NO)
        lhs = l_v[pl.ds(pl.multiple_of(s * 32, 32), 32), :]
        qdst = []
        for j in range(3):
            t0 = PRE + s * TPS + 8 * j
            qdst.append((lax.rem(lax.div(t0, SEG), NS), M + lax.rem(t0, SEG)))
        odst = []
        for j in range(4):
            g = 4 * s + j
            r_ring = lax.rem(lax.div(g, 3), NO) * 32 + M + lax.rem(g, 3) * 8
            r_epi = (NO + s - (NSEG - NE)) * 32 + 8 * j
            odst.append(pl.multiple_of(jnp.where(s < NSEG - NE, r_ring, r_epi), 8))
        orow = pl.multiple_of(oslot * 32, 32)

        def qkv(p):
            for t in range(3):
                w = pltpu.bitcast(wqkv[3 * p + t], BF16)
                y = jnp.dot(lhs, w, preferred_element_type=F32).astype(BF16)
                for hh in range(2):
                    yc = y[:, hh * E:(hh + 1) * E]
                    ring[slot, t, p, hh * 40:hh * 40 + M, :] = yc[0:M]
                    for j in range(3):
                        qs, qr = qdst[j]
                        ring[qs, t, p, pl.ds(pl.multiple_of(hh * 40 + qr, 8), 8), :] = (
                            yc[M + 8 * j:M + 8 * j + 8])

        PRENORM = opt('prenorm', 0)
        LAGA = opt('laga', 1)
        LAGB = opt('lagb', 2)

        def attn_a(q, k):
            sc = lax.dot_general(q, k, (((1,), (1,)), ((), ())), preferred_element_type=F32)
            fill = fill_v[...]
            sc = jnp.where(fill == 0.0, sc * SCALE, fill)
            mx = jnp.max(sc, axis=-1, keepdims=True)
            e = jnp.exp(sc - mx)
            den = jnp.sum(e, axis=-1, keepdims=True)
            inv = pl.reciprocal(den, approx=True)
            if PRENORM:
                return (e * inv).astype(BF16), None
            return e.astype(BF16), inv

        def attn_b(p, e, inv, v):
            o = jnp.dot(e, v, preferred_element_type=F32)
            if inv is not None:
                o = o * inv
            o = o.astype(BF16)
            oc = o_vs[p // PPC]
            for hh in range(2):
                cs = (2 * (p % PPC) + hh) * E
                oc[pl.ds(orow, M), cs:cs + E] = o[hh * 40:hh * 40 + M]
                for j in range(4):
                    oc[pl.ds(odst[j], 8), cs:cs + E] = o[hh * 40 + M + 8 * j:hh * 40 + M + 8 * j + 8]

        def wo_chunk(c):
            a = o_vs[c][pl.ds(orow, 32), :]
            w = pltpu.bitcast(wo_v[c * KC // 2:(c + 1) * KC // 2, :], BF16)
            return jnp.dot(a, w, preferred_element_type=F32)

        pe = {}
        acc = None
        for p in range(NP):
            pa, pb = p - LAGA, p - LAGB
            if 0 <= pa < NP:
                q, k = ring[slot, 0, pa], ring[slot, 1, pa]
            if 0 <= pb < NP:
                v = ring[slot, 2, pb]
            qkv(p)
            if 0 <= pa < NP:
                pe[pa] = attn_a(q, k)
            if 0 <= pb < NP:
                attn_b(pb, *pe.pop(pb), v)
        for tok in OPT.get('tail', 'W0.W1.A15.B14.W2.W3.W4.B15.W5.W6.W7').split('.'):
            i = int(tok[1:])
            if tok[0] == 'W':
                y = wo_chunk(i)
                acc = y if acc is None else acc + y
            elif tok[0] == 'A':
                pe[i] = attn_a(ring[slot, 0, i], ring[slot, 1, i])
            else:
                attn_b(i, *pe.pop(i), ring[slot, 2, i])
        assert not pe
        r0 = pl.multiple_of(s * TPS, 8)
        base = x_v[pl.ds(r0, TPS), :].astype(F32) + xn_v[pl.ds(r0, TPS), :].astype(F32)
        racc = ln_step(s + 1, racc)
        l_v[pl.ds(pl.multiple_of(s * 32 + 32, 32), M), :] = acc[0:M].astype(BF16)
        x_v[pl.ds(r0, TPS), :] = (base + acc[M:]).astype(BF16)
        return racc

    with scope('main'):
        racc = lax.fori_loop(0, NSEG, step, racc)

    with scope('moe'):
        r = racc
        idx = (lax.broadcasted_iota(jnp.int32, r.shape, 1) * 8
               + lax.broadcasted_iota(jnp.int32, r.shape, 0)).astype(F32)

        def allred(fn, v):
            return fn(fn(v, axis=1, keepdims=True), axis=0, keepdims=True)

        m1 = allred(jnp.max, r)
        i1 = allred(jnp.min, jnp.where(r == m1, idx, float(S - 1)))
        r2 = jnp.where(idx == i1, -jnp.inf, r)
        m2 = allred(jnp.max, r2)
        i2 = allred(jnp.min, jnp.where((r2 == m2) & (idx != i1), idx, float(S - 1)))
        sel = []
        for iv in (i1, i2):
            i = jnp.clip(jnp.max(iv).astype(jnp.int32), 0, S - 1)
            sel.append((pl.multiple_of(lax.div(i, 8) * 8, 8), lax.rem(i, 8), i))
        row8 = lax.broadcasted_iota(jnp.int32, (8, D), 0)
        rows = []
        for base, off, _ in sel:
            blk = xn_v[pl.ds(base, 8), :].astype(F32)
            rows.append(jnp.sum(jnp.where(row8 == off, blk, 0.0), axis=0, keepdims=True))
        row16 = lax.broadcasted_iota(jnp.int32, (16, D), 0)
        xs = jnp.where(row16 == 0, rows[0], jnp.where(row16 == 1, rows[1], 0.0)).astype(BF16)
        wg_copy.wait()
        wu_copy.wait()
        wd_copy.wait()
        gp = _rb(jnp.dot(xs, pltpu.bitcast(wg_v[...], BF16), preferred_element_type=F32))
        up = _rb(jnp.dot(xs, pltpu.bitcast(wu_v[...], BF16), preferred_element_type=F32))
        g = _rb(gp * (1.0 / (1.0 + jnp.exp(-gp))))
        hm = (g * up).astype(BF16)
        y = _rb(jnp.dot(hm, pltpu.bitcast(wd_v[...], BF16), preferred_element_type=F32))
        for n, ((base, off, i), mv) in enumerate(zip(sel, (m1, m2))):
            gate = _rb(1.0 / (1.0 + jnp.exp(-mv)))
            upd = _rb(y[n:n + 1, :] * gate)
            done = i < S - PRE
            hit = row8 == off
            x_v[pl.ds(base, 8), :] = (x_v[pl.ds(base, 8), :].astype(F32)
                                      + jnp.where(hit & done, upd, 0.0)).astype(BF16)
            xn_v[pl.ds(base, 8), :] = (xn_v[pl.ds(base, 8), :].astype(F32)
                                       + jnp.where(hit & jnp.logical_not(done), upd, 0.0)).astype(BF16)

    def out_copy(r0, n, k):
        return pltpu.make_async_copy(x_v.at[pl.ds(r0, n)], out_hbm.at[pl.ds(r0, n)], sem_o.at[k])

    out_copy(0, S - PRE, 0).start()

    def epi(b, carry):
        ar = pl.ds(pl.multiple_of(NO * 32 + b * 128, 32), 128)
        a = jnp.concatenate([oc[ar, :] for oc in o_vs], axis=1)
        acc = jnp.dot(a, pltpu.bitcast(wo_v[...], BF16), preferred_element_type=F32)
        r0 = pl.multiple_of(S - PRE + b * 128, 128)
        x_v[pl.ds(r0, 128), :] = (x_v[pl.ds(r0, 128), :].astype(F32)
                                  + xn_v[pl.ds(r0, 128), :].astype(F32) + acc).astype(BF16)
        out_copy(r0, 128, 1 + b).start()
        return carry

    with scope('epi'):
        lax.fori_loop(0, PRE // 128, epi, 0)
    with scope('fin'):
        out_copy(0, S - PRE, 0).wait()
        for b in range(PRE // 128):
            out_copy(S - PRE + b * 128, 128, 1 + b).wait()


@jax.jit
def pallas_parallel_sum__memory_aug_recurrent_mem_tr__moe_arch_mod__prompt_kernel(
    A_x: jax.Array,
    A_mem0: jax.Array,
    A_Wq: jax.Array,
    A_Wk: jax.Array,
    A_Wv: jax.Array,
    A_Wo: jax.Array,
    A_seg_len: jax.Array,
    B_x: jax.Array,
    B_w_r: jax.Array,
    B_w_gate: jax.Array,
    B_w_up: jax.Array,
    B_w_down: jax.Array,
):
    del A_seg_len, B_x
    assert A_x.shape == (1, S, D) and A_Wq.shape == (D, H, E) and A_mem0.shape == (1, M, D)
    wshape = (D // 2, 2, NP, 2, E)
    any_spec = pl.BlockSpec(memory_space=pl.ANY)
    out = pl.pallas_call(
        _kernel,
        out_shape=jax.ShapeDtypeStruct((S, D), BF16),
        in_specs=[any_spec] * 10,
        out_specs=any_spec,
        scratch_shapes=[
            pltpu.VMEM((S, D), BF16),
            pltpu.VMEM((S, D), BF16),
            pltpu.VMEM((PRE, D), BF16),
            pltpu.VMEM((S + 32, D), BF16),
            pltpu.VMEM((NS, 3, NP, L2, E), BF16),
            pltpu.VMEM((NCH + 1, D // 2, 2 * E), U32),
            pltpu.VMEM((H * E // 2, D), U32),
            pltpu.VMEM((NST + 1, 3, 2, D // 2, E), U32),
            pltpu.VMEM((D // 2, 2 * E), U32),
            pltpu.VMEM((D // 2, 2 * E), U32),
            pltpu.VMEM((D // 2, 2 * E), U32),
            pltpu.VMEM((D // 2, FF), U32),
            pltpu.VMEM((D // 2, FF), U32),
            pltpu.VMEM((FF // 2, D), U32),
            pltpu.VMEM((1, D), BF16),
            pltpu.VMEM((L2, L2), F32),
            pltpu.SemaphoreType.DMA((PRE // XA,)),
            pltpu.SemaphoreType.DMA,
            pltpu.SemaphoreType.DMA((3,)),
            pltpu.SemaphoreType.DMA((NST + 1, 3, 2)),
            pltpu.SemaphoreType.DMA,
            pltpu.SemaphoreType.DMA((3,)),
            pltpu.SemaphoreType.DMA((1 + PRE // 128,)),
            *[pltpu.VMEM(((NO + NE) * 32, KC), BF16)] * NOC,
        ],
        compiler_params=pltpu.CompilerParams(vmem_limit_bytes=120 * 1024 * 1024,
                                             disable_bounds_checks=bool(opt('nobc', 1)),
                                             shape_invariant_numerics=bool(opt('sin', 1))),
    )(
        A_x.reshape(S, D),
        A_mem0.reshape(M, D),
        A_Wq.reshape(wshape),
        A_Wk.reshape(wshape),
        A_Wv.reshape(wshape),
        A_Wo.reshape(H * E, D),
        B_w_r.reshape(1, D),
        B_w_gate,
        B_w_up,
        B_w_down,
    )
    return out.reshape(1, S, D)
```

```python
import functools
import os

import jax
import jax.numpy as jnp
from jax import lax
import jax.experimental.pallas as pl
import jax.experimental.pallas.tpu as pltpu

OPT = dict(kv.split('=') for kv in os.environ.get('KOPT', '').split(',') if kv)


def opt(k, d):
    return int(OPT.get(k, d))


class _NoScope:
    def __enter__(self):
        return self

    def __exit__(self, *a):
        return False


def scope(name):
    return jax.named_scope(name) if opt('scopes', 0) else _NoScope()


F32 = jnp.float32
BF16 = jnp.bfloat16
U32 = jnp.uint32

S = 2048
D = 1024
H = 32
E = 128
M = 8
SEG = 32
NSEG = S // SEG
FF = 3584
NP = H // 2
L2 = 2 * (M + SEG)

PRE = 512
TPS = 24
NS = 17
NO = 17
NE = PRE // SEG
NST = 2
NCH = 3 * NP
NOC = opt('noc', 8)
KC = H * E // NOC
PPC = NP // NOC
XA = 128
XBR = (S - PRE) // NP
WOP = (H * E // 2) // NP

EPS = 1e-05
SCALE = float(E) ** -0.5


def _rb(v):
    return v.astype(BF16).astype(F32)


def _layernorm_rows(xb, wr):
    xf = xb.astype(F32)
    mean = jnp.sum(xf, axis=-1, keepdims=True) * (1.0 / D)
    xc = xf - mean
    var = jnp.sum(xc * xc, axis=-1, keepdims=True) * (1.0 / D)
    den = _rb(jnp.sqrt(_rb(_rb(var) + EPS)))
    d = _rb(xf - _rb(mean))
    xn = (d * (1.0 / den)).astype(BF16)
    r = _rb(jnp.sum(xn.astype(F32) * wr, axis=-1, keepdims=True))
    return xn, r


def _scatter_scores(acc, r, g0):
    lane = lax.broadcasted_iota(jnp.int32, acc.shape, 1)
    for j in range(r.shape[0] // 8):
        acc = jnp.where(lane == g0 + j, r[j * 8:(j + 1) * 8, :], acc)
    return acc


def _kernel(x_hbm, mem0_hbm, wq_hbm, wk_hbm, wv_hbm, wo_hbm, wr_hbm, wg_hbm, wu_hbm, wd_hbm,
            out_hbm,
            x_v, xn_v, xp_v, l_v, ring, wqkv, wo_v, stage, wc0, wc1, wc2, wg_v, wu_v, wd_v, wr_v, fill_v,
            sem_xa, sem_xb, sem_s, sem_st, sem_wo, sem_w, sem_o, *o_vs):
    w32 = [w.bitcast(U32) for w in (wq_hbm, wk_hbm, wv_hbm)]
    wo32 = wo_hbm.bitcast(U32)
    wcur = (wc0, wc1, wc2)

    def xa_copy(c):
        return pltpu.make_async_copy(x_hbm.at[pl.ds(c * XA, XA)], x_v.at[pl.ds(c * XA, XA)],
                                     sem_xa.at[c])

    xc_copy = pltpu.make_async_copy(x_hbm.at[pl.ds(PRE, TPS)], x_v.at[pl.ds(PRE, TPS)], sem_s.at[2])

    def xb_copy(i):
        r0 = pl.multiple_of(PRE + i * XBR, 32)
        return pltpu.make_async_copy(x_hbm.at[pl.ds(r0, XBR)], x_v.at[pl.ds(r0, XBR)], sem_xb)

    def st_copy(t, p, slot, k, dp):
        return pltpu.make_async_copy(w32[t].at[:, dp, p, 0, :], stage.at[slot, k, dp],
                                     sem_st.at[slot, k, dp])

    def grp_copies(g):
        slot = lax.rem(g, NST)
        cps = []
        for k, (t, p) in enumerate(((1, g), (2, g), (0, g + 1))):
            p = jnp.minimum(p, NP - 1)
            cps += [st_copy(t, p, slot, k, 0), st_copy(t, p, slot, k, 1)]
        return cps

    def wo_copy(i):
        r0 = pl.multiple_of(i * WOP, 8)
        return pltpu.make_async_copy(wo32.at[pl.ds(r0, WOP)], wo_v.at[pl.ds(r0, WOP)], sem_wo)

    mem0_copy = pltpu.make_async_copy(mem0_hbm, l_v.at[pl.ds(0, M)], sem_s.at[0])
    wr_copy = pltpu.make_async_copy(wr_hbm, wr_v, sem_s.at[1])
    first_copies = [st_copy(0, 0, NST, 0, 0), st_copy(0, 0, NST, 0, 1)]
    wg_copy = pltpu.make_async_copy(wg_hbm.bitcast(U32), wg_v, sem_w.at[0])
    wu_copy = pltpu.make_async_copy(wu_hbm.bitcast(U32), wu_v, sem_w.at[1])
    wd_copy = pltpu.make_async_copy(wd_hbm.bitcast(U32), wd_v, sem_w.at[2])

    xa_copy(0).start()
    wr_copy.start()
    for c in range(1, PRE // XA):
        xa_copy(c).start()
    xc_copy.start()
    for cp in first_copies:
        cp.start()
    for cp in grp_copies(0):
        cp.start()
    mem0_copy.start()

    row = lax.broadcasted_iota(jnp.int32, (L2, L2), 0)
    col = lax.broadcasted_iota(jnp.int32, (L2, L2), 1)
    rl = jnp.where(row >= L2 // 2, row - L2 // 2, row)
    cl = jnp.where(col >= L2 // 2, col - L2 // 2, col)
    same = (row >= L2 // 2) == (col >= L2 // 2)
    keep = (rl < M) | (rl >= cl)
    fill_v[...] = jnp.where(same, jnp.where(keep, 0.0, -1000000000.0), -jnp.inf).astype(F32)

    with scope('wait_wr'):
        wr_copy.wait()
        if opt('w0', 0):
            xa_copy(0).wait()
            xa_copy(0).start()

    def ln0(i, racc):
        xa_copy(i).wait()
        for j in range(XA // 32):
            r0 = pl.multiple_of(i * XA + j * 32, 32)
            xn, r = _layernorm_rows(x_v[pl.ds(r0, 32), :], wr_v[...].astype(F32))
            xn_v[pl.ds(r0, 32), :] = xn
            xp_v[pl.ds(r0, 32), :] = xn
            racc = _scatter_scores(racc, r, i * (XA // 8) + j * 4)
        return racc

    with scope('ln0'):
        racc = lax.fori_loop(0, PRE // XA, ln0, jnp.zeros((8, S // 8), F32))

    def ln_step(i, racc):
        ic = jnp.minimum(i, NSEG - 1)
        r0 = pl.multiple_of(PRE + ic * TPS, 8)
        xn, r = _layernorm_rows(x_v[pl.ds(r0, TPS), :], wr_v[...].astype(F32))
        xn_v[pl.ds(r0, TPS), :] = xn
        racc = _scatter_scores(racc, r, PRE // 8 + ic * (TPS // 8))
        if opt('tokval', 0):
            return racc, xn.astype(F32)
        l_v[pl.ds(pl.multiple_of(i * 32 + M, 8), TPS), :] = xn
        return racc, jnp.zeros((8, 128), F32)

    with scope('ln_s0'):
        xc_copy.wait()
        racc, tok0 = ln_step(0, racc)

    def relayout(slot, k, c, dst):
        for j in range(D // 2 // 64):
            a = stage[slot, k, 0, j * 64:(j + 1) * 64, :]
            b = stage[slot, k, 1, j * 64:(j + 1) * 64, :]
            ev = (a & jnp.uint32(0xFFFF)) | (b << 16)
            od = (a >> 16) | (b & jnp.uint32(0xFFFF0000))
            dst[j * 64:(j + 1) * 64, 0:E] = ev
            dst[j * 64:(j + 1) * 64, E:2 * E] = od
            wqkv[c, j * 64:(j + 1) * 64, 0:E] = ev
            wqkv[c, j * 64:(j + 1) * 64, E:2 * E] = od

    with scope('pre_pro'):
        for cp in first_copies:
            cp.wait()
        relayout(NST, 0, 0, wc0)

    MB = opt('promb', 128)

    def pro(p, carry):
        for cp in grp_copies(p):
            cp.wait()
        for cp in grp_copies(p + 1):
            cp.start()
        wo_copy(p).start()
        xb_copy(p).start()

        slot = lax.rem(p, NST)
        for t in range(3):
            relayout(slot, t, 3 * p + t + 1, wcur[(t + 1) % 3])
            for rb in range(PRE // MB):
                w = pltpu.bitcast(wcur[t][...], BF16)
                y = jnp.dot(xp_v[rb * MB:(rb + 1) * MB, :], w, preferred_element_type=F32)
                y = y.astype(BF16)
                for sg in range(MB // 32):
                    for hh in range(2):
                        ring[rb * (MB // 32) + sg, t, p, hh * 40 + M:hh * 40 + 40, :] = (
                            y[sg * 32:(sg + 1) * 32, hh * E:(hh + 1) * E])
        return carry

    xb_all = pltpu.make_async_copy(x_hbm.at[pl.ds(PRE, S - PRE)], x_v.at[pl.ds(PRE, S - PRE)], sem_xb)
    with scope('pro'):
        lax.fori_loop(0, NP, pro, 0)

    for cp in grp_copies(NP):
        cp.wait()
    xb_all.wait()
    wg_copy.start()
    wu_copy.start()
    wd_copy.start()
    mem0_copy.wait()
    pltpu.make_async_copy(wo32, wo_v, sem_wo).wait()

    def step(s, carry):
        racc, mem, tok = carry
        slot = lax.rem(s, NS)
        oslot = lax.rem(s, NO)
        top = l_v[pl.ds(pl.multiple_of(s * 32 + M, 8), 8), :].astype(F32)
        bot = l_v[pl.ds(pl.multiple_of(s * 32 + 16, 16), 16), :]

        def mk_lhs(m, lo, hi):
            return jnp.concatenate(
                [jnp.concatenate([m, top[:, lo:hi]], axis=0).astype(BF16), bot[:, lo:hi]], axis=0)

        ks = opt('ksplit', 0) * 128
        if ks:
            lhs_lo = mk_lhs(mem[:, :ks], 0, ks)
            part = [jnp.dot(lhs_lo, pltpu.bitcast(wqkv[t, 0:ks // 2, :], BF16),
                            preferred_element_type=F32) for t in range(3)]
            mem_hi = mem[:, ks:]
            if opt('dep', 1):
                dn = opt('depn', 0)
                dep = part[dn // 2][0:M, (dn % 2) * E:(dn % 2 + 1) * E]
                dep = jnp.concatenate([dep] * ((D - ks) // E), axis=1)
                mem_hi = jnp.where(dep != dep, dep, mem_hi)
            lhs = jnp.concatenate([lhs_lo, mk_lhs(mem_hi, ks, D)], axis=1)
        else:
            lhs = mk_lhs(mem, 0, D)
        qdst = []
        for j in range(3):
            t0 = PRE + s * TPS + 8 * j
            qdst.append((lax.rem(lax.div(t0, SEG), NS), M + lax.rem(t0, SEG)))
        odst = []
        for j in range(4):
            g = 4 * s + j
            r_ring = lax.rem(lax.div(g, 3), NO) * 32 + M + lax.rem(g, 3) * 8
            r_epi = (NO + s - (NSEG - NE)) * 32 + 8 * j
            odst.append(pl.multiple_of(jnp.where(s < NSEG - NE, r_ring, r_epi), 8))
        orow = pl.multiple_of(oslot * 32, 32)

        def qkv(p, ts=(0, 1, 2)):
            for t in ts:
                if p == 0 and ks:
                    y = part[t] + jnp.dot(lhs[:, ks:], pltpu.bitcast(wqkv[t, ks // 2:, :], BF16),
                                          preferred_element_type=F32)
                    y = y.astype(BF16)
                else:
                    w = pltpu.bitcast(wqkv[3 * p + t], BF16)
                    y = jnp.dot(lhs, w, preferred_element_type=F32).astype(BF16)
                for hh in range(2):
                    yc = y[:, hh * E:(hh + 1) * E]
                    ring[slot, t, p, hh * 40:hh * 40 + M, :] = yc[0:M]
                    for j in range(3):
                        qs, qr = qdst[j]
                        ring[qs, t, p, pl.ds(pl.multiple_of(hh * 40 + qr, 8), 8), :] = (
                            yc[M + 8 * j:M + 8 * j + 8])

        PRENORM = opt('prenorm', 1)
        LAGA = opt('laga', 1)
        LAGB = opt('lagb', 2)

        def attn_a(q, k):
            sc = lax.dot_general(q, k, (((1,), (1,)), ((), ())), preferred_element_type=F32)
            fill = fill_v[...]
            sc = jnp.where(fill == 0.0, sc * SCALE, fill)
            mx = jnp.max(sc, axis=-1, keepdims=True)
            e = jnp.exp(sc - mx)
            den = jnp.sum(e, axis=-1, keepdims=True)
            inv = pl.reciprocal(den, approx=True)
            if PRENORM:
                return (e * inv).astype(BF16), None
            return e.astype(BF16), inv

        def attn_b(p, e, inv, v):
            o = jnp.dot(e, v, preferred_element_type=F32)
            if inv is not None:
                o = o * inv
            o = o.astype(BF16)
            oc = o_vs[p // PPC]
            for hh in range(2):
                cs = (2 * (p % PPC) + hh) * E
                oc[pl.ds(orow, M), cs:cs + E] = o[hh * 40:hh * 40 + M]
                for j in range(4):
                    oc[pl.ds(odst[j], 8), cs:cs + E] = o[hh * 40 + M + 8 * j:hh * 40 + M + 8 * j + 8]

        def wo_chunk(c, c1):
            a = jnp.concatenate([o_vs[i][pl.ds(orow, 32), :] for i in range(c, c1)], axis=1)
            w = pltpu.bitcast(wo_v[c * KC // 2:c1 * KC // 2, :], BF16)
            return jnp.dot(a, w, preferred_element_type=F32)

        wl = OPT.get('wl', '0.1.2.3.4.5-7').split('.')
        nslot = 3 * NP + len(wl)
        ev = {n: [] for n in range(nslot + 1)}
        lq, aa, lv, bb = opt('lq', 2), opt('a', 4), opt('lv', 6), opt('b', 8)
        ta = [int(x) for x in OPT.get('ta', '50').split('.')]
        tb = [int(x) for x in OPT.get('tb', '51.52').split('.')]
        for p in range(NP):
            pa_ = 3 * p + aa if p < NP - len(ta) else ta[p - (NP - len(ta))]
            pb_ = 3 * p + bb if p < NP - len(tb) else tb[p - (NP - len(tb))]
            assert pa_ <= pb_ <= nslot
            ev[min(3 * p + lq, pa_)].append((0, 'Q', p))
            ev[min(3 * p + lv, pb_)].append((1, 'V', p))
            ev[pa_].append((3 if opt('bfirst', 1) else 2, 'A', p))
            ev[pb_].append((2 if opt('bfirst', 1) else 3, 'B', p))
        pe, qk, vv = {}, {}, {}
        acc = None
        for n in range(nslot + 1):
            for _, kind, p in sorted(ev[n]):
                if kind == 'Q':
                    qk[p] = (ring[slot, 0, p], ring[slot, 1, p])
                elif kind == 'V':
                    vv[p] = ring[slot, 2, p]
                elif kind == 'A':
                    pe[p] = attn_a(*qk.pop(p))
                else:
                    attn_b(p, *pe.pop(p), vv.pop(p))
            if n < 3 * NP:
                qkv(n // 3, (n % 3,))
            elif n < nslot:
                tk = wl[n - 3 * NP].split('-')
                y = wo_chunk(int(tk[0]), int(tk[-1]) + 1)
                acc = y if acc is None else acc + y
        assert not pe
        r0 = pl.multiple_of(s * TPS, 8)
        base = x_v[pl.ds(r0, TPS), :].astype(F32) + xn_v[pl.ds(r0, TPS), :].astype(F32)
        racc, tok = ln_step(s + 1, racc)
        x_v[pl.ds(r0, TPS), :] = (base + acc[M:]).astype(BF16)
        return racc, acc[0:M], tok

    with scope('main'):
        U = opt('unroll', 4)

        def steps(i, carry):
            for u in range(U):
                carry = step(i * U + u, carry)
            return carry

        racc, _, _ = lax.fori_loop(0, NSEG // U, steps, (racc, l_v[0:M, :].astype(F32), tok0))

    with scope('moe'):
        r = racc
        idx = (lax.broadcasted_iota(jnp.int32, r.shape, 1) * 8
               + lax.broadcasted_iota(jnp.int32, r.shape, 0)).astype(F32)

        def allred(fn, v):
            return fn(fn(v, axis=1, keepdims=True), axis=0, keepdims=True)

        m1 = allred(jnp.max, r)
        i1 = allred(jnp.min, jnp.where(r == m1, idx, float(S - 1)))
        r2 = jnp.where(idx == i1, -jnp.inf, r)
        m2 = allred(jnp.max, r2)
        i2 = allred(jnp.min, jnp.where((r2 == m2) & (idx != i1), idx, float(S - 1)))
        sel = []
        for iv in (i1, i2):
            i = jnp.clip(jnp.max(iv).astype(jnp.int32), 0, S - 1)
            sel.append((pl.multiple_of(lax.div(i, 8) * 8, 8), lax.rem(i, 8), i))
        row8 = lax.broadcasted_iota(jnp.int32, (8, D), 0)
        rows = []
        for base, off, _ in sel:
            blk = xn_v[pl.ds(base, 8), :].astype(F32)
            rows.append(jnp.sum(jnp.where(row8 == off, blk, 0.0), axis=0, keepdims=True))
        row16 = lax.broadcasted_iota(jnp.int32, (16, D), 0)
        xs = jnp.where(row16 == 0, rows[0], jnp.where(row16 == 1, rows[1], 0.0)).astype(BF16)
        wg_copy.wait()
        wu_copy.wait()
        wd_copy.wait()
        gp = _rb(jnp.dot(xs, pltpu.bitcast(wg_v[...], BF16), preferred_element_type=F32))
        up = _rb(jnp.dot(xs, pltpu.bitcast(wu_v[...], BF16), preferred_element_type=F32))
        g = _rb(gp * (1.0 / (1.0 + jnp.exp(-gp))))
        hm = (g * up).astype(BF16)
        y = _rb(jnp.dot(hm, pltpu.bitcast(wd_v[...], BF16), preferred_element_type=F32))
        for n, ((base, off, i), mv) in enumerate(zip(sel, (m1, m2))):
            gate = _rb(1.0 / (1.0 + jnp.exp(-mv)))
            upd = _rb(y[n:n + 1, :] * gate)
            done = i < S - PRE
            hit = row8 == off
            x_v[pl.ds(base, 8), :] = (x_v[pl.ds(base, 8), :].astype(F32)
                                      + jnp.where(hit & done, upd, 0.0)).astype(BF16)
            xn_v[pl.ds(base, 8), :] = (xn_v[pl.ds(base, 8), :].astype(F32)
                                       + jnp.where(hit & jnp.logical_not(done), upd, 0.0)).astype(BF16)

    def out_copy(r0, n, k):
        return pltpu.make_async_copy(x_v.at[pl.ds(r0, n)], out_hbm.at[pl.ds(r0, n)], sem_o.at[k])

    out_copy(0, S - PRE, 0).start()

    def epi(b, carry):
        ar = pl.ds(pl.multiple_of(NO * 32 + b * 128, 32), 128)
        a = jnp.concatenate([oc[ar, :] for oc in o_vs], axis=1)
        acc = jnp.dot(a, pltpu.bitcast(wo_v[...], BF16), preferred_element_type=F32)
        r0 = pl.multiple_of(S - PRE + b * 128, 128)
        x_v[pl.ds(r0, 128), :] = (x_v[pl.ds(r0, 128), :].astype(F32)
                                  + xn_v[pl.ds(r0, 128), :].astype(F32) + acc).astype(BF16)
        out_copy(r0, 128, 1 + b).start()
        return carry

    with scope('epi'):
        lax.fori_loop(0, PRE // 128, epi, 0)
    with scope('fin'):
        out_copy(0, S - PRE, 0).wait()
        for b in range(PRE // 128):
            out_copy(S - PRE + b * 128, 128, 1 + b).wait()


@jax.jit
def pallas_parallel_sum__memory_aug_recurrent_mem_tr__moe_arch_mod__prompt_kernel(
    A_x: jax.Array,
    A_mem0: jax.Array,
    A_Wq: jax.Array,
    A_Wk: jax.Array,
    A_Wv: jax.Array,
    A_Wo: jax.Array,
    A_seg_len: jax.Array,
    B_x: jax.Array,
    B_w_r: jax.Array,
    B_w_gate: jax.Array,
    B_w_up: jax.Array,
    B_w_down: jax.Array,
):
    del A_seg_len, B_x
    assert A_x.shape == (1, S, D) and A_Wq.shape == (D, H, E) and A_mem0.shape == (1, M, D)
    wshape = (D // 2, 2, NP, 2, E)
    any_spec = pl.BlockSpec(memory_space=pl.ANY)
    out = pl.pallas_call(
        _kernel,
        out_shape=jax.ShapeDtypeStruct((S, D), BF16),
        in_specs=[any_spec] * 10,
        out_specs=any_spec,
        scratch_shapes=[
            pltpu.VMEM((S, D), BF16),
            pltpu.VMEM((S, D), BF16),
            pltpu.VMEM((PRE, D), BF16),
            pltpu.VMEM((S + 32, D), BF16),
            pltpu.VMEM((NS, 3, NP, L2, E), BF16),
            pltpu.VMEM((NCH + 1, D // 2, 2 * E), U32),
            pltpu.VMEM((H * E // 2, D), U32),
            pltpu.VMEM((NST + 1, 3, 2, D // 2, E), U32),
            pltpu.VMEM((D // 2, 2 * E), U32),
            pltpu.VMEM((D // 2, 2 * E), U32),
            pltpu.VMEM((D // 2, 2 * E), U32),
            pltpu.VMEM((D // 2, FF), U32),
            pltpu.VMEM((D // 2, FF), U32),
            pltpu.VMEM((FF // 2, D), U32),
            pltpu.VMEM((1, D), BF16),
            pltpu.VMEM((L2, L2), F32),
            pltpu.SemaphoreType.DMA((PRE // XA,)),
            pltpu.SemaphoreType.DMA,
            pltpu.SemaphoreType.DMA((3,)),
            pltpu.SemaphoreType.DMA((NST + 1, 3, 2)),
            pltpu.SemaphoreType.DMA,
            pltpu.SemaphoreType.DMA((3,)),
            pltpu.SemaphoreType.DMA((1 + PRE // 128,)),
            *[pltpu.VMEM(((NO + NE) * 32, KC), BF16)] * NOC,
        ],
        compiler_params=pltpu.CompilerParams(vmem_limit_bytes=120 * 1024 * 1024,
                                             disable_bounds_checks=bool(opt('nobc', 1)),
                                             shape_invariant_numerics=bool(opt('sin', 1))),
    )(
        A_x.reshape(S, D),
        A_mem0.reshape(M, D),
        A_Wq.reshape(wshape),
        A_Wk.reshape(wshape),
        A_Wv.reshape(wshape),
        A_Wo.reshape(H * E, D),
        B_w_r.reshape(1, D),
        B_w_gate,
        B_w_up,
        B_w_down,
    )
    return out.reshape(1, S, D)
```

```python
import functools
import os

import jax
import jax.numpy as jnp
from jax import lax
import jax.experimental.pallas as pl
import jax.experimental.pallas.tpu as pltpu

OPT = dict(kv.split('=') for kv in os.environ.get('KOPT', '').split(',') if kv)


def opt(k, d):
    return int(OPT.get(k, d))


class _NoScope:
    def __enter__(self):
        return self

    def __exit__(self, *a):
        return False


def scope(name):
    return jax.named_scope(name) if opt('scopes', 0) else _NoScope()


F32 = jnp.float32
BF16 = jnp.bfloat16
U32 = jnp.uint32

S = 2048
D = 1024
H = 32
E = 128
M = 8
SEG = 32
NSEG = S // SEG
FF = 3584
NP = H // 2
L2 = 2 * (M + SEG)

PRE = 512
TPS = 24
NS = 17
NO = 17
NE = PRE // SEG
NST = 2
NCH = 3 * NP
NOC = opt('noc', 8)
KC = H * E // NOC
PPC = NP // NOC
XA = 128
XBR = (S - PRE) // NP
WOP = (H * E // 2) // NP

EPS = 1e-05
SCALE = float(E) ** -0.5


def _rb(v):
    return v.astype(BF16).astype(F32)


def _layernorm_rows(xb, wr):
    xf = xb.astype(F32)
    mean = jnp.sum(xf, axis=-1, keepdims=True) * (1.0 / D)
    xc = xf - mean
    var = jnp.sum(xc * xc, axis=-1, keepdims=True) * (1.0 / D)
    den = _rb(jnp.sqrt(_rb(_rb(var) + EPS)))
    d = _rb(xf - _rb(mean))
    xn = (d * (1.0 / den)).astype(BF16)
    r = _rb(jnp.sum(xn.astype(F32) * wr, axis=-1, keepdims=True))
    return xn, r


def _scatter_scores(acc, r, g0):
    lane = lax.broadcasted_iota(jnp.int32, acc.shape, 1)
    for j in range(r.shape[0] // 8):
        acc = jnp.where(lane == g0 + j, r[j * 8:(j + 1) * 8, :], acc)
    return acc


def _kernel(x_hbm, mem0_hbm, wq_hbm, wk_hbm, wv_hbm, wo_hbm, wr_hbm, wg_hbm, wu_hbm, wd_hbm,
            out_hbm,
            x_v, xn_v, xp_v, l_v, ring, wqkv, wo_v, stage, wc0, wc1, wc2, wg_v, wu_v, wd_v, wr_v, fill_v,
            sem_xa, sem_xb, sem_s, sem_st, sem_wo, sem_w, sem_o, *o_vs):
    w32 = [w.bitcast(U32) for w in (wq_hbm, wk_hbm, wv_hbm)]
    wo32 = wo_hbm.bitcast(U32)
    wcur = (wc0, wc1, wc2)

    def xa_copy(c):
        return pltpu.make_async_copy(x_hbm.at[pl.ds(c * XA, XA)], x_v.at[pl.ds(c * XA, XA)],
                                     sem_xa.at[c])

    xc_copy = pltpu.make_async_copy(x_hbm.at[pl.ds(PRE, TPS)], x_v.at[pl.ds(PRE, TPS)], sem_s.at[2])

    def xb_copy(i):
        r0 = pl.multiple_of(PRE + i * XBR, 32)
        return pltpu.make_async_copy(x_hbm.at[pl.ds(r0, XBR)], x_v.at[pl.ds(r0, XBR)], sem_xb)

    def st_copy(t, p, slot, k, dp):
        return pltpu.make_async_copy(w32[t].at[:, dp, p, 0, :], stage.at[slot, k, dp],
                                     sem_st.at[slot, k, dp])

    def grp_copies(g):
        slot = lax.rem(g, NST)
        cps = []
        for k, (t, p) in enumerate(((1, g), (2, g), (0, g + 1))):
            p = jnp.minimum(p, NP - 1)
            cps += [st_copy(t, p, slot, k, 0), st_copy(t, p, slot, k, 1)]
        return cps

    def wo_copy(i):
        r0 = pl.multiple_of(i * WOP, 8)
        return pltpu.make_async_copy(wo32.at[pl.ds(r0, WOP)], wo_v.at[pl.ds(r0, WOP)], sem_wo)

    mem0_copy = pltpu.make_async_copy(mem0_hbm, l_v.at[pl.ds(0, M)], sem_s.at[0])
    wr_copy = pltpu.make_async_copy(wr_hbm, wr_v, sem_s.at[1])
    first_copies = [st_copy(0, 0, NST, 0, 0), st_copy(0, 0, NST, 0, 1)]
    wg_copy = pltpu.make_async_copy(wg_hbm.bitcast(U32), wg_v, sem_w.at[0])
    wu_copy = pltpu.make_async_copy(wu_hbm.bitcast(U32), wu_v, sem_w.at[1])
    wd_copy = pltpu.make_async_copy(wd_hbm.bitcast(U32), wd_v, sem_w.at[2])

    xa_copy(0).start()
    wr_copy.start()
    for c in range(1, PRE // XA):
        xa_copy(c).start()
    xc_copy.start()
    for cp in first_copies:
        cp.start()
    for cp in grp_copies(0):
        cp.start()
    mem0_copy.start()

    row = lax.broadcasted_iota(jnp.int32, (L2, L2), 0)
    col = lax.broadcasted_iota(jnp.int32, (L2, L2), 1)
    rl = jnp.where(row >= L2 // 2, row - L2 // 2, row)
    cl = jnp.where(col >= L2 // 2, col - L2 // 2, col)
    same = (row >= L2 // 2) == (col >= L2 // 2)
    keep = (rl < M) | (rl >= cl)
    fill_v[...] = jnp.where(same, jnp.where(keep, 0.0, -1000000000.0), -jnp.inf).astype(F32)

    with scope('wait_wr'):
        wr_copy.wait()
        if opt('w0', 0):
            xa_copy(0).wait()
            xa_copy(0).start()

    def ln0(i, racc):
        xa_copy(i).wait()
        for j in range(XA // 32):
            r0 = pl.multiple_of(i * XA + j * 32, 32)
            xn, r = _layernorm_rows(x_v[pl.ds(r0, 32), :], wr_v[...].astype(F32))
            xn_v[pl.ds(r0, 32), :] = xn
            xp_v[pl.ds(r0, 32), :] = xn
            racc = _scatter_scores(racc, r, i * (XA // 8) + j * 4)
        return racc

    with scope('ln0'):
        racc = lax.fori_loop(0, PRE // XA, ln0, jnp.zeros((8, S // 8), F32))

    def ln_step(i, racc):
        ic = jnp.minimum(i, NSEG - 1)
        r0 = pl.multiple_of(PRE + ic * TPS, 8)
        xn, r = _layernorm_rows(x_v[pl.ds(r0, TPS), :], wr_v[...].astype(F32))
        xn_v[pl.ds(r0, TPS), :] = xn
        racc = _scatter_scores(racc, r, PRE // 8 + ic * (TPS // 8))
        if opt('tokval', 0):
            return racc, xn.astype(F32)
        l_v[pl.ds(pl.multiple_of(i * 32 + M, 8), TPS), :] = xn
        return racc, jnp.zeros((8, 128), F32)

    with scope('ln_s0'):
        xc_copy.wait()
        racc, tok0 = ln_step(0, racc)

    def relayout(slot, k, c, dst):
        for j in range(D // 2 // 64):
            a = stage[slot, k, 0, j * 64:(j + 1) * 64, :]
            b = stage[slot, k, 1, j * 64:(j + 1) * 64, :]
            ev = (a & jnp.uint32(0xFFFF)) | (b << 16)
            od = (a >> 16) | (b & jnp.uint32(0xFFFF0000))
            dst[j * 64:(j + 1) * 64, 0:E] = ev
            dst[j * 64:(j + 1) * 64, E:2 * E] = od
            wqkv[c, j * 64:(j + 1) * 64, 0:E] = ev
            wqkv[c, j * 64:(j + 1) * 64, E:2 * E] = od

    with scope('pre_pro'):
        for cp in first_copies:
            cp.wait()
        relayout(NST, 0, 0, wc0)

    MB = opt('promb', 128)

    def pro(p, carry):
        for cp in grp_copies(p):
            cp.wait()
        for cp in grp_copies(p + 1):
            cp.start()
        wo_copy(p).start()
        xb_copy(p).start()

        slot = lax.rem(p, NST)
        for t in range(3):
            relayout(slot, t, 3 * p + t + 1, wcur[(t + 1) % 3])
            for rb in range(PRE // MB):
                w = pltpu.bitcast(wcur[t][...], BF16)
                y = jnp.dot(xp_v[rb * MB:(rb + 1) * MB, :], w, preferred_element_type=F32)
                y = y.astype(BF16)
                for sg in range(MB // 32):
                    for hh in range(2):
                        ring[rb * (MB // 32) + sg, t, p, hh * 40 + M:hh * 40 + 40, :] = (
                            y[sg * 32:(sg + 1) * 32, hh * E:(hh + 1) * E])
        return carry

    xb_all = pltpu.make_async_copy(x_hbm.at[pl.ds(PRE, S - PRE)], x_v.at[pl.ds(PRE, S - PRE)], sem_xb)
    with scope('pro'):
        lax.fori_loop(0, NP, pro, 0)

    for cp in grp_copies(NP):
        cp.wait()
    xb_all.wait()
    wg_copy.start()
    wu_copy.start()
    wd_copy.start()
    mem0_copy.wait()
    pltpu.make_async_copy(wo32, wo_v, sem_wo).wait()

    def step(s, carry):
        racc, mem, tok = carry
        slot = lax.rem(s, NS)
        oslot = lax.rem(s, NO)
        top = l_v[pl.ds(pl.multiple_of(s * 32 + M, 8), 8), :].astype(F32)
        bot = l_v[pl.ds(pl.multiple_of(s * 32 + 16, 16), 16), :]

        def mk_lhs(m, lo, hi):
            return jnp.concatenate(
                [jnp.concatenate([m, top[:, lo:hi]], axis=0).astype(BF16), bot[:, lo:hi]], axis=0)

        ks = opt('ksplit', 4) * 128
        if ks:
            lhs_lo = mk_lhs(mem[:, :ks], 0, ks)
            part = [jnp.dot(lhs_lo, pltpu.bitcast(wqkv[t, 0:ks // 2, :], BF16),
                            preferred_element_type=F32) for t in range(3)]
            mem_hi = mem[:, ks:]
            if opt('dep', 0):
                dn = opt('depn', 0)
                dep = part[dn // 2][0:M, (dn % 2) * E:(dn % 2 + 1) * E]
                dep = jnp.concatenate([dep] * ((D - ks) // E), axis=1)
                mem_hi = jnp.where(dep != dep, dep, mem_hi)
            lhs = jnp.concatenate([lhs_lo, mk_lhs(mem_hi, ks, D)], axis=1)
        else:
            lhs = mk_lhs(mem, 0, D)
        qdst = []
        for j in range(3):
            t0 = PRE + s * TPS + 8 * j
            qdst.append((lax.rem(lax.div(t0, SEG), NS), M + lax.rem(t0, SEG)))
        odst = []
        for j in range(4):
            g = 4 * s + j
            r_ring = lax.rem(lax.div(g, 3), NO) * 32 + M + lax.rem(g, 3) * 8
            r_epi = (NO + s - (NSEG - NE)) * 32 + 8 * j
            odst.append(pl.multiple_of(jnp.where(s < NSEG - NE, r_ring, r_epi), 8))
        orow = pl.multiple_of(oslot * 32, 32)

        def qkv(p, ts=(0, 1, 2)):
            for t in ts:
                if p == 0 and ks:
                    y2 = jnp.dot(lhs[:, ks:], pltpu.bitcast(wqkv[t, ks // 2:, :], BF16),
                                 preferred_element_type=F32)
                    y = y2 + part[t] if opt('swp', 1) else part[t] + y2
                    y = y.astype(BF16)
                else:
                    w = pltpu.bitcast(wqkv[3 * p + t], BF16)
                    y = jnp.dot(lhs, w, preferred_element_type=F32).astype(BF16)
                for hh in range(2):
                    yc = y[:, hh * E:(hh + 1) * E]
                    ring[slot, t, p, hh * 40:hh * 40 + M, :] = yc[0:M]
                    for j in range(3):
                        qs, qr = qdst[j]
                        ring[qs, t, p, pl.ds(pl.multiple_of(hh * 40 + qr, 8), 8), :] = (
                            yc[M + 8 * j:M + 8 * j + 8])

        PRENORM = opt('prenorm', 1)
        LAGA = opt('laga', 1)
        LAGB = opt('lagb', 2)

        def attn_a(q, k):
            sc = lax.dot_general(q, k, (((1,), (1,)), ((), ())), preferred_element_type=F32)
            fill = fill_v[...]
            sc = jnp.where(fill == 0.0, sc * SCALE, fill)
            mx = jnp.max(sc, axis=-1, keepdims=True)
            e = jnp.exp(sc - mx)
            den = jnp.sum(e, axis=-1, keepdims=True)
            inv = pl.reciprocal(den, approx=True)
            if PRENORM:
                return (e * inv).astype(BF16), None
            return e.astype(BF16), inv

        def attn_b(p, e, inv, v):
            o = jnp.dot(e, v, preferred_element_type=F32)
            if inv is not None:
                o = o * inv
            o = o.astype(BF16)
            oc = o_vs[p // PPC]
            for hh in range(2):
                cs = (2 * (p % PPC) + hh) * E
                oc[pl.ds(orow, M), cs:cs + E] = o[hh * 40:hh * 40 + M]
                for j in range(4):
                    oc[pl.ds(odst[j], 8), cs:cs + E] = o[hh * 40 + M + 8 * j:hh * 40 + M + 8 * j + 8]

        def wo_chunk(c, c1):
            a = jnp.concatenate([o_vs[i][pl.ds(orow, 32), :] for i in range(c, c1)], axis=1)
            w = pltpu.bitcast(wo_v[c * KC // 2:c1 * KC // 2, :], BF16)
            return jnp.dot(a, w, preferred_element_type=F32)

        wl = OPT.get('wl', '0.1.2.3.4.5-7').split('.')
        nslot = 3 * NP + len(wl)
        ev = {n: [] for n in range(nslot + 1)}
        lq, aa, lv, bb = opt('lq', 2), opt('a', 4), opt('lv', 6), opt('b', 8)
        ta = [int(x) for x in OPT.get('ta', '50').split('.')]
        tb = [int(x) for x in OPT.get('tb', '51.52').split('.')]
        for p in range(NP):
            pa_ = 3 * p + aa if p < NP - len(ta) else ta[p - (NP - len(ta))]
            pb_ = 3 * p + bb if p < NP - len(tb) else tb[p - (NP - len(tb))]
            assert pa_ <= pb_ <= nslot
            ev[min(3 * p + lq, pa_)].append((0, 'Q', p))
            ev[min(3 * p + lv, pb_)].append((1, 'V', p))
            ev[pa_].append((3 if opt('bfirst', 1) else 2, 'A', p))
            ev[pb_].append((2 if opt('bfirst', 1) else 3, 'B', p))
        pe, qk, vv = {}, {}, {}
        acc = None
        for n in range(nslot + 1):
            for _, kind, p in sorted(ev[n]):
                if kind == 'Q':
                    qk[p] = (ring[slot, 0, p], ring[slot, 1, p])
                elif kind == 'V':
                    vv[p] = ring[slot, 2, p]
                elif kind == 'A':
                    pe[p] = attn_a(*qk.pop(p))
                else:
                    attn_b(p, *pe.pop(p), vv.pop(p))
            if n < 3 * NP:
                qkv(n // 3, (n % 3,))
            elif n < nslot:
                tk = wl[n - 3 * NP].split('-')
                y = wo_chunk(int(tk[0]), int(tk[-1]) + 1)
                acc = y if acc is None else (y + acc if opt('swpw', 1) else acc + y)
        assert not pe
        r0 = pl.multiple_of(s * TPS, 8)
        base = x_v[pl.ds(r0, TPS), :].astype(F32) + xn_v[pl.ds(r0, TPS), :].astype(F32)
        racc, tok = ln_step(s + 1, racc)
        x_v[pl.ds(r0, TPS), :] = (base + acc[M:]).astype(BF16)
        return racc, acc[0:M], tok

    with scope('main'):
        U = opt('unroll', 4)

        def steps(i, carry):
            for u in range(U):
                carry = step(i * U + u, carry)
            return carry

        racc, _, _ = lax.fori_loop(0, NSEG // U, steps, (racc, l_v[0:M, :].astype(F32), tok0))

    with scope('moe'):
        r = racc
        idx = (lax.broadcasted_iota(jnp.int32, r.shape, 1) * 8
               + lax.broadcasted_iota(jnp.int32, r.shape, 0)).astype(F32)

        def allred(fn, v):
            return fn(fn(v, axis=1, keepdims=True), axis=0, keepdims=True)

        m1 = allred(jnp.max, r)
        i1 = allred(jnp.min, jnp.where(r == m1, idx, float(S - 1)))
        r2 = jnp.where(idx == i1, -jnp.inf, r)
        m2 = allred(jnp.max, r2)
        i2 = allred(jnp.min, jnp.where((r2 == m2) & (idx != i1), idx, float(S - 1)))
        sel = []
        for iv in (i1, i2):
            i = jnp.clip(jnp.max(iv).astype(jnp.int32), 0, S - 1)
            sel.append((pl.multiple_of(lax.div(i, 8) * 8, 8), lax.rem(i, 8), i))
        row8 = lax.broadcasted_iota(jnp.int32, (8, D), 0)
        rows = []
        for base, off, _ in sel:
            blk = xn_v[pl.ds(base, 8), :].astype(F32)
            rows.append(jnp.sum(jnp.where(row8 == off, blk, 0.0), axis=0, keepdims=True))
        row16 = lax.broadcasted_iota(jnp.int32, (16, D), 0)
        xs = jnp.where(row16 == 0, rows[0], jnp.where(row16 == 1, rows[1], 0.0)).astype(BF16)
        wg_copy.wait()
        wu_copy.wait()
        wd_copy.wait()
        gp = _rb(jnp.dot(xs, pltpu.bitcast(wg_v[...], BF16), preferred_element_type=F32))
        up = _rb(jnp.dot(xs, pltpu.bitcast(wu_v[...], BF16), preferred_element_type=F32))
        g = _rb(gp * (1.0 / (1.0 + jnp.exp(-gp))))
        hm = (g * up).astype(BF16)
        y = _rb(jnp.dot(hm, pltpu.bitcast(wd_v[...], BF16), preferred_element_type=F32))
        for n, ((base, off, i), mv) in enumerate(zip(sel, (m1, m2))):
            gate = _rb(1.0 / (1.0 + jnp.exp(-mv)))
            upd = _rb(y[n:n + 1, :] * gate)
            done = i < S - PRE
            hit = row8 == off
            x_v[pl.ds(base, 8), :] = (x_v[pl.ds(base, 8), :].astype(F32)
                                      + jnp.where(hit & done, upd, 0.0)).astype(BF16)
            xn_v[pl.ds(base, 8), :] = (xn_v[pl.ds(base, 8), :].astype(F32)
                                       + jnp.where(hit & jnp.logical_not(done), upd, 0.0)).astype(BF16)

    def out_copy(r0, n, k):
        return pltpu.make_async_copy(x_v.at[pl.ds(r0, n)], out_hbm.at[pl.ds(r0, n)], sem_o.at[k])

    out_copy(0, S - PRE, 0).start()

    def epi(b, carry):
        ar = pl.ds(pl.multiple_of(NO * 32 + b * 128, 32), 128)
        a = jnp.concatenate([oc[ar, :] for oc in o_vs], axis=1)
        acc = jnp.dot(a, pltpu.bitcast(wo_v[...], BF16), preferred_element_type=F32)
        r0 = pl.multiple_of(S - PRE + b * 128, 128)
        x_v[pl.ds(r0, 128), :] = (x_v[pl.ds(r0, 128), :].astype(F32)
                                  + xn_v[pl.ds(r0, 128), :].astype(F32) + acc).astype(BF16)
        out_copy(r0, 128, 1 + b).start()
        return carry

    with scope('epi'):
        lax.fori_loop(0, PRE // 128, epi, 0)
    with scope('fin'):
        out_copy(0, S - PRE, 0).wait()
        for b in range(PRE // 128):
            out_copy(S - PRE + b * 128, 128, 1 + b).wait()


@jax.jit
def pallas_parallel_sum__memory_aug_recurrent_mem_tr__moe_arch_mod__prompt_kernel(
    A_x: jax.Array,
    A_mem0: jax.Array,
    A_Wq: jax.Array,
    A_Wk: jax.Array,
    A_Wv: jax.Array,
    A_Wo: jax.Array,
    A_seg_len: jax.Array,
    B_x: jax.Array,
    B_w_r: jax.Array,
    B_w_gate: jax.Array,
    B_w_up: jax.Array,
    B_w_down: jax.Array,
):
    del A_seg_len, B_x
    assert A_x.shape == (1, S, D) and A_Wq.shape == (D, H, E) and A_mem0.shape == (1, M, D)
    wshape = (D // 2, 2, NP, 2, E)
    any_spec = pl.BlockSpec(memory_space=pl.ANY)
    out = pl.pallas_call(
        _kernel,
        out_shape=jax.ShapeDtypeStruct((S, D), BF16),
        in_specs=[any_spec] * 10,
        out_specs=any_spec,
        scratch_shapes=[
            pltpu.VMEM((S, D), BF16),
            pltpu.VMEM((S, D), BF16),
            pltpu.VMEM((PRE, D), BF16),
            pltpu.VMEM((S + 32, D), BF16),
            pltpu.VMEM((NS, 3, NP, L2, E), BF16),
            pltpu.VMEM((NCH + 1, D // 2, 2 * E), U32),
            pltpu.VMEM((H * E // 2, D), U32),
            pltpu.VMEM((NST + 1, 3, 2, D // 2, E), U32),
            pltpu.VMEM((D // 2, 2 * E), U32),
            pltpu.VMEM((D // 2, 2 * E), U32),
            pltpu.VMEM((D // 2, 2 * E), U32),
            pltpu.VMEM((D // 2, FF), U32),
            pltpu.VMEM((D // 2, FF), U32),
            pltpu.VMEM((FF // 2, D), U32),
            pltpu.VMEM((1, D), BF16),
            pltpu.VMEM((L2, L2), F32),
            pltpu.SemaphoreType.DMA((PRE // XA,)),
            pltpu.SemaphoreType.DMA,
            pltpu.SemaphoreType.DMA((3,)),
            pltpu.SemaphoreType.DMA((NST + 1, 3, 2)),
            pltpu.SemaphoreType.DMA,
            pltpu.SemaphoreType.DMA((3,)),
            pltpu.SemaphoreType.DMA((1 + PRE // 128,)),
            *[pltpu.VMEM(((NO + NE) * 32, KC), BF16)] * NOC,
        ],
        compiler_params=pltpu.CompilerParams(vmem_limit_bytes=120 * 1024 * 1024,
                                             disable_bounds_checks=bool(opt('nobc', 1)),
                                             shape_invariant_numerics=bool(opt('sin', 1))),
    )(
        A_x.reshape(S, D),
        A_mem0.reshape(M, D),
        A_Wq.reshape(wshape),
        A_Wk.reshape(wshape),
        A_Wv.reshape(wshape),
        A_Wo.reshape(H * E, D),
        B_w_r.reshape(1, D),
        B_w_gate,
        B_w_up,
        B_w_down,
    )
    return out.reshape(1, S, D)
```

```python
import functools
import os

import jax
import jax.numpy as jnp
from jax import lax
import jax.experimental.pallas as pl
import jax.experimental.pallas.tpu as pltpu

OPT = dict(kv.split('=') for kv in os.environ.get('KOPT', '').split(',') if kv)


def opt(k, d):
    return int(OPT.get(k, d))


class _NoScope:
    def __enter__(self):
        return self

    def __exit__(self, *a):
        return False


def scope(name):
    return jax.named_scope(name) if opt('scopes', 0) else _NoScope()


F32 = jnp.float32
BF16 = jnp.bfloat16
U32 = jnp.uint32

S = 2048
D = 1024
H = 32
E = 128
M = 8
SEG = 32
NSEG = S // SEG
FF = 3584
NP = H // 2
L1 = M + SEG
L2 = 2 * L1

PRE = 512
TPS = 24
NS = 17
U = 4
WG = (3, 3, 3, 5)
WGS = (0, 3, 6, 9)
GPI = sum(WG)
REC = (GPI + U) * 8
NREC = 4
EPI = S - (NSEG // U) * GPI * 8
OEPI = NREC * REC
NST = 2
NCH = 3 * NP
NOC = 8
KC = H * E // NOC
PPC = NP // NOC
XA = PRE // 2
XBR = (S - PRE) // NP
WOP = (H * E // 2) // NP
KS = D // 2

EPS = 1e-05
SCALE = float(E) ** -0.5


def _mod17(x):
    return x - 17 * ((x * 241) >> 12)


def _div14(x):
    return (x * 293) >> 12


assert NS == 17 and SEG == 32 and GPI == 14
assert all(_mod17(x) == x % 17 for x in range(128))
assert all(_div14(x) == x // 14 for x in range(256))
assert all(min((r * 11) >> 5, 3) == max(u for u in range(U) if WGS[u] <= r) for r in range(GPI))


def _rb(v):
    return v.astype(BF16).astype(F32)


def _layernorm_rows(xb, wr):
    xf = xb.astype(F32)
    mean = jnp.sum(xf, axis=-1, keepdims=True) * (1.0 / D)
    xc = xf - mean
    var = jnp.sum(xc * xc, axis=-1, keepdims=True) * (1.0 / D)
    den = _rb(jnp.sqrt(_rb(_rb(var) + EPS)))
    d = _rb(xf - _rb(mean))
    xn = (d * (1.0 / den)).astype(BF16)
    r = _rb(jnp.sum(xn.astype(F32) * wr, axis=-1, keepdims=True))
    return xn, r


def _scatter_scores(acc, r, g0):
    lane = lax.broadcasted_iota(jnp.int32, acc.shape, 1)
    for j in range(r.shape[0] // 8):
        acc = jnp.where(lane == g0 + j, r[j * 8:(j + 1) * 8, :], acc)
    return acc


def _dot(a, w32):
    return jnp.dot(a, pltpu.bitcast(w32, BF16), preferred_element_type=F32)


def _kernel(x_hbm, mem0_hbm, wq_hbm, wk_hbm, wv_hbm, wo_hbm, wr_hbm, wg_hbm, wu_hbm, wd_hbm,
            out_hbm,
            x_v, xn_v, xp_v, mem0_v, ring, wqkv, wo_v, stage, wc0, wc1, wc2, wg_v, wu_v, wd_v,
            wr_in, wr_v, fill_v, fix_v,
            sem_xa, sem_xb, sem_s, sem_st, sem_wo, sem_w, sem_o, *o_vs):
    w32 = [w.bitcast(U32) for w in (wq_hbm, wk_hbm, wv_hbm)]
    wo32 = wo_hbm.bitcast(U32)
    wcur = (wc0, wc1, wc2)

    def xa_copy(c):
        n = XA if c == 0 else PRE + TPS - XA
        return pltpu.make_async_copy(x_hbm.at[pl.ds(c * XA, n)], x_v.at[pl.ds(c * XA, n)],
                                     sem_xa.at[c])

    def xb_copy(i):
        r0 = pl.multiple_of(PRE + i * XBR, 32)
        return pltpu.make_async_copy(x_hbm.at[pl.ds(r0, XBR)], x_v.at[pl.ds(r0, XBR)], sem_xb)

    def st_copy(t, p, slot, k, dp):
        return pltpu.make_async_copy(w32[t].at[:, dp, p, 0, :], stage.at[slot, k, dp],
                                     sem_st.at[slot, k, dp])

    def grp_copies(g):
        slot = g & (NST - 1)
        cps = []
        for k, (t, p) in enumerate(((1, g), (2, g), (0, g + 1))):
            p = jnp.minimum(p, NP - 1)
            cps += [st_copy(t, p, slot, k, 0), st_copy(t, p, slot, k, 1)]
        return cps

    def wo_copy(i):
        r0 = pl.multiple_of(i * WOP, 8)
        return pltpu.make_async_copy(wo32.at[pl.ds(r0, WOP)], wo_v.at[pl.ds(r0, WOP)], sem_wo)

    mem0_copy = pltpu.make_async_copy(mem0_hbm, mem0_v, sem_s.at[0])
    wr_copy = pltpu.make_async_copy(wr_hbm, wr_in, sem_s.at[1])
    first_copies = [st_copy(0, 0, NST, 0, 0), st_copy(0, 0, NST, 0, 1)]
    moe_copies = [pltpu.make_async_copy(src.bitcast(U32), dst, sem_w.at[k])
                  for k, (src, dst) in enumerate(((wg_hbm, wg_v), (wu_hbm, wu_v), (wd_hbm, wd_v)))]

    cps0 = grp_copies(0)
    xa_copy(0).start()
    wr_copy.start()
    for cp in first_copies:
        cp.start()
    xa_copy(1).start()

    row = lax.broadcasted_iota(jnp.int32, (L2, L2), 0)
    col = lax.broadcasted_iota(jnp.int32, (L2, L2), 1)
    rl = jnp.where(row >= L1, row - L1, row)
    cl = jnp.where(col >= L1, col - L1, col)
    same = (row >= L1) == (col >= L1)
    keep = (rl < M) | (rl >= cl)
    fill_v[...] = jnp.where(same, jnp.where(keep, 0.0, -1000000000.0), -jnp.inf).astype(F32)

    def ln_rows(r0, n, racc):
        for j in range(n // 32):
            r = r0 + j * 32
            rs = pl.ds(r if isinstance(r, int) else pl.multiple_of(r, 32), 32)
            xn, sc = _layernorm_rows(x_v[rs, :], wr_v[0:1, :])
            xn_v[rs, :] = xn
            xp_v[rs, :] = xn
            racc = _scatter_scores(racc, sc, r // 8 if isinstance(r, int) else r >> 3)
        return racc

    def ln_step(i, racc):
        ic = jnp.minimum(i, NSEG - 1)
        r0 = pl.multiple_of(PRE + ic * TPS, 8)
        xn, r = _layernorm_rows(x_v[pl.ds(r0, TPS), :], wr_v[0:1, :])
        xn_v[pl.ds(r0, TPS), :] = xn
        return _scatter_scores(racc, r, PRE // 8 + ic * (TPS // 8))

    with scope('ln0'):
        wr_copy.wait()
        wrf = wr_in[...].astype(F32)
        wr_v[...] = jnp.broadcast_to(
            jnp.concatenate([wrf[k:k + 1, :] for k in range(D // E)], axis=1), (8, D))
        xa_copy(0).wait()
        for cp in cps0:
            cp.start()
        LB = opt('lnb', 64)
        racc = jnp.zeros((8, S // 8), F32)
        if LB == XA:
            racc = ln_rows(0, XA, racc)
        else:
            racc = lax.fori_loop(0, XA // LB, lambda i, ra: ln_rows(i * LB, LB, ra), racc)

    def relayout(slot, k, c, dst):
        for j in range(D // 2 // 64):
            a = stage[slot, k, 0, j * 64:(j + 1) * 64, :]
            b = stage[slot, k, 1, j * 64:(j + 1) * 64, :]
            ev = (a & jnp.uint32(0xFFFF)) | (b << 16)
            od = (a >> 16) | (b & jnp.uint32(0xFFFF0000))
            dst[j * 64:(j + 1) * 64, 0:E] = ev
            dst[j * 64:(j + 1) * 64, E:2 * E] = od
            wqkv[c, j * 64:(j + 1) * 64, 0:E] = ev
            wqkv[c, j * 64:(j + 1) * 64, E:2 * E] = od

    MB = opt('promb', 256)

    def pro_dots(t, p):
        for rb in range(PRE // MB):
            y = _dot(xp_v[rb * MB:(rb + 1) * MB, :], wcur[t][...]).astype(BF16)
            for sg in range(MB // SEG):
                for hh in range(2):
                    ring[rb * (MB // SEG) + sg, t, p, hh * L1 + M:(hh + 1) * L1, :] = (
                        y[sg * SEG:(sg + 1) * SEG, hh * E:(hh + 1) * E])

    with scope('blkB'):
        for cp in first_copies:
            cp.wait()
        xa_copy(1).wait()
        mem0_copy.start()
        for cp in grp_copies(1):
            cp.start()
        relayout(NST, 0, 0, wc0)
        racc = ln_rows(XA, PRE - XA, racc)
        pro_dots(0, 0)
        racc = ln_step(0, racc)
    with scope('blkC'):
        for cp in cps0[:4]:
            cp.wait()
        wo_copy(0).start()
        xb_copy(0).start()
        relayout(0, 0, 1, wc1)
        relayout(0, 1, 2, wc2)
        pro_dots(1, 0)
    with scope('blkD'):
        for cp in cps0[4:]:
            cp.wait()
        relayout(0, 2, 3, wc0)
        pro_dots(2, 0)

    def pro(p, carry):
        for cp in grp_copies(p):
            cp.wait()
        for cp in grp_copies(p + 1):
            cp.start()
        wo_copy(p).start()
        xb_copy(p).start()
        slot = p & (NST - 1)
        for t in range(3):
            relayout(slot, t, 3 * p + t + 1, wcur[(t + 1) % 3])
            pro_dots(t, p)
        return carry

    with scope('pro'):
        lax.fori_loop(1, NP, pro, 0)

    for cp in grp_copies(NP):
        cp.wait()
    pltpu.make_async_copy(x_hbm.at[pl.ds(PRE, S - PRE)], x_v.at[pl.ds(PRE, S - PRE)], sem_xb).wait()
    mem0_copy.wait()
    pltpu.make_async_copy(wo32, wo_v, sem_wo).wait()

    def step(it, u, carry):
        racc, mem = carry
        s = it * U + u
        slot = _mod17(s)
        t0 = pl.multiple_of(PRE + s * TPS, 8)
        top = xn_v[pl.ds(t0, 8), :].astype(F32)
        bot = xn_v[pl.ds(t0 + 8, 16), :]
        lhs = jnp.concatenate([jnp.concatenate([mem, top], axis=0).astype(BF16), bot], axis=0)
        part = [_dot(lhs[:, :KS], wqkv[t, 0:KS // 2, :]) for t in range(3)]
        qdst = []
        for j in range(TPS // 8):
            tj = t0 + 8 * j
            qdst.append((_mod17(tj >> 5), M + (tj & (SEG - 1))))
        odst = []
        for j in range(SEG // 8):
            g = (SEG // 8) * s + j
            gi = _div14(g)
            gr = g - GPI * gi
            r_ring = (gi & (NREC - 1)) * REC + (gr + 1 + jnp.minimum((gr * 11) >> 5, 3)) * 8
            r_epi = OEPI + (g - (S - EPI) // 8) * 8
            odst.append(pl.multiple_of(jnp.where(g < (S - EPI) // 8, r_ring, r_epi), 8))
        orow = pl.multiple_of((it & (NREC - 1)) * REC + (WGS[u] + u) * 8, 16)
        nw = WG[u] * 8

        def qkv(p, t):
            if p == 0:
                y = _dot(lhs[:, KS:], wqkv[t, KS // 2:, :]) + part[t]
            else:
                y = _dot(lhs, wqkv[3 * p + t])
            y = y.astype(BF16)
            for hh in range(2):
                yc = y[:, hh * E:(hh + 1) * E]
                ring[slot, t, p, hh * L1:hh * L1 + M, :] = yc[0:M]
                for j in range(TPS // 8):
                    qs, qr = qdst[j]
                    ring[qs, t, p, pl.ds(pl.multiple_of(hh * L1 + qr, 8), 8), :] = (
                        yc[M + 8 * j:M + 8 * j + 8])

        def attn_a(q, k):
            sc = lax.dot_general(q, k, (((1,), (1,)), ((), ())), preferred_element_type=F32)
            fill = fill_v[...]
            sc = jnp.where(fill == 0.0, sc * SCALE, fill)
            e = jnp.exp(sc - jnp.max(sc, axis=-1, keepdims=True))
            den = jnp.sum(e, axis=-1, keepdims=True)
            return (e * pl.reciprocal(den, approx=True)).astype(BF16)

        def attn_b(p, pr, v):
            o = jnp.dot(pr, v, preferred_element_type=F32).astype(BF16)
            oc = o_vs[p // PPC]
            for hh in range(2):
                cs = (2 * (p % PPC) + hh) * E
                oc[pl.ds(orow, M), cs:cs + E] = o[hh * L1:hh * L1 + M]
                for j in range(SEG // 8):
                    r = hh * L1 + M + 8 * j
                    oc[pl.ds(odst[j], 8), cs:cs + E] = o[r:r + 8]

        def wo_chunk(c, c1):
            a = jnp.concatenate([o_vs[i][pl.ds(orow, M + nw), :] for i in range(c, c1)], axis=1)
            return _dot(a, wo_v[c * KC // 2:c1 * KC // 2, :])

        wl = OPT.get('wl', '0.1.2.3.4.5-7').split('.')
        nslot = 3 * NP + len(wl)
        ev = {n: [] for n in range(nslot + 1)}
        lq, aa, lv, bb = opt('lq', 2), opt('a', 4), opt('lv', 6), opt('b', 8)
        ta = [int(x) for x in OPT.get('ta', '50').split('.')]
        tb = [int(x) for x in OPT.get('tb', '51.52').split('.')]
        for p in range(NP):
            pa_ = 3 * p + aa if p < NP - len(ta) else ta[p - (NP - len(ta))]
            pb_ = 3 * p + bb if p < NP - len(tb) else tb[p - (NP - len(tb))]
            assert pa_ <= pb_ <= nslot
            ev[min(3 * p + lq, pa_)].append((0, 'Q', p))
            ev[min(3 * p + lv, pb_)].append((1, 'V', p))
            ev[pa_].append((3, 'A', p))
            ev[pb_].append((2, 'B', p))
        pe, qk, vv = {}, {}, {}
        acc = None
        for n in range(nslot + 1):
            for _, kind, p in sorted(ev[n]):
                if kind == 'Q':
                    qk[p] = (ring[slot, 0, p], ring[slot, 1, p])
                elif kind == 'V':
                    vv[p] = ring[slot, 2, p]
                elif kind == 'A':
                    pe[p] = attn_a(*qk.pop(p))
                else:
                    attn_b(p, pe.pop(p), vv.pop(p))
            if n < 3 * NP:
                qkv(n // 3, n % 3)
            elif n < nslot:
                tk = wl[n - 3 * NP].split('-')
                y = wo_chunk(int(tk[0]), int(tk[-1]) + 1)
                acc = y if acc is None else y + acc
        r0 = pl.multiple_of((it * GPI + WGS[u]) * 8, 8)
        base = x_v[pl.ds(r0, nw), :].astype(F32) + xn_v[pl.ds(r0, nw), :].astype(F32)
        racc = ln_step(s + 1, racc)
        x_v[pl.ds(r0, nw), :] = (base + acc[M:]).astype(BF16)
        return racc, acc[0:M]

    def steps(it, carry):
        @pl.when(it == 1)
        def _():
            for cp in moe_copies:
                cp.start()

        with scope('it'):
            for u in range(U):
                carry = step(it, u, carry)
        return carry

    with scope('main'):
        racc, _ = lax.fori_loop(0, NSEG // U, steps, (racc, mem0_v[...].astype(F32)))

    def out_copy(r0, n, k):
        return pltpu.make_async_copy(x_v.at[pl.ds(r0, n)], out_hbm.at[pl.ds(r0, n)], sem_o.at[k])

    for cp in moe_copies:
        cp.wait()
    out_copy(0, S - EPI, 0).start()

    idx = (lax.broadcasted_iota(jnp.int32, racc.shape, 1) * 8
           + lax.broadcasted_iota(jnp.int32, racc.shape, 0)).astype(F32)

    def allred(fn, v):
        return fn(fn(v, axis=1, keepdims=True), axis=0, keepdims=True)

    m1 = allred(jnp.max, racc)
    i1 = allred(jnp.min, jnp.where(racc == m1, idx, float(S - 1)))
    r2 = jnp.where(idx == i1, -jnp.inf, racc)
    m2 = allred(jnp.max, r2)
    i2 = allred(jnp.min, jnp.where((r2 == m2) & (idx != i1), idx, float(S - 1)))
    sel = [jnp.clip(jnp.max(iv).astype(jnp.int32), 0, S - 1) for iv in (i1, i2)]
    grp = [pl.multiple_of((i >> 3) << 3, 8) for i in sel]
    row8 = lax.broadcasted_iota(jnp.int32, (8, D), 0)
    rows = [jnp.sum(jnp.where(row8 == (i & 7), xn_v[pl.ds(g, 8), :].astype(F32), 0.0),
                    axis=0, keepdims=True) for i, g in zip(sel, grp)]
    row16 = lax.broadcasted_iota(jnp.int32, (16, D), 0)
    xs = jnp.where(row16 == 0, rows[0], jnp.where(row16 == 1, rows[1], 0.0)).astype(BF16)

    hs, ys, gps = {}, {}, {}

    def moe_gate(j):
        gps[j] = _rb(_dot(xs, wg_v[:, j * E:(j + 1) * E]))

    def moe_up(j):
        up = _rb(_dot(xs, wu_v[:, j * E:(j + 1) * E]))
        gp = gps.pop(j)
        g = _rb(gp * (1.0 / (1.0 + jnp.exp(-gp))))
        hs[j] = (g * up).astype(BF16)

    def moe_down(kc, nq):
        hk = jnp.concatenate([hs[4 * kc + i] for i in range(4)], axis=1)
        d = _dot(hk, wd_v[kc * 256:(kc + 1) * 256, nq * 256:(nq + 1) * 256])
        ys[nq] = d + ys[nq] if nq in ys else d

    def moe_apply():
        y = _rb(jnp.concatenate([ys[nq] for nq in range(4)], axis=1))
        upd = [_rb(y[n:n + 1, :] * _rb(1.0 / (1.0 + jnp.exp(-mv)))) for n, mv in enumerate((m1, m2))]
        for n in range(2):
            blk = x_v[pl.ds(grp[n], 8), :].astype(F32)
            for k in range(2):
                blk = blk + jnp.where(row8 + grp[n] == sel[k], upd[k], 0.0)
            fix_v[n] = blk.astype(BF16)
        for n in range(2):
            g = pl.multiple_of(jnp.maximum(grp[n], S - MOE_LATE), 8)
            x_v[pl.ds(g, 8), :] = (x_v[pl.ds(g, 8), :].astype(F32)
                                   + jnp.where(row8 + g == sel[n], upd[n], 0.0)).astype(BF16)

    waves = []
    for j in range(FF // E):
        waves += [functools.partial(moe_gate, j), functools.partial(moe_up, j)]
    for kc in range(FF // 512):
        waves += [functools.partial(moe_down, kc, nq) for nq in range(4)]
    waves = [None] * opt('mlead', 10) + waves + [None] * opt('mgap', 1) + [moe_apply]
    NM = opt('nm', 6)
    MOE_LATE = EPI

    def finish(rs, cs, acc):
        x_v[rs, cs] = (x_v[rs, cs].astype(F32) + xn_v[rs, cs].astype(F32) + acc).astype(BF16)

    with scope('epi0'):
        for blk in range(EPI // 128):
            ar = OEPI + blk * 128
            r0 = S - EPI + blk * 128
            for n in range(NM):
                acc = None
                for kc in range(NOC):
                    d = _dot(o_vs[kc][ar:ar + 128, :],
                             wo_v[kc * KC // 2:(kc + 1) * KC // 2, n * E:(n + 1) * E])
                    acc = d if acc is None else d + acc
                    if kc == NOC - 1:
                        finish(slice(r0, r0 + 128), slice(n * E, (n + 1) * E), acc)
                    if waves:
                        wv = waves.pop(0)
                        if wv is not None:
                            wv()
        for wv in waves:
            if wv is not None:
                wv()

    fixes = [pltpu.make_async_copy(fix_v.at[n], out_hbm.at[pl.ds(grp[n], 8)], sem_o.at[3 + n])
             for n in range(2)]
    need = [sel[0] < S - EPI, jnp.logical_and(sel[1] < S - EPI, grp[1] != grp[0])]
    out_copy(0, S - EPI, 0).wait()
    for n in range(2):
        @pl.when(need[n])
        def _():
            fixes[n].start()

    def epi(blk, carry):
        ar = pl.ds(pl.multiple_of(OEPI + blk * 128, 16), 128)
        a = jnp.concatenate([oc[ar, :] for oc in o_vs], axis=1)
        r0 = pl.multiple_of(S - EPI + blk * 128, 128)
        finish(pl.ds(r0, 128), slice(NM * E, D), _dot(a, wo_v[:, NM * E:]))
        out_copy(r0, 128, 1 + blk).start()
        return carry

    with scope('epi'):
        lax.fori_loop(0, EPI // 128, epi, 0)

    with scope('fin'):
        for n in range(2):
            @pl.when(need[n])
            def _():
                fixes[n].wait()
        for blk in range(EPI // 128):
            out_copy(S - EPI + blk * 128, 128, 1 + blk).wait()


@jax.jit
def pallas_parallel_sum__memory_aug_recurrent_mem_tr__moe_arch_mod__prompt_kernel(
    A_x: jax.Array,
    A_mem0: jax.Array,
    A_Wq: jax.Array,
    A_Wk: jax.Array,
    A_Wv: jax.Array,
    A_Wo: jax.Array,
    A_seg_len: jax.Array,
    B_x: jax.Array,
    B_w_r: jax.Array,
    B_w_gate: jax.Array,
    B_w_up: jax.Array,
    B_w_down: jax.Array,
):
    del A_seg_len, B_x
    assert A_x.shape == (1, S, D) and A_Wq.shape == (D, H, E) and A_mem0.shape == (1, M, D)
    wshape = (D // 2, 2, NP, 2, E)
    any_spec = pl.BlockSpec(memory_space=pl.ANY)
    out = pl.pallas_call(
        _kernel,
        out_shape=jax.ShapeDtypeStruct((S, D), BF16),
        in_specs=[any_spec] * 10,
        out_specs=any_spec,
        scratch_shapes=[
            pltpu.VMEM((S, D), BF16),
            pltpu.VMEM((S, D), BF16),
            pltpu.VMEM((PRE, D), BF16),
            pltpu.VMEM((M, D), BF16),
            pltpu.VMEM((NS, 3, NP, L2, E), BF16),
            pltpu.VMEM((NCH + 1, D // 2, 2 * E), U32),
            pltpu.VMEM((H * E // 2, D), U32),
            pltpu.VMEM((NST + 1, 3, 2, D // 2, E), U32),
            pltpu.VMEM((D // 2, 2 * E), U32),
            pltpu.VMEM((D // 2, 2 * E), U32),
            pltpu.VMEM((D // 2, 2 * E), U32),
            pltpu.VMEM((D // 2, FF), U32),
            pltpu.VMEM((D // 2, FF), U32),
            pltpu.VMEM((FF // 2, D), U32),
            pltpu.VMEM((D // E, E), BF16),
            pltpu.VMEM((8, D), F32),
            pltpu.VMEM((L2, L2), F32),
            pltpu.VMEM((2, 8, D), BF16),
            pltpu.SemaphoreType.DMA((2,)),
            pltpu.SemaphoreType.DMA,
            pltpu.SemaphoreType.DMA((2,)),
            pltpu.SemaphoreType.DMA((NST + 1, 3, 2)),
            pltpu.SemaphoreType.DMA,
            pltpu.SemaphoreType.DMA((3,)),
            pltpu.SemaphoreType.DMA((5,)),
            *[pltpu.VMEM((OEPI + EPI, KC), BF16)] * NOC,
        ],
        compiler_params=pltpu.CompilerParams(vmem_limit_bytes=120 * 1024 * 1024,
                                             disable_bounds_checks=True),
    )(
        A_x.reshape(S, D),
        A_mem0.reshape(M, D),
        A_Wq.reshape(wshape),
        A_Wk.reshape(wshape),
        A_Wv.reshape(wshape),
        A_Wo.reshape(H * E, D),
        B_w_r.reshape(D // E, E),
        B_w_gate,
        B_w_up,
        B_w_down,
    )
    return out.reshape(1, S, D)
```

```python
import functools
import os

import jax
import jax.numpy as jnp
from jax import lax
import jax.experimental.pallas as pl
import jax.experimental.pallas.tpu as pltpu

OPT = dict(kv.split('=') for kv in os.environ.get('KOPT', '').split(',') if kv)


def opt(k, d):
    return int(OPT.get(k, d))


class _NoScope:
    def __enter__(self):
        return self

    def __exit__(self, *a):
        return False


def scope(name):
    return jax.named_scope(name) if opt('scopes', 0) else _NoScope()


F32 = jnp.float32
BF16 = jnp.bfloat16
U32 = jnp.uint32

S = 2048
D = 1024
H = 32
E = 128
M = 8
SEG = 32
NSEG = S // SEG
FF = 3584
NP = H // 2
L1 = M + SEG
L2 = 2 * L1

PRE = 512
TPS = 24
NS = 17
U = 4
WG = (3, 3, 3, 5)
WGS = (0, 3, 6, 9)
GPI = sum(WG)
REC = (GPI + U) * 8
NREC = 4
EPI = S - (NSEG // U) * GPI * 8
OEPI = NREC * REC
NST = 2
NCH = 3 * NP
NOC = 8
KC = H * E // NOC
PPC = NP // NOC
XA = PRE // 2
XBR = (S - PRE) // NP
WOP = (H * E // 2) // NP
KS = D // 2

EPS = 1e-05
SCALE = float(E) ** -0.5


def _mod17(x):
    return x - 17 * ((x * 241) >> 12)


def _div14(x):
    return (x * 293) >> 12


assert NS == 17 and SEG == 32 and GPI == 14
assert all(_mod17(x) == x % 17 for x in range(128))
assert all(_div14(x) == x // 14 for x in range(256))
assert all(min((r * 11) >> 5, 3) == max(u for u in range(U) if WGS[u] <= r) for r in range(GPI))


def _rb(v):
    return v.astype(BF16).astype(F32)


def _recip(v):
    y = pl.reciprocal(v, approx=True)
    return y * (2.0 - v * y)


def _layernorm_rows(xb, wr8):
    xf = xb.astype(F32)
    mean = jnp.sum(xf, axis=-1, keepdims=True) * (1.0 / D)
    mb = _rb(mean)
    d = xf - mb
    dm = mean - mb
    var = jnp.maximum(jnp.sum(d * d, axis=-1, keepdims=True) * (1.0 / D) - dm * dm, 0.0)
    ve = _rb(_rb(var) + EPS)
    if opt('lnq', 1):
        inv = _recip(_rb(ve * lax.rsqrt(ve)))
    else:
        inv = 1.0 / _rb(jnp.sqrt(ve))
    xw = d * inv
    wr = jnp.concatenate([wr8] * (xb.shape[0] // 8), axis=0)
    r = _rb(jnp.sum(xw * wr, axis=-1, keepdims=True))
    return xw, r


def _scatter_scores(acc, r, g0):
    lane = lax.broadcasted_iota(jnp.int32, acc.shape, 1)
    for j in range(r.shape[0] // 8):
        acc = jnp.where(lane == g0 + j, r[j * 8:(j + 1) * 8, :], acc)
    return acc


def _dot(a, w32):
    return jnp.dot(a, pltpu.bitcast(w32, BF16), preferred_element_type=F32)


def _kernel(x_hbm, mem0_hbm, wq_hbm, wk_hbm, wv_hbm, wo_hbm, wr_hbm, wg_hbm, wu_hbm, wd_hbm,
            out_hbm,
            x_v, xn_v, xp_v, mem0_v, ring, wqkv, wo_v, stage, wc0, wc1, wc2, wg_v, wu_v, wd_v,
            wr_in, wr_v, fill_v, fix_v,
            sem_xa, sem_xb, sem_s, sem_st, sem_wo, sem_w, sem_o, *o_vs):
    w32 = [w.bitcast(U32) for w in (wq_hbm, wk_hbm, wv_hbm)]
    wo32 = wo_hbm.bitcast(U32)
    wcur = (wc0, wc1, wc2)

    def xa_copy(c):
        n = XA if c == 0 else PRE + TPS - XA
        return pltpu.make_async_copy(x_hbm.at[pl.ds(c * XA, n)], x_v.at[pl.ds(c * XA, n)],
                                     sem_xa.at[c])

    def xb_copy(i):
        r0 = pl.multiple_of(PRE + i * XBR, 32)
        return pltpu.make_async_copy(x_hbm.at[pl.ds(r0, XBR)], x_v.at[pl.ds(r0, XBR)], sem_xb)

    def st_copy(t, p, slot, k, dp):
        return pltpu.make_async_copy(w32[t].at[:, dp, p, 0, :], stage.at[slot, k, dp],
                                     sem_st.at[slot, k, dp])

    def grp_copies(g):
        slot = g & (NST - 1)
        cps = []
        for k, (t, p) in enumerate(((1, g), (2, g), (0, g + 1))):
            p = jnp.minimum(p, NP - 1)
            cps += [st_copy(t, p, slot, k, 0), st_copy(t, p, slot, k, 1)]
        return cps

    def wo_copy(i):
        r0 = pl.multiple_of(i * WOP, 8)
        return pltpu.make_async_copy(wo32.at[pl.ds(r0, WOP)], wo_v.at[pl.ds(r0, WOP)], sem_wo)

    mem0_copy = pltpu.make_async_copy(mem0_hbm, mem0_v, sem_s.at[0])
    wr_copy = pltpu.make_async_copy(wr_hbm, wr_in, sem_s.at[1])
    first_copies = [st_copy(0, 0, NST, 0, 0), st_copy(0, 0, NST, 0, 1)]
    moe_copies = [pltpu.make_async_copy(src.bitcast(U32), dst, sem_w.at[k])
                  for k, (src, dst) in enumerate(((wg_hbm, wg_v), (wu_hbm, wu_v), (wd_hbm, wd_v)))]

    cps0 = grp_copies(0)
    xa_copy(0).start()
    wr_copy.start()
    for cp in first_copies:
        cp.start()
    xa_copy(1).start()

    row = lax.broadcasted_iota(jnp.int32, (L2, L2), 0)
    col = lax.broadcasted_iota(jnp.int32, (L2, L2), 1)
    rl = jnp.where(row >= L1, row - L1, row)
    cl = jnp.where(col >= L1, col - L1, col)
    same = (row >= L1) == (col >= L1)
    keep = (rl < M) | (rl >= cl)
    fill_v[...] = jnp.where(same, jnp.where(keep, 0.0, -1000000000.0), -jnp.inf).astype(F32)

    def ln_rows(r0, n, racc):
        LR = opt('lnr', 32)
        for j in range(n // LR):
            r = r0 + j * LR
            rs = pl.ds(r if isinstance(r, int) else pl.multiple_of(r, LR), LR)
            xw, sc = _layernorm_rows(x_v[rs, :], wr_v[...])
            r2 = r // 2 if isinstance(r, int) else pl.multiple_of(r >> 1, LR // 2)
            xn_v[rs, :] = xw.astype(BF16)
            xp_v[pl.ds(r2, LR // 2), :] = pltpu.bitcast(xn_v[rs, :], U32)
            racc = _scatter_scores(racc, sc, r // 8 if isinstance(r, int) else r >> 3)
        return racc

    def ln_step(i, racc):
        ic = jnp.minimum(i, NSEG - 1)
        r0 = pl.multiple_of(PRE + ic * TPS, 8)
        xw, r = _layernorm_rows(x_v[pl.ds(r0, TPS), :], wr_v[...])
        xn_v[pl.ds(r0, TPS), :] = xw.astype(BF16)
        return _scatter_scores(racc, r, PRE // 8 + ic * (TPS // 8))

    with scope('ln0'):
        wr_copy.wait()
        wrf = wr_in[...].astype(F32)
        wr_v[...] = jnp.broadcast_to(
            jnp.concatenate([wrf[k:k + 1, :] for k in range(D // E)], axis=1), (8, D))
        xa_copy(0).wait()
        for cp in cps0:
            cp.start()
        LB = opt('lnb', 256)
        racc = jnp.zeros((8, S // 8), F32)
        if LB == XA:
            racc = ln_rows(0, XA, racc)
        else:
            racc = lax.fori_loop(0, XA // LB, lambda i, ra: ln_rows(i * LB, LB, ra), racc)

    def relayout(slot, k, c, dst):
        for j in range(D // 2 // 64):
            a = stage[slot, k, 0, j * 64:(j + 1) * 64, :]
            b = stage[slot, k, 1, j * 64:(j + 1) * 64, :]
            ev = (a & jnp.uint32(0xFFFF)) | (b << 16)
            od = (a >> 16) | (b & jnp.uint32(0xFFFF0000))
            dst[j * 64:(j + 1) * 64, 0:E] = ev
            dst[j * 64:(j + 1) * 64, E:2 * E] = od
            wqkv[c, j * 64:(j + 1) * 64, 0:E] = ev
            wqkv[c, j * 64:(j + 1) * 64, E:2 * E] = od

    MB = opt('promb', 256)

    def pro_dots(t, p):
        for rb in range(PRE // MB):
            if opt('xpn', 1):
                a = pltpu.bitcast(xp_v[rb * MB // 2:(rb + 1) * MB // 2, :], BF16)
            else:
                a = xp_v[rb * MB:(rb + 1) * MB, :]
            y = _dot(a, wcur[t][...]).astype(BF16)
            for sg in range(MB // SEG):
                for hh in range(2):
                    ring[rb * (MB // SEG) + sg, t, p, hh * L1 + M:(hh + 1) * L1, :] = (
                        y[sg * SEG:(sg + 1) * SEG, hh * E:(hh + 1) * E])

    with scope('blkB'):
        for cp in first_copies:
            cp.wait()
        xa_copy(1).wait()
        mem0_copy.start()
        for cp in grp_copies(1):
            cp.start()
        relayout(NST, 0, 0, wc0)
        racc = ln_rows(XA, PRE - XA, racc)
        pro_dots(0, 0)
        racc = ln_step(0, racc)
    with scope('blkC'):
        for cp in cps0[:4]:
            cp.wait()
        wo_copy(0).start()
        xb_copy(0).start()
        relayout(0, 0, 1, wc1)
        relayout(0, 1, 2, wc2)
        pro_dots(1, 0)
    with scope('blkD'):
        for cp in cps0[4:]:
            cp.wait()
        relayout(0, 2, 3, wc0)
        pro_dots(2, 0)

    def pro(p, carry):
        for cp in grp_copies(p):
            cp.wait()
        for cp in grp_copies(p + 1):
            cp.start()
        wo_copy(p).start()
        xb_copy(p).start()
        slot = p & (NST - 1)
        for t in range(3):
            relayout(slot, t, 3 * p + t + 1, wcur[(t + 1) % 3])
            pro_dots(t, p)
        return carry

    with scope('pro'):
        lax.fori_loop(1, NP, pro, 0)

    for cp in grp_copies(NP):
        cp.wait()
    pltpu.make_async_copy(x_hbm.at[pl.ds(PRE, S - PRE)], x_v.at[pl.ds(PRE, S - PRE)], sem_xb).wait()
    mem0_copy.wait()
    pltpu.make_async_copy(wo32, wo_v, sem_wo).wait()

    def step(it, u, carry):
        racc, mem = carry
        s = it * U + u
        slot = _mod17(s)
        t0 = pl.multiple_of(PRE + s * TPS, 8)
        top = xn_v[pl.ds(t0, 8), :].astype(F32)
        bot = xn_v[pl.ds(t0 + 8, 16), :]
        lhs = jnp.concatenate([jnp.concatenate([mem, top], axis=0).astype(BF16), bot], axis=0)
        part = [_dot(lhs[:, :KS], wqkv[t, 0:KS // 2, :]) for t in range(3)]
        qdst = []
        for j in range(TPS // 8):
            tj = t0 + 8 * j
            qdst.append((_mod17(tj >> 5), M + (tj & (SEG - 1))))
        odst = []
        for j in range(SEG // 8):
            g = (SEG // 8) * s + j
            gi = _div14(g)
            gr = g - GPI * gi
            r_ring = (gi & (NREC - 1)) * REC + (gr + 1 + jnp.minimum((gr * 11) >> 5, 3)) * 8
            r_epi = OEPI + (g - (S - EPI) // 8) * 8
            odst.append(pl.multiple_of(jnp.where(g < (S - EPI) // 8, r_ring, r_epi), 8))
        orow = pl.multiple_of((it & (NREC - 1)) * REC + (WGS[u] + u) * 8, 16)
        nw = WG[u] * 8

        def qkv(p, t):
            if p == 0:
                y = _dot(lhs[:, KS:], wqkv[t, KS // 2:, :]) + part[t]
            else:
                y = _dot(lhs, wqkv[3 * p + t])
            y = y.astype(BF16)
            for hh in range(2):
                yc = y[:, hh * E:(hh + 1) * E]
                ring[slot, t, p, hh * L1:hh * L1 + M, :] = yc[0:M]
                for j in range(TPS // 8):
                    qs, qr = qdst[j]
                    ring[qs, t, p, pl.ds(pl.multiple_of(hh * L1 + qr, 8), 8), :] = (
                        yc[M + 8 * j:M + 8 * j + 8])

        def attn_a(q, k):
            sc = lax.dot_general(q, k, (((1,), (1,)), ((), ())), preferred_element_type=F32)
            fill = fill_v[...]
            sc = jnp.where(fill == 0.0, sc * SCALE, fill)
            e = jnp.exp(sc - jnp.max(sc, axis=-1, keepdims=True))
            den = jnp.sum(e, axis=-1, keepdims=True)
            return (e * pl.reciprocal(den, approx=True)).astype(BF16)

        def attn_b(p, pr, v):
            o = jnp.dot(pr, v, preferred_element_type=F32).astype(BF16)
            oc = o_vs[p // PPC]
            for hh in range(2):
                cs = (2 * (p % PPC) + hh) * E
                oc[pl.ds(orow, M), cs:cs + E] = o[hh * L1:hh * L1 + M]
                for j in range(SEG // 8):
                    r = hh * L1 + M + 8 * j
                    oc[pl.ds(odst[j], 8), cs:cs + E] = o[r:r + 8]

        def wo_chunk(c, c1):
            a = jnp.concatenate([o_vs[i][pl.ds(orow, M + nw), :] for i in range(c, c1)], axis=1)
            return _dot(a, wo_v[c * KC // 2:c1 * KC // 2, :])

        wl = OPT.get('wl', '0.1.2.3.4.5.6-7').split('.')
        nslot = 3 * NP + len(wl)
        ev = {n: [] for n in range(nslot + 1)}
        lq, aa, lv, bb = opt('lq', 3), opt('a', 5), opt('lv', 7), opt('b', 9)
        ta = [int(x) for x in OPT.get('ta', '50').split('.')]
        tb = [int(x) for x in OPT.get('tb', '49.51.53').split('.')]
        for p in range(NP):
            pa_ = 3 * p + aa if p < NP - len(ta) else ta[p - (NP - len(ta))]
            pb_ = 3 * p + bb if p < NP - len(tb) else tb[p - (NP - len(tb))]
            assert pa_ <= pb_ <= nslot
            ev[min(3 * p + lq, pa_)].append((0, 'Q', p))
            ev[min(3 * p + lv, pb_)].append((1, 'V', p))
            ev[pa_].append((3, 'A', p))
            ev[pb_].append((2, 'B', p))
        pe, qk, vv = {}, {}, {}
        acc = None
        r0 = pl.multiple_of((it * GPI + WGS[u]) * 8, 8)
        for n in range(nslot + 1):
            for _, kind, p in sorted(ev[n]):
                if kind == 'Q':
                    qk[p] = (ring[slot, 0, p], ring[slot, 1, p])
                elif kind == 'V':
                    vv[p] = ring[slot, 2, p]
                elif kind == 'A':
                    pe[p] = attn_a(*qk.pop(p))
                else:
                    attn_b(p, pe.pop(p), vv.pop(p))
            if n == opt('lnpos', 99):
                base = x_v[pl.ds(r0, nw), :].astype(F32) + xn_v[pl.ds(r0, nw), :].astype(F32)
                racc = ln_step(s + 1, racc)
            if n < 3 * NP:
                qkv(n // 3, [int(c) for c in OPT.get('mo', '012')][n % 3])
            elif n < nslot:
                tk = wl[n - 3 * NP].split('-')
                y = wo_chunk(int(tk[0]), int(tk[-1]) + 1)
                acc = y if acc is None else y + acc
        if opt('lnpos', 99) > nslot:
            base = x_v[pl.ds(r0, nw), :].astype(F32) + xn_v[pl.ds(r0, nw), :].astype(F32)
        if opt('lnpos', 99) > nslot:
            racc = ln_step(s + 1, racc)
        x_v[pl.ds(r0, nw), :] = (base + acc[M:]).astype(BF16)
        return racc, acc[0:M]

    def steps(it, carry):
        def start_moe(_, c):
            for cp in moe_copies:
                cp.start()
            return c

        lax.fori_loop(0, (it == 1).astype(jnp.int32), start_moe, 0)

        with scope('it'):
            for u in range(U):
                carry = step(it, u, carry)
        return carry

    with scope('main'):
        racc, _ = lax.fori_loop(0, NSEG // U, steps, (racc, mem0_v[...].astype(F32)))

    def out_copy(r0, n, k):
        return pltpu.make_async_copy(x_v.at[pl.ds(r0, n)], out_hbm.at[pl.ds(r0, n)], sem_o.at[k])

    for cp in moe_copies:
        cp.wait()
    out_copy(0, S - EPI, 0).start()

    idx = (lax.broadcasted_iota(jnp.int32, racc.shape, 1) * 8
           + lax.broadcasted_iota(jnp.int32, racc.shape, 0)).astype(F32)

    def allred(fn, v):
        return fn(fn(v, axis=1, keepdims=True), axis=0, keepdims=True)

    m1 = allred(jnp.max, racc)
    i1 = allred(jnp.min, jnp.where(racc == m1, idx, float(S - 1)))
    r2 = jnp.where(idx == i1, -jnp.inf, racc)
    m2 = allred(jnp.max, r2)
    i2 = allred(jnp.min, jnp.where((r2 == m2) & (idx != i1), idx, float(S - 1)))
    sel = [jnp.clip(jnp.max(iv).astype(jnp.int32), 0, S - 1) for iv in (i1, i2)]
    grp = [pl.multiple_of((i >> 3) << 3, 8) for i in sel]
    row8 = lax.broadcasted_iota(jnp.int32, (8, D), 0)
    rows = [jnp.sum(jnp.where(row8 == (i & 7), xn_v[pl.ds(g, 8), :].astype(F32), 0.0),
                    axis=0, keepdims=True) for i, g in zip(sel, grp)]
    row16 = lax.broadcasted_iota(jnp.int32, (16, D), 0)
    xs = jnp.where(row16 == 0, rows[0], jnp.where(row16 == 1, rows[1], 0.0)).astype(BF16)

    hs, ys, gps = {}, {}, {}

    def moe_gate(j):
        gps[j] = _rb(_dot(xs, wg_v[:, j * E:(j + 1) * E]))

    def moe_up(j):
        up = _rb(_dot(xs, wu_v[:, j * E:(j + 1) * E]))
        gp = gps.pop(j)
        g = _rb(gp * (1.0 / (1.0 + jnp.exp(-gp))))
        hs[j] = (g * up).astype(BF16)

    def moe_down(kc, nq):
        hk = jnp.concatenate([hs[4 * kc + i] for i in range(4)], axis=1)
        d = _dot(hk, wd_v[kc * 256:(kc + 1) * 256, nq * 256:(nq + 1) * 256])
        ys[nq] = d + ys[nq] if nq in ys else d

    def moe_apply():
        y = _rb(jnp.concatenate([ys[nq] for nq in range(4)], axis=1))
        upd = [_rb(y[n:n + 1, :] * _rb(1.0 / (1.0 + jnp.exp(-mv)))) for n, mv in enumerate((m1, m2))]
        for n in range(2):
            blk = x_v[pl.ds(grp[n], 8), :].astype(F32)
            for k in range(2):
                blk = blk + jnp.where(row8 + grp[n] == sel[k], upd[k], 0.0)
            fix_v[n] = blk.astype(BF16)
        for n in range(2):
            g = pl.multiple_of(jnp.maximum(grp[n], S - MOE_LATE), 8)
            x_v[pl.ds(g, 8), :] = (x_v[pl.ds(g, 8), :].astype(F32)
                                   + jnp.where(row8 + g == sel[n], upd[n], 0.0)).astype(BF16)

    waves = []
    for j in range(FF // E):
        waves += [functools.partial(moe_gate, j), functools.partial(moe_up, j)]
    for kc in range(FF // 512):
        waves += [functools.partial(moe_down, kc, nq) for nq in range(4)]
    waves = [None] * opt('mlead', 10) + waves + [None] * opt('mgap', 1) + [moe_apply]
    NM = opt('nm', 6)
    MOE_LATE = EPI

    def finish(rs, cs, acc):
        x_v[rs, cs] = (x_v[rs, cs].astype(F32) + xn_v[rs, cs].astype(F32) + acc).astype(BF16)

    with scope('epi0'):
        for blk in range(EPI // 128):
            ar = OEPI + blk * 128
            r0 = S - EPI + blk * 128
            for n in range(NM):
                acc = None
                for kc in range(NOC):
                    d = _dot(o_vs[kc][ar:ar + 128, :],
                             wo_v[kc * KC // 2:(kc + 1) * KC // 2, n * E:(n + 1) * E])
                    acc = d if acc is None else d + acc
                    if kc == NOC - 1:
                        finish(slice(r0, r0 + 128), slice(n * E, (n + 1) * E), acc)
                    if waves:
                        wv = waves.pop(0)
                        if wv is not None:
                            wv()
        for wv in waves:
            if wv is not None:
                wv()

    fixes = [pltpu.make_async_copy(fix_v.at[n], out_hbm.at[pl.ds(grp[n], 8)], sem_o.at[3 + n])
             for n in range(2)]
    need = [sel[0] < S - EPI, jnp.logical_and(sel[1] < S - EPI, grp[1] != grp[0])]
    out_copy(0, S - EPI, 0).wait()
    for n in range(2):
        @pl.when(need[n])
        def _():
            fixes[n].start()

    def epi(blk, carry):
        ar = pl.ds(pl.multiple_of(OEPI + blk * 128, 16), 128)
        a = jnp.concatenate([oc[ar, :] for oc in o_vs], axis=1)
        r0 = pl.multiple_of(S - EPI + blk * 128, 128)
        finish(pl.ds(r0, 128), slice(NM * E, D), _dot(a, wo_v[:, NM * E:]))
        out_copy(r0, 128, 1 + blk).start()
        return carry

    with scope('epi'):
        lax.fori_loop(0, EPI // 128, epi, 0)

    with scope('fin'):
        for n in range(2):
            @pl.when(need[n])
            def _():
                fixes[n].wait()
        for blk in range(EPI // 128):
            out_copy(S - EPI + blk * 128, 128, 1 + blk).wait()


@jax.jit
def pallas_parallel_sum__memory_aug_recurrent_mem_tr__moe_arch_mod__prompt_kernel(
    A_x: jax.Array,
    A_mem0: jax.Array,
    A_Wq: jax.Array,
    A_Wk: jax.Array,
    A_Wv: jax.Array,
    A_Wo: jax.Array,
    A_seg_len: jax.Array,
    B_x: jax.Array,
    B_w_r: jax.Array,
    B_w_gate: jax.Array,
    B_w_up: jax.Array,
    B_w_down: jax.Array,
):
    del A_seg_len, B_x
    assert A_x.shape == (1, S, D) and A_Wq.shape == (D, H, E) and A_mem0.shape == (1, M, D)
    wshape = (D // 2, 2, NP, 2, E)
    any_spec = pl.BlockSpec(memory_space=pl.ANY)
    out = pl.pallas_call(
        _kernel,
        out_shape=jax.ShapeDtypeStruct((S, D), BF16),
        in_specs=[any_spec] * 10,
        out_specs=any_spec,
        scratch_shapes=[
            pltpu.VMEM((S, D), BF16),
            pltpu.VMEM((S, D), BF16),
            pltpu.VMEM((PRE // 2, D), U32) if opt('xpn', 1) else pltpu.VMEM((PRE, D), BF16),
            pltpu.VMEM((M, D), BF16),
            pltpu.VMEM((NS, 3, NP, L2, E), BF16),
            pltpu.VMEM((NCH + 1, D // 2, 2 * E), U32),
            pltpu.VMEM((H * E // 2, D), U32),
            pltpu.VMEM((NST + 1, 3, 2, D // 2, E), U32),
            pltpu.VMEM((D // 2, 2 * E), U32),
            pltpu.VMEM((D // 2, 2 * E), U32),
            pltpu.VMEM((D // 2, 2 * E), U32),
            pltpu.VMEM((D // 2, FF), U32),
            pltpu.VMEM((D // 2, FF), U32),
            pltpu.VMEM((FF // 2, D), U32),
            pltpu.VMEM((D // E, E), BF16),
            pltpu.VMEM((8, D), F32),
            pltpu.VMEM((L2, L2), F32),
            pltpu.VMEM((2, 8, D), BF16),
            pltpu.SemaphoreType.DMA((2,)),
            pltpu.SemaphoreType.DMA,
            pltpu.SemaphoreType.DMA((2,)),
            pltpu.SemaphoreType.DMA((NST + 1, 3, 2)),
            pltpu.SemaphoreType.DMA,
            pltpu.SemaphoreType.DMA((3,)),
            pltpu.SemaphoreType.DMA((5,)),
            *[pltpu.VMEM((OEPI + EPI, KC), BF16)] * NOC,
        ],
        compiler_params=pltpu.CompilerParams(vmem_limit_bytes=120 * 1024 * 1024,
                                             disable_bounds_checks=True),
    )(
        A_x.reshape(S, D),
        A_mem0.reshape(M, D),
        A_Wq.reshape(wshape),
        A_Wk.reshape(wshape),
        A_Wv.reshape(wshape),
        A_Wo.reshape(H * E, D),
        B_w_r.reshape(D // E, E),
        B_w_gate,
        B_w_up,
        B_w_down,
    )
    return out.reshape(1, S, D)
```

```python
import functools
import os

import jax
import jax.numpy as jnp
from jax import lax
import jax.experimental.pallas as pl
import jax.experimental.pallas.tpu as pltpu

OPT = dict(kv.split('=') for kv in os.environ.get('KOPT', '').split(',') if kv)


def opt(k, d):
    return int(OPT.get(k, d))


class _NoScope:
    def __enter__(self):
        return self

    def __exit__(self, *a):
        return False


def scope(name):
    return jax.named_scope(name) if opt('scopes', 0) else _NoScope()


F32 = jnp.float32
BF16 = jnp.bfloat16
U32 = jnp.uint32

S = 2048
D = 1024
H = 32
E = 128
M = 8
SEG = 32
NSEG = S // SEG
FF = 3584
NP = H // 2
L1 = M + SEG
L2 = 2 * L1

PRE = 512
TPS = 24
NS = 17
U = 4
WG = (3, 3, 3, 5)
WGS = (0, 3, 6, 9)
GPI = sum(WG)
REC = (GPI + U) * 8
NREC = 4
EPI = S - (NSEG // U) * GPI * 8
OEPI = NREC * REC
NST = 2
NCH = 3 * NP
NOC = 8
KC = H * E // NOC
PPC = NP // NOC
OGR = [int(c) for c in OPT.get('ogr', '11111111')]
OMAP = [(a, k) for a, n in enumerate(OGR) for k in range(n)]
RSPLIT = opt('rsplit', 1)
XA = PRE // 2
XBR = (S - PRE) // NP
WOP = (H * E // 2) // NP
KS = D // 2

EPS = 1e-05
SCALE = float(E) ** -0.5
LOG2E = 1.4426950408889634


def _mod17(x):
    return x - 17 * ((x * 241) >> 12)


def _div14(x):
    return (x * 293) >> 12


assert NS == 17 and SEG == 32 and GPI == 14
assert all(_mod17(x) == x % 17 for x in range(128))
assert all(_div14(x) == x // 14 for x in range(256))
assert all(min((r * 11) >> 5, 3) == max(u for u in range(U) if WGS[u] <= r) for r in range(GPI))


def _rb(v):
    return v.astype(BF16).astype(F32)


def _recip(v):
    y = pl.reciprocal(v, approx=True)
    return y * (2.0 - v * y)


def _layernorm_rows(xb, wr8):
    xf = xb.astype(F32)
    mean = jnp.sum(xf, axis=-1, keepdims=True) * (1.0 / D)
    mb = _rb(mean)
    d = xf - mb
    dm = mean - mb
    var = jnp.maximum(jnp.sum(d * d, axis=-1, keepdims=True) * (1.0 / D) - dm * dm, 0.0)
    ve = _rb(_rb(var) + EPS)
    if opt('lnq', 1):
        inv = _recip(_rb(ve * lax.rsqrt(ve)))
    else:
        inv = 1.0 / _rb(jnp.sqrt(ve))
    xw = d * inv
    wr = jnp.concatenate([wr8] * (xb.shape[0] // 8), axis=0)
    r = _rb(jnp.sum(xw * wr, axis=-1, keepdims=True))
    return xw, r


def _scatter_scores(acc, r, g0):
    lane = lax.broadcasted_iota(jnp.int32, acc.shape, 1)
    for j in range(r.shape[0] // 8):
        acc = jnp.where(lane == g0 + j, r[j * 8:(j + 1) * 8, :], acc)
    return acc


def _dot(a, w32):
    return jnp.dot(a, pltpu.bitcast(w32, BF16), preferred_element_type=F32)


def _kernel(x_hbm, mem0_hbm, wq_hbm, wk_hbm, wv_hbm, wo_hbm, wr_hbm, wg_hbm, wu_hbm, wd_hbm,
            out_hbm,
            x_v, xn_v, xp_v, mem0_v, wqkv, wo_v, stage, wc0, wc1, wc2, wg_v, wu_v, wd_v,
            wr_v, fix_v,
            sem_xa, sem_xb, sem_s, sem_st, sem_wo, sem_w, sem_o, *rest):
    w32 = [w.bitcast(U32) for w in (wq_hbm, wk_hbm, wv_hbm)]
    wo32 = wo_hbm.bitcast(U32)
    wcur = (wc0, wc1, wc2)
    rings, o_vs = rest[:3 if RSPLIT else 1], rest[3 if RSPLIT else 1:-2]
    fill_v, wr_in = rest[-2:]

    class _Ring:
        def __getitem__(self, ix):
            return rings[ix[1]][(ix[0],) + ix[2:]] if RSPLIT else rings[0][ix]

        def __setitem__(self, ix, v):
            if RSPLIT:
                rings[ix[1]][(ix[0],) + ix[2:]] = v
            else:
                rings[0][ix] = v

    ring = _Ring()

    def o_ld(c, rows):
        oa, ok = OMAP[c]
        return o_vs[oa][rows, ok * KC:(ok + 1) * KC]

    def xa_copy(c):
        n = XA if c == 0 else PRE + TPS - XA
        return pltpu.make_async_copy(x_hbm.at[pl.ds(c * XA, n)], x_v.at[pl.ds(c * XA, n)],
                                     sem_xa.at[c])

    def xb_copy(i):
        r0 = pl.multiple_of(PRE + i * XBR, 32)
        return pltpu.make_async_copy(x_hbm.at[pl.ds(r0, XBR)], x_v.at[pl.ds(r0, XBR)], sem_xb)

    def st_copy(t, p, slot, k, dp):
        return pltpu.make_async_copy(w32[t].at[:, dp, p, 0, :], stage.at[slot, k, dp],
                                     sem_st.at[slot, k, dp])

    def grp_copies(g):
        slot = g & (NST - 1)
        cps = []
        for k, (t, p) in enumerate(((1, g), (2, g), (0, g + 1))):
            p = jnp.minimum(p, NP - 1)
            cps += [st_copy(t, p, slot, k, 0), st_copy(t, p, slot, k, 1)]
        return cps

    def wo_copy(i):
        r0 = pl.multiple_of(i * WOP, 8)
        return pltpu.make_async_copy(wo32.at[pl.ds(r0, WOP)], wo_v.at[pl.ds(r0, WOP)], sem_wo)

    mem0_copy = pltpu.make_async_copy(mem0_hbm, mem0_v, sem_s.at[0])
    wr_copy = pltpu.make_async_copy(wr_hbm, wr_in, sem_s.at[1])
    first_copies = [st_copy(0, 0, NST, 0, 0), st_copy(0, 0, NST, 0, 1)]
    moe_copies = [pltpu.make_async_copy(src.bitcast(U32), dst, sem_w.at[k])
                  for k, (src, dst) in enumerate(((wg_hbm, wg_v), (wu_hbm, wu_v), (wd_hbm, wd_v)))]

    cps0 = grp_copies(0)
    xa_copy(0).start()
    wr_copy.start()
    for cp in first_copies:
        cp.start()
    xa_copy(1).start()

    row = lax.broadcasted_iota(jnp.int32, (L2, L2), 0)
    col = lax.broadcasted_iota(jnp.int32, (L2, L2), 1)
    rl = jnp.where(row >= L1, row - L1, row)
    cl = jnp.where(col >= L1, col - L1, col)
    same = (row >= L1) == (col >= L1)
    keep = (rl < M) | (rl >= cl)
    fill_v[...] = jnp.where(same, jnp.where(keep, 0.0, -1000000000.0), -jnp.inf).astype(F32)

    def ln_rows(r0, n, racc):
        LR = opt('lnr', 32)
        for j in range(n // LR):
            r = r0 + j * LR
            rs = pl.ds(r if isinstance(r, int) else pl.multiple_of(r, LR), LR)
            xw, sc = _layernorm_rows(x_v[rs, :], wr_v[...])
            r2 = r // 2 if isinstance(r, int) else pl.multiple_of(r >> 1, LR // 2)
            xn_v[rs, :] = xw.astype(BF16)
            xp_v[pl.ds(r2, LR // 2), :] = pltpu.bitcast(xn_v[rs, :], U32)
            racc = _scatter_scores(racc, sc, r // 8 if isinstance(r, int) else r >> 3)
        return racc

    def ln_step(i, racc):
        ic = jnp.minimum(i, NSEG - 1)
        r0 = pl.multiple_of(PRE + ic * TPS, 8)
        xw, r = _layernorm_rows(x_v[pl.ds(r0, TPS), :], wr_v[...])
        xn_v[pl.ds(r0, TPS), :] = xw.astype(BF16)
        return _scatter_scores(racc, r, PRE // 8 + ic * (TPS // 8))

    with scope('ln0'):
        wr_copy.wait()
        wrf = wr_in[...].astype(F32)
        wr_v[...] = jnp.broadcast_to(
            jnp.concatenate([wrf[k:k + 1, :] for k in range(D // E)], axis=1), (8, D))
        xa_copy(0).wait()
        for cp in cps0:
            cp.start()
        LB = opt('lnb', 256)
        racc = jnp.zeros((8, S // 8), F32)
        if LB == XA:
            racc = ln_rows(0, XA, racc)
        else:
            racc = lax.fori_loop(0, XA // LB, lambda i, ra: ln_rows(i * LB, LB, ra), racc)

    def relayout(slot, k, c, dst):
        for j in range(D // 2 // 64):
            a = stage[slot, k, 0, j * 64:(j + 1) * 64, :]
            b = stage[slot, k, 1, j * 64:(j + 1) * 64, :]
            ev = (a & jnp.uint32(0xFFFF)) | (b << 16)
            od = (a >> 16) | (b & jnp.uint32(0xFFFF0000))
            dst[j * 64:(j + 1) * 64, 0:E] = ev
            dst[j * 64:(j + 1) * 64, E:2 * E] = od
            wqkv[c, j * 64:(j + 1) * 64, 0:E] = ev
            wqkv[c, j * 64:(j + 1) * 64, E:2 * E] = od

    MB = opt('promb', 256)

    def pro_dots(t, p):
        for rb in range(PRE // MB):
            if opt('xpn', 1):
                a = pltpu.bitcast(xp_v[rb * MB // 2:(rb + 1) * MB // 2, :], BF16)
            else:
                a = xp_v[rb * MB:(rb + 1) * MB, :]
            y = _dot(a, wcur[t][...]).astype(BF16)
            for sg in range(MB // SEG):
                for hh in range(2):
                    ring[rb * (MB // SEG) + sg, t, p, hh * L1 + M:(hh + 1) * L1, :] = (
                        y[sg * SEG:(sg + 1) * SEG, hh * E:(hh + 1) * E])

    with scope('blkB'):
        for cp in first_copies:
            cp.wait()
        xa_copy(1).wait()
        mem0_copy.start()
        for cp in grp_copies(1):
            cp.start()
        relayout(NST, 0, 0, wc0)
        racc = ln_rows(XA, PRE - XA, racc)
        pro_dots(0, 0)
        racc = ln_step(0, racc)
    with scope('blkC'):
        for cp in cps0[:4]:
            cp.wait()
        wo_copy(0).start()
        xb_copy(0).start()
        relayout(0, 0, 1, wc1)
        relayout(0, 1, 2, wc2)
        pro_dots(1, 0)
    with scope('blkD'):
        for cp in cps0[4:]:
            cp.wait()
        relayout(0, 2, 3, wc0)
        pro_dots(2, 0)

    def pro(p, carry):
        for cp in grp_copies(p):
            cp.wait()
        for cp in grp_copies(p + 1):
            cp.start()
        wo_copy(p).start()
        xb_copy(p).start()
        slot = p & (NST - 1)
        for t in range(3):
            relayout(slot, t, 3 * p + t + 1, wcur[(t + 1) % 3])
            pro_dots(t, p)
        return carry

    with scope('pro'):
        lax.fori_loop(1, NP, pro, 0)

    for cp in grp_copies(NP):
        cp.wait()
    pltpu.make_async_copy(x_hbm.at[pl.ds(PRE, S - PRE)], x_v.at[pl.ds(PRE, S - PRE)], sem_xb).wait()
    mem0_copy.wait()
    pltpu.make_async_copy(wo32, wo_v, sem_wo).wait()

    def step(it, u, carry):
        racc, mem = carry
        s = it * U + u
        slot = _mod17(s)
        t0 = pl.multiple_of(PRE + s * TPS, 8)
        top = xn_v[pl.ds(t0, 8), :].astype(F32)
        bot = xn_v[pl.ds(t0 + 8, 16), :]
        lhs = jnp.concatenate([jnp.concatenate([mem, top], axis=0).astype(BF16), bot], axis=0)
        part = [_dot(lhs[:, :KS], wqkv[t, 0:KS // 2, :]) for t in range(3)]
        qdst = []
        for j in range(TPS // 8):
            tj = t0 + 8 * j
            qdst.append((_mod17(tj >> 5), M + (tj & (SEG - 1))))
        odst = []
        for j in range(SEG // 8):
            g = (SEG // 8) * s + j
            gi = _div14(g)
            gr = g - GPI * gi
            r_ring = (gi & (NREC - 1)) * REC + (gr + 1 + jnp.minimum((gr * 11) >> 5, 3)) * 8
            r_epi = OEPI + (g - (S - EPI) // 8) * 8
            odst.append(pl.multiple_of(jnp.where(g < (S - EPI) // 8, r_ring, r_epi), 8))
        orow = pl.multiple_of((it & (NREC - 1)) * REC + (WGS[u] + u) * 8, 16)
        nw = WG[u] * 8
        if opt('fake', 0) & 1:
            slot = u
            qdst = [(4 + u, 8 + 8 * j) for j in range(3)]
        if opt('fake', 0) & 2:
            odst = [REC + 8 + 8 * j + 40 * u for j in range(4)]
        if opt('fake', 0) & 4:
            orow = (WGS[u] + u) * 8

        def qkv(p, t):
            if p == 0:
                y = _dot(lhs[:, KS:], wqkv[t, KS // 2:, :]) + part[t]
            elif opt('n128', 0):
                y = jnp.concatenate([_dot(lhs, wqkv[3 * p + t, :, hh * E:(hh + 1) * E])
                                     for hh in range(2)], axis=1)
            else:
                y = _dot(lhs, wqkv[3 * p + t])
            y = y.astype(BF16)
            for hh in range(2):
                yc = y[:, hh * E:(hh + 1) * E]
                ring[slot, t, p, hh * L1:hh * L1 + M, :] = yc[0:M]
                for j in range(TPS // 8):
                    qs, qr = qdst[j]
                    ring[qs, t, p, pl.ds(hh * L1 + qr if isinstance(qr, int) else pl.multiple_of(hh * L1 + qr, 8), 8), :] = (
                        yc[M + 8 * j:M + 8 * j + 8])

        def attn_a(q, k):
            sc = lax.dot_general(q, k, (((1,), (1,)), ((), ())), preferred_element_type=F32)
            fill = fill_v[...]
            if opt('sm', 0) == 0:
                sc = jnp.where(fill == 0.0, sc * SCALE, fill)
                e = jnp.exp(sc - jnp.max(sc, axis=-1, keepdims=True))
            elif opt('sm', 0) == 1:
                sc = jnp.where(fill == 0.0, sc * (SCALE * LOG2E), fill * LOG2E)
                e = jnp.exp2(sc - jnp.max(sc, axis=-1, keepdims=True))
            den = jnp.sum(e, axis=-1, keepdims=True)
            return (e * pl.reciprocal(den, approx=True)).astype(BF16)

        def attn_b(p, pr, v):
            o = jnp.dot(pr, v, preferred_element_type=F32).astype(BF16)
            oa, ok = OMAP[p // PPC]
            oc = o_vs[oa]
            for hh in range(2):
                cs = ok * KC + (2 * (p % PPC) + hh) * E
                oc[pl.ds(orow, M), cs:cs + E] = o[hh * L1:hh * L1 + M]
                for j in range(SEG // 8):
                    r = hh * L1 + M + 8 * j
                    oc[pl.ds(odst[j], 8), cs:cs + E] = o[r:r + 8]

        def wo_chunk(c, c1):
            a = jnp.concatenate([o_ld(i, pl.ds(orow, M + nw)) for i in range(c, c1)], axis=1)
            return _dot(a, wo_v[c * KC // 2:c1 * KC // 2, :])

        wl = OPT.get('wl', '0.1.2.3.4.5.6-7').split('.')
        nslot = 3 * NP + len(wl)
        ev = {n: [] for n in range(nslot + 1)}
        lq, aa, lv, bb = opt('lq', 3), opt('a', 5), opt('lv', 7), opt('b', 9)
        ta = [int(x) for x in OPT.get('ta', '50').split('.')]
        tb = [int(x) for x in OPT.get('tb', '49.51.53').split('.')]
        for p in range(NP):
            pa_ = 3 * p + aa if p < NP - len(ta) else ta[p - (NP - len(ta))]
            pb_ = 3 * p + bb if p < NP - len(tb) else tb[p - (NP - len(tb))]
            ql, vl = min(3 * p + lq, pa_), min(3 * p + lv, pb_)
            if 'ga' in OPT:
                G = opt('G', 4)
                pa_ = [int(x) for x in OPT['ga'].split('.')][p // G]
                pb_ = [int(x) for x in OPT['gb'].split('.')][p // G]
                ql = max(3 * p + 2, pa_ - opt('gl', 2))
                vl = max(3 * p + 3, pb_ - opt('gl', 2))
            assert pa_ <= pb_ <= nslot
            ev[ql].append((0, 'Q', p))
            ev[vl].append((1, 'V', p))
            ev[pa_].append((3, 'A', p))
            ev[pb_].append((2, 'B', p))
        pe, qk, vv = {}, {}, {}
        acc = None
        r0 = pl.multiple_of((it * GPI + WGS[u]) * 8, 8)
        for n in range(nslot + 1):
            for _, kind, p in sorted(ev[n]):
                if kind == 'Q':
                    qk[p] = (ring[slot, 0, p], ring[slot, 1, p])
                elif kind == 'V':
                    vv[p] = ring[slot, 2, p]
                elif kind == 'A':
                    pe[p] = attn_a(*qk.pop(p))
                else:
                    attn_b(p, pe.pop(p), vv.pop(p))
            if n == opt('lnpos', 99):
                base = x_v[pl.ds(r0, nw), :].astype(F32) + xn_v[pl.ds(r0, nw), :].astype(F32)
                racc = ln_step(s + 1, racc)
            if n < 3 * NP:
                qkv(n // 3, [int(c) for c in OPT.get('mo', '012')][n % 3])
            elif n < nslot:
                tk = wl[n - 3 * NP].split('-')
                y = wo_chunk(int(tk[0]), int(tk[-1]) + 1)
                acc = y if acc is None else y + acc
        if opt('lnpos', 99) > nslot:
            base = x_v[pl.ds(r0, nw), :].astype(F32) + xn_v[pl.ds(r0, nw), :].astype(F32)
        if opt('lnpos', 99) > nslot:
            racc = ln_step(s + 1, racc)
        x_v[pl.ds(r0, nw), :] = (base + acc[M:]).astype(BF16)
        return racc, acc[0:M]

    def steps(it, carry):
        def start_moe(_, c):
            for cp in moe_copies:
                cp.start()
            return c

        lax.fori_loop(0, (it == 1).astype(jnp.int32), start_moe, 0)

        with scope('it'):
            for u in range(U):
                carry = step(it, u, carry)
        return carry

    with scope('main'):
        racc, _ = lax.fori_loop(0, NSEG // U, steps, (racc, mem0_v[...].astype(F32)))

    def out_copy(r0, n, k):
        return pltpu.make_async_copy(x_v.at[pl.ds(r0, n)], out_hbm.at[pl.ds(r0, n)], sem_o.at[k])

    for cp in moe_copies:
        cp.wait()
    out_copy(0, S - EPI, 0).start()

    idx = (lax.broadcasted_iota(jnp.int32, racc.shape, 1) * 8
           + lax.broadcasted_iota(jnp.int32, racc.shape, 0)).astype(F32)

    def allred(fn, v):
        return fn(fn(v, axis=1, keepdims=True), axis=0, keepdims=True)

    m1 = allred(jnp.max, racc)
    i1 = allred(jnp.min, jnp.where(racc == m1, idx, float(S - 1)))
    r2 = jnp.where(idx == i1, -jnp.inf, racc)
    m2 = allred(jnp.max, r2)
    i2 = allred(jnp.min, jnp.where((r2 == m2) & (idx != i1), idx, float(S - 1)))
    sel = [jnp.clip(jnp.max(iv).astype(jnp.int32), 0, S - 1) for iv in (i1, i2)]
    grp = [pl.multiple_of((i >> 3) << 3, 8) for i in sel]
    row8 = lax.broadcasted_iota(jnp.int32, (8, D), 0)
    rows = [jnp.sum(jnp.where(row8 == (i & 7), xn_v[pl.ds(g, 8), :].astype(F32), 0.0),
                    axis=0, keepdims=True) for i, g in zip(sel, grp)]
    row16 = lax.broadcasted_iota(jnp.int32, (16, D), 0)
    xs = jnp.where(row16 == 0, rows[0], jnp.where(row16 == 1, rows[1], 0.0)).astype(BF16)

    hs, ys, gps = {}, {}, {}

    def moe_gate(j):
        gps[j] = _rb(_dot(xs, wg_v[:, j * E:(j + 1) * E]))

    def moe_up(j):
        up = _rb(_dot(xs, wu_v[:, j * E:(j + 1) * E]))
        gp = gps.pop(j)
        g = _rb(gp * (1.0 / (1.0 + jnp.exp(-gp))))
        hs[j] = (g * up).astype(BF16)

    def moe_down(kc, nq):
        hk = jnp.concatenate([hs[4 * kc + i] for i in range(4)], axis=1)
        d = _dot(hk, wd_v[kc * 256:(kc + 1) * 256, nq * 256:(nq + 1) * 256])
        ys[nq] = d + ys[nq] if nq in ys else d

    def moe_apply():
        y = _rb(jnp.concatenate([ys[nq] for nq in range(4)], axis=1))
        upd = [_rb(y[n:n + 1, :] * _rb(1.0 / (1.0 + jnp.exp(-mv)))) for n, mv in enumerate((m1, m2))]
        for n in range(2):
            blk = x_v[pl.ds(grp[n], 8), :].astype(F32)
            for k in range(2):
                blk = blk + jnp.where(row8 + grp[n] == sel[k], upd[k], 0.0)
            fix_v[n] = blk.astype(BF16)
        for n in range(2):
            g = pl.multiple_of(jnp.maximum(grp[n], S - MOE_LATE), 8)
            x_v[pl.ds(g, 8), :] = (x_v[pl.ds(g, 8), :].astype(F32)
                                   + jnp.where(row8 + g == sel[n], upd[n], 0.0)).astype(BF16)

    waves = []
    for j in range(FF // E):
        waves += [functools.partial(moe_gate, j), functools.partial(moe_up, j)]
    for kc in range(FF // 512):
        waves += [functools.partial(moe_down, kc, nq) for nq in range(4)]
    waves = [None] * opt('mlead', 10) + waves + [None] * opt('mgap', 1) + [moe_apply]
    NM = opt('nm', 6)
    MOE_LATE = EPI

    def finish(rs, cs, acc):
        x_v[rs, cs] = (x_v[rs, cs].astype(F32) + xn_v[rs, cs].astype(F32) + acc).astype(BF16)

    with scope('epi0'):
        for blk in range(EPI // 128):
            ar = OEPI + blk * 128
            r0 = S - EPI + blk * 128
            for n in range(NM):
                acc = None
                for kc in range(NOC):
                    d = _dot(o_ld(kc, slice(ar, ar + 128)),
                             wo_v[kc * KC // 2:(kc + 1) * KC // 2, n * E:(n + 1) * E])
                    acc = d if acc is None else d + acc
                    if kc == NOC - 1:
                        finish(slice(r0, r0 + 128), slice(n * E, (n + 1) * E), acc)
                    if waves:
                        wv = waves.pop(0)
                        if wv is not None:
                            wv()
        for wv in waves:
            if wv is not None:
                wv()

    fixes = [pltpu.make_async_copy(fix_v.at[n], out_hbm.at[pl.ds(grp[n], 8)], sem_o.at[3 + n])
             for n in range(2)]
    need = [sel[0] < S - EPI, jnp.logical_and(sel[1] < S - EPI, grp[1] != grp[0])]
    out_copy(0, S - EPI, 0).wait()
    for n in range(2):
        @pl.when(need[n])
        def _():
            fixes[n].start()

    def epi(blk, carry):
        ar = pl.ds(pl.multiple_of(OEPI + blk * 128, 16), 128)
        a = jnp.concatenate([o_ld(c, ar) for c in range(NOC)], axis=1)
        r0 = pl.multiple_of(S - EPI + blk * 128, 128)
        finish(pl.ds(r0, 128), slice(NM * E, D), _dot(a, wo_v[:, NM * E:]))
        out_copy(r0, 128, 1 + blk).start()
        return carry

    with scope('epi'):
        lax.fori_loop(0, EPI // 128, epi, 0)

    with scope('fin'):
        for n in range(2):
            @pl.when(need[n])
            def _():
                fixes[n].wait()
        for blk in range(EPI // 128):
            out_copy(S - EPI + blk * 128, 128, 1 + blk).wait()


@jax.jit
def pallas_parallel_sum__memory_aug_recurrent_mem_tr__moe_arch_mod__prompt_kernel(
    A_x: jax.Array,
    A_mem0: jax.Array,
    A_Wq: jax.Array,
    A_Wk: jax.Array,
    A_Wv: jax.Array,
    A_Wo: jax.Array,
    A_seg_len: jax.Array,
    B_x: jax.Array,
    B_w_r: jax.Array,
    B_w_gate: jax.Array,
    B_w_up: jax.Array,
    B_w_down: jax.Array,
):
    del A_seg_len, B_x
    assert A_x.shape == (1, S, D) and A_Wq.shape == (D, H, E) and A_mem0.shape == (1, M, D)
    wshape = (D // 2, 2, NP, 2, E)
    any_spec = pl.BlockSpec(memory_space=pl.ANY)
    out = pl.pallas_call(
        _kernel,
        out_shape=jax.ShapeDtypeStruct((S, D), BF16),
        in_specs=[any_spec] * 10,
        out_specs=any_spec,
        scratch_shapes=[
            pltpu.VMEM((S, D), BF16),
            pltpu.VMEM((S, D), BF16),
            pltpu.VMEM((PRE // 2, D), U32) if opt('xpn', 1) else pltpu.VMEM((PRE, D), BF16),
            pltpu.VMEM((M, D), BF16),
            pltpu.VMEM((NCH + 1, D // 2, 2 * E), U32),
            pltpu.VMEM((H * E // 2, D), U32),
            pltpu.VMEM((NST + 1, 3, 2, D // 2, E), U32),
            pltpu.VMEM((D // 2, 2 * E), U32),
            pltpu.VMEM((D // 2, 2 * E), U32),
            pltpu.VMEM((D // 2, 2 * E), U32),
            pltpu.VMEM((D // 2, FF), U32),
            pltpu.VMEM((D // 2, FF), U32),
            pltpu.VMEM((FF // 2, D), U32),
            pltpu.VMEM((8, D), F32),
            pltpu.VMEM((2, 8, D), BF16),
            pltpu.SemaphoreType.DMA((2,)),
            pltpu.SemaphoreType.DMA,
            pltpu.SemaphoreType.DMA((2,)),
            pltpu.SemaphoreType.DMA((NST + 1, 3, 2)),
            pltpu.SemaphoreType.DMA,
            pltpu.SemaphoreType.DMA((3,)),
            pltpu.SemaphoreType.DMA((5,)),
            *([pltpu.VMEM((NS, NP, L2, E), BF16)] * 3 if RSPLIT else [pltpu.VMEM((NS, 3, NP, L2, E), BF16)]),
            *[pltpu.VMEM((OEPI + EPI, n * KC), BF16) for n in OGR],
            pltpu.VMEM((L2, L2), F32),
            pltpu.VMEM((D // E, E), BF16),
        ],
        compiler_params=pltpu.CompilerParams(vmem_limit_bytes=120 * 1024 * 1024,
                                             disable_bounds_checks=True),
    )(
        A_x.reshape(S, D),
        A_mem0.reshape(M, D),
        A_Wq.reshape(wshape),
        A_Wk.reshape(wshape),
        A_Wv.reshape(wshape),
        A_Wo.reshape(H * E, D),
        B_w_r.reshape(D // E, E),
        B_w_gate,
        B_w_up,
        B_w_down,
    )
    return out.reshape(1, S, D)
```

```python
import functools
import os

import jax
import jax.numpy as jnp
from jax import lax
import jax.experimental.pallas as pl
import jax.experimental.pallas.tpu as pltpu

OPT = dict(kv.split('=') for kv in os.environ.get('KOPT', '').split(',') if kv)


def opt(k, d):
    return int(OPT.get(k, d))


class _NoScope:
    def __enter__(self):
        return self

    def __exit__(self, *a):
        return False


def scope(name):
    return jax.named_scope(name) if opt('scopes', 0) else _NoScope()


F32 = jnp.float32
BF16 = jnp.bfloat16
U32 = jnp.uint32

S = 2048
D = 1024
H = 32
E = 128
M = 8
SEG = 32
NSEG = S // SEG
FF = 3584
NP = H // 2
L1 = M + SEG
L2 = 2 * L1

PRE = 512
TPS = 24
NS = 17
U = 4
WG = (3, 3, 3, 5)
WGS = (0, 3, 6, 9)
GPI = sum(WG)
REC = (GPI + U) * 8
NREC = 4
EPI = S - (NSEG // U) * GPI * 8
OEPI = NREC * REC
NST = 4
NCH = 3 * NP
NOC = 8
KC = H * E // NOC
PPC = NP // NOC
OGR = [int(c) for c in OPT.get('ogr', '11111111')]
OMAP = [(a, k) for a, n in enumerate(OGR) for k in range(n)]
RSPLIT = opt('rsplit', 1)
RP = opt('rp', 1)
NPR = NP // RP + (RP > 1)
RPAD = (-NPR) % 4
XA = PRE // 2
XBR = (S - PRE) // NP
WOP = (H * E // 2) // NP
KS = D // 2

EPS = 1e-05
SCALE = float(E) ** -0.5
LOG2E = 1.4426950408889634


def _mod17(x):
    return x - 17 * ((x * 241) >> 12)


def _div14(x):
    return (x * 293) >> 12


assert NS == 17 and SEG == 32 and GPI == 14
assert all(_mod17(x) == x % 17 for x in range(128))
assert all(_div14(x) == x // 14 for x in range(256))
assert all(min((r * 11) >> 5, 3) == max(u for u in range(U) if WGS[u] <= r) for r in range(GPI))


def _rb(v):
    return v.astype(BF16).astype(F32)


def _recip(v):
    y = pl.reciprocal(v, approx=True)
    return y * (2.0 - v * y)


def _layernorm_rows(xb, wr8):
    xf = xb.astype(F32)
    mean = jnp.sum(xf, axis=-1, keepdims=True) * (1.0 / D)
    mb = _rb(mean)
    d = xf - mb
    dm = mean - mb
    var = jnp.maximum(jnp.sum(d * d, axis=-1, keepdims=True) * (1.0 / D) - dm * dm, 0.0)
    ve = _rb(_rb(var) + EPS)
    if opt('lnq', 1):
        inv = _recip(_rb(ve * lax.rsqrt(ve)))
    else:
        inv = 1.0 / _rb(jnp.sqrt(ve))
    xw = d * inv
    wr = jnp.concatenate([wr8] * (xb.shape[0] // 8), axis=0)
    r = _rb(jnp.sum(xw * wr, axis=-1, keepdims=True))
    return xw, r


def _scatter_scores(acc, r, g0):
    lane = lax.broadcasted_iota(jnp.int32, acc.shape, 1)
    for j in range(r.shape[0] // 8):
        acc = jnp.where(lane == g0 + j, r[j * 8:(j + 1) * 8, :], acc)
    return acc


def _dot(a, w32):
    return jnp.dot(a, pltpu.bitcast(w32, BF16), preferred_element_type=F32)


def _kernel(x_hbm, mem0_hbm, wq_hbm, wk_hbm, wv_hbm, wo_hbm, wr_hbm, wg_hbm, wu_hbm, wd_hbm,
            out_hbm,
            x_v, xn_v, xp_v, mem0_v, wqkv, wo_v, stage, wc0, wc1, wc2, wg_v, wu_v, wd_v,
            wr_v, fix_v,
            sem_xa, sem_xb, sem_s, sem_st, sem_wo, sem_w, sem_o, *rest):
    w32 = [w.bitcast(U32) for w in (wq_hbm, wk_hbm, wv_hbm)]
    wo32 = wo_hbm.bitcast(U32)
    wcur = (wc0, wc1, wc2)
    nring = (3 if RSPLIT else 1) * RP
    rings, o_vs = rest[:nring], rest[nring:-2]
    fill_v, wr_in = rest[-2:]

    class _Ring:
        def _ix(self, ix, c, pi):
            if RSPLIT:
                return rings[ix[1] * RP + c], (ix[0], pi) + ix[3:]
            return rings[c], (ix[0], ix[1], pi) + ix[3:]

        def __getitem__(self, ix):
            ref, j = self._ix(ix, ix[2] % RP, ix[2] // RP)
            return ref[j]

        def __setitem__(self, ix, v):
            p = ix[2]
            if isinstance(p, int):
                ref, j = self._ix(ix, p % RP, p // RP)
                ref[j] = v
            else:
                for c in range(RP):
                    pi = p if RP == 1 else jnp.where((p & (RP - 1)) == c, p >> (RP // 2), NP // RP)
                    ref, j = self._ix(ix, c, pi)
                    ref[j] = v

    ring = _Ring()

    def o_ld(c, rows):
        oa, ok = OMAP[c]
        return o_vs[oa][rows, ok * KC:(ok + 1) * KC]

    def xa_copy(c):
        n = XA if c == 0 else PRE + TPS - XA
        return pltpu.make_async_copy(x_hbm.at[pl.ds(c * XA, n)], x_v.at[pl.ds(c * XA, n)],
                                     sem_xa.at[c])

    def xb_copy(i):
        src = pl.multiple_of(PRE + jnp.minimum(i, NP - 1) * XBR, 32)
        dst = pl.multiple_of(PRE + i * XBR, 32)
        return pltpu.make_async_copy(x_hbm.at[pl.ds(src, XBR)], x_v.at[pl.ds(dst, XBR)],
                                     sem_xb.at[i >> 4])

    def st_copy(t, p, slot, k, dp, sem):
        return pltpu.make_async_copy(w32[t].at[:, dp, p, 0, :], stage.at[slot, k, dp], sem)

    def grp_start(g, sems=None):
        slot = g & (NST - 1)
        for k, (t, p) in enumerate(((1, g), (2, g), (0, g + 1))):
            p = jnp.minimum(p, NP - 1)
            for dp in range(2):
                st_copy(t, p, slot, k, dp, sem_st.at[slot] if sems is None else sems[k]).start()

    def st_wait(view, sem):
        pltpu.make_async_copy(view, view, sem).wait()

    def grp_wait(g):
        slot = g & (NST - 1)
        st_wait(stage.at[slot], sem_st.at[slot])

    def wo_copy(i):
        src = pl.multiple_of(jnp.minimum(i, NP - 1) * WOP, 8)
        dst = pl.multiple_of(i * WOP, 8)
        return pltpu.make_async_copy(wo32.at[pl.ds(src, WOP)], wo_v.at[pl.ds(dst, WOP)],
                                     sem_wo.at[i >> 4])

    mem0_copy = pltpu.make_async_copy(mem0_hbm, mem0_v, sem_s.at[0])
    wr_copy = pltpu.make_async_copy(wr_hbm, wr_in, sem_s.at[1])
    first_copies = [st_copy(0, 0, NST, 0, dp, sem_st.at[NST]) for dp in range(2)]
    moe_copies = [pltpu.make_async_copy(src.bitcast(U32), dst, sem_w.at[k])
                  for k, (src, dst) in enumerate(((wg_hbm, wg_v), (wu_hbm, wu_v), (wd_hbm, wd_v)))]

    xa_copy(0).start()
    wr_copy.start()
    for cp in first_copies:
        cp.start()
    xa_copy(1).start()

    row = lax.broadcasted_iota(jnp.int32, (L2, L2), 0)
    col = lax.broadcasted_iota(jnp.int32, (L2, L2), 1)
    rl = jnp.where(row >= L1, row - L1, row)
    cl = jnp.where(col >= L1, col - L1, col)
    same = (row >= L1) == (col >= L1)
    keep = (rl < M) | (rl >= cl)
    fill_v[...] = jnp.where(same, jnp.where(keep, 0.0, -1000000000.0 / (SCALE if opt('sm', 2) == 2 else 1.0)), -jnp.inf).astype(F32)

    def ln_rows(r0, n, racc):
        LR = opt('lnr', 32)
        for j in range(n // LR):
            r = r0 + j * LR
            rs = pl.ds(r if isinstance(r, int) else pl.multiple_of(r, LR), LR)
            xw, sc = _layernorm_rows(x_v[rs, :], wr_v[...])
            r2 = r // 2 if isinstance(r, int) else pl.multiple_of(r >> 1, LR // 2)
            xn_v[rs, :] = xw.astype(BF16)
            xp_v[pl.ds(r2, LR // 2), :] = pltpu.bitcast(xn_v[rs, :], U32)
            racc = _scatter_scores(racc, sc, r // 8 if isinstance(r, int) else r >> 3)
        return racc

    def ln_step(i, racc):
        ic = jnp.minimum(i, NSEG - 1)
        r0 = pl.multiple_of(PRE + ic * TPS, 8)
        xw, r = _layernorm_rows(x_v[pl.ds(r0, TPS), :], wr_v[...])
        xn_v[pl.ds(r0, TPS), :] = xw.astype(BF16)
        return _scatter_scores(racc, r, PRE // 8 + ic * (TPS // 8))

    with scope('ln0'):
        wr_copy.wait()
        wrf = wr_in[...].astype(F32)
        wr_v[...] = jnp.broadcast_to(
            jnp.concatenate([wrf[k:k + 1, :] for k in range(D // E)], axis=1), (8, D))
        xa_copy(0).wait()
        grp_start(0, (sem_st.at[0], sem_st.at[0], sem_st.at[NST + 1]))
        LB = opt('lnb', 256)
        racc = jnp.zeros((8, S // 8), F32)
        if LB == XA:
            racc = ln_rows(0, XA, racc)
        else:
            racc = lax.fori_loop(0, XA // LB, lambda i, ra: ln_rows(i * LB, LB, ra), racc)

    def relayout(slot, k, c, dst):
        for j in range(D // 2 // 64):
            a = stage[slot, k, 0, j * 64:(j + 1) * 64, :]
            b = stage[slot, k, 1, j * 64:(j + 1) * 64, :]
            ev = (a & jnp.uint32(0xFFFF)) | (b << 16)
            od = (a >> 16) | (b & jnp.uint32(0xFFFF0000))
            dst[j * 64:(j + 1) * 64, 0:E] = ev
            dst[j * 64:(j + 1) * 64, E:2 * E] = od
            wqkv[c, j * 64:(j + 1) * 64, 0:E] = ev
            wqkv[c, j * 64:(j + 1) * 64, E:2 * E] = od

    MB = opt('promb', 256)

    def pro_dots(t, p):
        for rb in range(PRE // MB):
            if opt('xpn', 1):
                a = pltpu.bitcast(xp_v[rb * MB // 2:(rb + 1) * MB // 2, :], BF16)
            else:
                a = xp_v[rb * MB:(rb + 1) * MB, :]
            y = _dot(a, wcur[t][...]).astype(BF16)
            for sg in range(MB // SEG):
                for hh in range(2):
                    ring[rb * (MB // SEG) + sg, t, p, hh * L1 + M:(hh + 1) * L1, :] = (
                        y[sg * SEG:(sg + 1) * SEG, hh * E:(hh + 1) * E])

    with scope('blkB'):
        st_wait(stage.at[NST, 0], sem_st.at[NST])
        xa_copy(1).wait()
        mem0_copy.start()
        grp_start(1)
        relayout(NST, 0, 0, wc0)
        racc = ln_rows(XA, PRE - XA, racc)
        pro_dots(0, 0)
        racc = ln_step(0, racc)
    with scope('blkC'):
        st_wait(stage.at[0, pl.ds(0, 2)], sem_st.at[0])
        grp_start(2)
        relayout(0, 0, 1, wc1)
        relayout(0, 1, 2, wc2)
        pro_dots(1, 0)
    with scope('blkD'):
        st_wait(stage.at[0, 2], sem_st.at[NST + 1])
        for i in range(3):
            wo_copy(i).start()
            xb_copy(i).start()
        relayout(0, 2, 3, wc0)
        pro_dots(2, 0)

    def pro(p, carry):
        grp_wait(p)
        slot = p & (NST - 1)
        for t in range(3):
            relayout(slot, t, 3 * p + t + 1, wcur[(t + 1) % 3])
            pro_dots(t, p)

        grp_start(p + 2)
        wo_copy(p + 2).start()
        xb_copy(p + 2).start()
        return carry

    with scope('pro'):
        lax.fori_loop(1, NP, pro, 0)

    st_wait(x_v.at[pl.ds(PRE, S - PRE)], sem_xb.at[0])
    mem0_copy.wait()
    st_wait(wo_v.at[pl.ds(0, NP * WOP)], sem_wo.at[0])

    def step(it, u, carry):
        racc, mem = carry
        s = it * U + u
        slot = _mod17(s)
        t0 = pl.multiple_of(PRE + s * TPS, 8)
        top = xn_v[pl.ds(t0, 8), :].astype(F32)
        bot = xn_v[pl.ds(t0 + 8, 16), :]
        lhs = jnp.concatenate([jnp.concatenate([mem, top], axis=0).astype(BF16), bot], axis=0)
        part = [_dot(lhs[:, :KS], wqkv[t, 0:KS // 2, :]) for t in range(3)]
        qdst = []
        for j in range(TPS // 8):
            tj = t0 + 8 * j
            qdst.append((_mod17(tj >> 5), M + (tj & (SEG - 1))))
        odst = []
        for j in range(SEG // 8):
            g = (SEG // 8) * s + j
            gi = _div14(g)
            gr = g - GPI * gi
            r_ring = (gi & (NREC - 1)) * REC + (gr + 1 + jnp.minimum((gr * 11) >> 5, 3)) * 8
            r_epi = OEPI + (g - (S - EPI) // 8) * 8
            odst.append(pl.multiple_of(jnp.where(g < (S - EPI) // 8, r_ring, r_epi), 8))
        orow = pl.multiple_of((it & (NREC - 1)) * REC + (WGS[u] + u) * 8, 16)
        nw = WG[u] * 8
        if opt('fake', 0) & 1:
            slot = u
            qdst = [(4 + u, 8 + 8 * j) for j in range(3)]
        if opt('fake', 0) & 2:
            odst = [REC + 8 + 8 * j + 40 * u for j in range(4)]
        if opt('fake', 0) & 4:
            orow = (WGS[u] + u) * 8

        def qkv(p, t):
            if p == 0:
                y = _dot(lhs[:, KS:], wqkv[t, KS // 2:, :]) + part[t]
            elif opt('n128', 0):
                y = jnp.concatenate([_dot(lhs, wqkv[3 * p + t, :, hh * E:(hh + 1) * E])
                                     for hh in range(2)], axis=1)
            else:
                y = _dot(lhs, wqkv[3 * p + t])
            y = y.astype(BF16)
            for hh in range(2):
                yc = y[:, hh * E:(hh + 1) * E]
                ring[slot, t, p, hh * L1:hh * L1 + M, :] = yc[0:M]
                for j in range(TPS // 8):
                    qs, qr = qdst[j]
                    ring[qs, t, p, pl.ds(hh * L1 + qr if isinstance(qr, int) else pl.multiple_of(hh * L1 + qr, 8), 8), :] = (
                        yc[M + 8 * j:M + 8 * j + 8])

        def attn_a(q, k):
            sc = lax.dot_general(q, k, (((1,), (1,)), ((), ())), preferred_element_type=F32)
            fill = fill_v[...]
            if opt('sm', 2) == 0:
                sc = jnp.where(fill == 0.0, sc * SCALE, fill)
                e = jnp.exp(sc - jnp.max(sc, axis=-1, keepdims=True))
            elif opt('sm', 2) == 1:
                sc = jnp.where(fill == 0.0, sc * (SCALE * LOG2E), fill * LOG2E)
                e = jnp.exp2(sc - jnp.max(sc, axis=-1, keepdims=True))
            else:
                sc = jnp.where(fill == 0.0, sc, fill)
                e = jnp.exp2((sc - jnp.max(sc, axis=-1, keepdims=True)) * (SCALE * LOG2E))
            den = jnp.sum(e, axis=-1, keepdims=True)
            return (e * pl.reciprocal(den, approx=True)).astype(BF16)

        def attn_b(p, pr, v):
            o = jnp.dot(pr, v, preferred_element_type=F32).astype(BF16)
            oa, ok = OMAP[p // PPC]
            oc = o_vs[oa]
            for hh in range(2):
                cs = ok * KC + (2 * (p % PPC) + hh) * E
                oc[pl.ds(orow, M), cs:cs + E] = o[hh * L1:hh * L1 + M]
                for j in range(SEG // 8):
                    r = hh * L1 + M + 8 * j
                    oc[pl.ds(odst[j], 8), cs:cs + E] = o[r:r + 8]

        def wo_chunk(c, c1):
            a = jnp.concatenate([o_ld(i, pl.ds(orow, M + nw)) for i in range(c, c1)], axis=1)
            return _dot(a, wo_v[c * KC // 2:c1 * KC // 2, :])

        wl = OPT.get('wl', '0.1.2.3.4.5.6-7').split('.')
        nslot = 3 * NP + len(wl)
        ev = {n: [] for n in range(nslot + 1)}
        lq, aa, lv, bb = opt('lq', 2), opt('a', 4), opt('lv', 6), opt('b', 8)
        ta = [int(x) for x in OPT.get('ta', '50').split('.')]
        tb = [int(x) for x in OPT.get('tb', '50.53').split('.')]
        for p in range(NP):
            pa_ = 3 * p + aa if p < NP - len(ta) else ta[p - (NP - len(ta))]
            pb_ = 3 * p + bb if p < NP - len(tb) else tb[p - (NP - len(tb))]
            ql, vl = min(3 * p + lq, pa_), min(3 * p + lv, pb_)
            if 'ga' in OPT:
                G = opt('G', 4)
                pa_ = [int(x) for x in OPT['ga'].split('.')][p // G]
                pb_ = [int(x) for x in OPT['gb'].split('.')][p // G]
                ql = max(3 * p + 2, pa_ - opt('gl', 2))
                vl = max(3 * p + 3, pb_ - opt('gl', 2))
            assert pa_ <= pb_ <= nslot
            ev[ql].append((0, 'Q', p))
            ev[vl].append((1, 'V', p))
            ev[pa_].append((3, 'A', p))
            ev[pb_].append((2, 'B', p))
        pe, qk, vv = {}, {}, {}
        acc = None
        r0 = pl.multiple_of((it * GPI + WGS[u]) * 8, 8)
        for n in range(nslot + 1):
            for _, kind, p in sorted(ev[n]):
                if kind == 'Q':
                    qk[p] = (ring[slot, 0, p], ring[slot, 1, p])
                elif kind == 'V':
                    vv[p] = ring[slot, 2, p]
                elif kind == 'A':
                    pe[p] = attn_a(*qk.pop(p))
                else:
                    attn_b(p, pe.pop(p), vv.pop(p))
            if n == opt('lnpos', 99):
                base = x_v[pl.ds(r0, nw), :].astype(F32) + xn_v[pl.ds(r0, nw), :].astype(F32)
                racc = ln_step(s + 1, racc)
            if n < 3 * NP:
                qkv(n // 3, [int(c) for c in OPT.get('mo', '012')][n % 3])
            elif n < nslot:
                tk = wl[n - 3 * NP].split('-')
                y = wo_chunk(int(tk[0]), int(tk[-1]) + 1)
                acc = y if acc is None else y + acc
        if opt('lnpos', 99) > nslot:
            base = x_v[pl.ds(r0, nw), :].astype(F32) + xn_v[pl.ds(r0, nw), :].astype(F32)
        if opt('lnpos', 99) > nslot:
            racc = ln_step(s + 1, racc)
        x_v[pl.ds(r0, nw), :] = (base + acc[M:]).astype(BF16)
        return racc, acc[0:M]

    def steps(it, carry):
        def start_moe(_, c):
            for cp in moe_copies:
                cp.start()
            return c

        lax.fori_loop(0, (it == 1).astype(jnp.int32), start_moe, 0)

        with scope('it'):
            for u in range(U):
                carry = step(it, u, carry)
        return carry

    with scope('main'):
        racc, _ = lax.fori_loop(0, NSEG // U, steps, (racc, mem0_v[...].astype(F32)))

    def out_copy(r0, n, k):
        return pltpu.make_async_copy(x_v.at[pl.ds(r0, n)], out_hbm.at[pl.ds(r0, n)], sem_o.at[k])

    for cp in moe_copies:
        cp.wait()
    grp_wait(NP)
    grp_wait(NP + 1)
    st_wait(x_v.at[pl.ds(S, 2 * XBR)], sem_xb.at[1])
    st_wait(wo_v.at[pl.ds(NP * WOP, 2 * WOP)], sem_wo.at[1])
    out_copy(0, S - EPI, 0).start()

    idx = (lax.broadcasted_iota(jnp.int32, racc.shape, 1) * 8
           + lax.broadcasted_iota(jnp.int32, racc.shape, 0)).astype(F32)

    def allred(fn, v):
        return fn(fn(v, axis=1, keepdims=True), axis=0, keepdims=True)

    m1 = allred(jnp.max, racc)
    i1 = allred(jnp.min, jnp.where(racc == m1, idx, float(S - 1)))
    r2 = jnp.where(idx == i1, -jnp.inf, racc)
    m2 = allred(jnp.max, r2)
    i2 = allred(jnp.min, jnp.where((r2 == m2) & (idx != i1), idx, float(S - 1)))
    sel = [jnp.clip(jnp.max(iv).astype(jnp.int32), 0, S - 1) for iv in (i1, i2)]
    grp = [pl.multiple_of((i >> 3) << 3, 8) for i in sel]
    row8 = lax.broadcasted_iota(jnp.int32, (8, D), 0)
    rows = [jnp.sum(jnp.where(row8 == (i & 7), xn_v[pl.ds(g, 8), :].astype(F32), 0.0),
                    axis=0, keepdims=True) for i, g in zip(sel, grp)]
    row16 = lax.broadcasted_iota(jnp.int32, (16, D), 0)
    xs = jnp.where(row16 == 0, rows[0], jnp.where(row16 == 1, rows[1], 0.0)).astype(BF16)

    hs, ys, gps = {}, {}, {}

    def moe_gate(j):
        gps[j] = _rb(_dot(xs, wg_v[:, j * E:(j + 1) * E]))

    def moe_up(j):
        up = _rb(_dot(xs, wu_v[:, j * E:(j + 1) * E]))
        gp = gps.pop(j)
        g = _rb(gp * (1.0 / (1.0 + jnp.exp(-gp))))
        hs[j] = (g * up).astype(BF16)

    def moe_down(kc, nq):
        hk = jnp.concatenate([hs[4 * kc + i] for i in range(4)], axis=1)
        d = _dot(hk, wd_v[kc * 256:(kc + 1) * 256, nq * 256:(nq + 1) * 256])
        ys[nq] = d + ys[nq] if nq in ys else d

    def moe_apply():
        y = _rb(jnp.concatenate([ys[nq] for nq in range(4)], axis=1))
        upd = [_rb(y[n:n + 1, :] * _rb(1.0 / (1.0 + jnp.exp(-mv)))) for n, mv in enumerate((m1, m2))]
        for n in range(2):
            blk = x_v[pl.ds(grp[n], 8), :].astype(F32)
            for k in range(2):
                blk = blk + jnp.where(row8 + grp[n] == sel[k], upd[k], 0.0)
            fix_v[n] = blk.astype(BF16)
        for n in range(2):
            g = pl.multiple_of(jnp.maximum(grp[n], S - MOE_LATE), 8)
            x_v[pl.ds(g, 8), :] = (x_v[pl.ds(g, 8), :].astype(F32)
                                   + jnp.where(row8 + g == sel[n], upd[n], 0.0)).astype(BF16)

    waves = []
    for j in range(FF // E):
        waves += [functools.partial(moe_gate, j), functools.partial(moe_up, j)]
    for kc in range(FF // 512):
        waves += [functools.partial(moe_down, kc, nq) for nq in range(4)]
    waves = [None] * opt('mlead', 10) + waves + [None] * opt('mgap', 1) + [moe_apply]
    NM = opt('nm', 6)
    MOE_LATE = EPI

    def finish(rs, cs, acc):
        x_v[rs, cs] = (x_v[rs, cs].astype(F32) + xn_v[rs, cs].astype(F32) + acc).astype(BF16)

    with scope('epi0'):
        for blk in range(EPI // 128):
            ar = OEPI + blk * 128
            r0 = S - EPI + blk * 128
            for n in range(NM):
                acc = None
                for kc in range(NOC):
                    d = _dot(o_ld(kc, slice(ar, ar + 128)),
                             wo_v[kc * KC // 2:(kc + 1) * KC // 2, n * E:(n + 1) * E])
                    acc = d if acc is None else d + acc
                    if kc == NOC - 1:
                        finish(slice(r0, r0 + 128), slice(n * E, (n + 1) * E), acc)
                    if waves:
                        wv = waves.pop(0)
                        if wv is not None:
                            wv()
        for wv in waves:
            if wv is not None:
                wv()

    fixes = [pltpu.make_async_copy(fix_v.at[n], out_hbm.at[pl.ds(grp[n], 8)], sem_o.at[3 + n])
             for n in range(2)]
    need = [sel[0] < S - EPI, jnp.logical_and(sel[1] < S - EPI, grp[1] != grp[0])]
    out_copy(0, S - EPI, 0).wait()
    for n in range(2):
        @pl.when(need[n])
        def _():
            fixes[n].start()

    def epi(blk, carry):
        ar = pl.ds(pl.multiple_of(OEPI + blk * 128, 16), 128)
        a = jnp.concatenate([o_ld(c, ar) for c in range(NOC)], axis=1)
        r0 = pl.multiple_of(S - EPI + blk * 128, 128)
        finish(pl.ds(r0, 128), slice(NM * E, D), _dot(a, wo_v[0:NP * WOP, NM * E:]))
        out_copy(r0, 128, 1 + blk).start()
        return carry

    with scope('epi'):
        lax.fori_loop(0, EPI // 128, epi, 0)

    with scope('fin'):
        for n in range(2):
            @pl.when(need[n])
            def _():
                fixes[n].wait()
        for blk in range(EPI // 128):
            out_copy(S - EPI + blk * 128, 128, 1 + blk).wait()


@jax.jit
def pallas_parallel_sum__memory_aug_recurrent_mem_tr__moe_arch_mod__prompt_kernel(
    A_x: jax.Array,
    A_mem0: jax.Array,
    A_Wq: jax.Array,
    A_Wk: jax.Array,
    A_Wv: jax.Array,
    A_Wo: jax.Array,
    A_seg_len: jax.Array,
    B_x: jax.Array,
    B_w_r: jax.Array,
    B_w_gate: jax.Array,
    B_w_up: jax.Array,
    B_w_down: jax.Array,
):
    del A_seg_len, B_x
    assert A_x.shape == (1, S, D) and A_Wq.shape == (D, H, E) and A_mem0.shape == (1, M, D)
    wshape = (D // 2, 2, NP, 2, E)
    any_spec = pl.BlockSpec(memory_space=pl.ANY)
    out = pl.pallas_call(
        _kernel,
        out_shape=jax.ShapeDtypeStruct((S, D), BF16),
        in_specs=[any_spec] * 10,
        out_specs=any_spec,
        scratch_shapes=[
            pltpu.VMEM((S + 2 * XBR, D), BF16),
            pltpu.VMEM((S, D), BF16),
            pltpu.VMEM((PRE // 2, D), U32) if opt('xpn', 1) else pltpu.VMEM((PRE, D), BF16),
            pltpu.VMEM((M, D), BF16),
            pltpu.VMEM((NCH + 1, D // 2, 2 * E), U32),
            pltpu.VMEM(((NP + 2) * WOP, D), U32),
            pltpu.VMEM((NST + 1, 3, 2, D // 2, E), U32),
            pltpu.VMEM((D // 2, 2 * E), U32),
            pltpu.VMEM((D // 2, 2 * E), U32),
            pltpu.VMEM((D // 2, 2 * E), U32),
            pltpu.VMEM((D // 2, FF), U32),
            pltpu.VMEM((D // 2, FF), U32),
            pltpu.VMEM((FF // 2, D), U32),
            pltpu.VMEM((8, D), F32),
            pltpu.VMEM((2, 8, D), BF16),
            pltpu.SemaphoreType.DMA((2,)),
            pltpu.SemaphoreType.DMA((2,)),
            pltpu.SemaphoreType.DMA((2,)),
            pltpu.SemaphoreType.DMA((NST + 2,)),
            pltpu.SemaphoreType.DMA((2,)),
            pltpu.SemaphoreType.DMA((3,)),
            pltpu.SemaphoreType.DMA((5,)),
            *([pltpu.VMEM((NS, NPR + RPAD, L2, E), BF16)] * (3 * RP) if RSPLIT
              else [pltpu.VMEM((NS, 3, NPR + RPAD, L2, E), BF16)] * RP),
            *[pltpu.VMEM((OEPI + EPI, n * KC), BF16) for n in OGR],
            pltpu.VMEM((L2, L2), F32),
            pltpu.VMEM((D // E, E), BF16),
        ],
        compiler_params=pltpu.CompilerParams(vmem_limit_bytes=120 * 1024 * 1024,
                                             disable_bounds_checks=True),
    )(
        A_x.reshape(S, D),
        A_mem0.reshape(M, D),
        A_Wq.reshape(wshape),
        A_Wk.reshape(wshape),
        A_Wv.reshape(wshape),
        A_Wo.reshape(H * E, D),
        B_w_r.reshape(D // E, E),
        B_w_gate,
        B_w_up,
        B_w_down,
    )
    return out.reshape(1, S, D)
```

```python
import functools
import os

import jax
import jax.numpy as jnp
from jax import lax
import jax.experimental.pallas as pl
import jax.experimental.pallas.tpu as pltpu

OPT = dict(kv.split('=') for kv in os.environ.get('KOPT', '').split(',') if kv)


def opt(k, d):
    return int(OPT.get(k, d))


class _NoScope:
    def __enter__(self):
        return self

    def __exit__(self, *a):
        return False


def scope(name):
    return jax.named_scope(name) if opt('scopes', 0) else _NoScope()


F32 = jnp.float32
BF16 = jnp.bfloat16
U32 = jnp.uint32

S = 2048
D = 1024
H = 32
E = 128
M = 8
SEG = 32
NSEG = S // SEG
FF = 3584
NP = H // 2
L1 = M + SEG
L2 = 2 * L1

PRE = 512
TPS = 24
NS = 17
U = 4
WG = tuple(int(c) for c in OPT.get('wg', '3353'))
WGS = tuple(sum(WG[:u]) for u in range(U))
GPI = sum(WG)
REC = (GPI + U) * 8
NREC = 4
EPI = S - (NSEG // U) * GPI * 8
OEPI = NREC * REC
NST = 4
NCH = 3 * NP
NOC = 8
KC = H * E // NOC
PPC = NP // NOC
OGR = [int(c) for c in OPT.get('ogr', '11111111')]
OMAP = [(a, k) for a, n in enumerate(OGR) for k in range(n)]
RSPLIT = opt('rsplit', 1)
RP = opt('rp', 1)
NPR = NP // RP + (RP > 1)
RPAD = (-NPR) % 4
XA = PRE // 2
XBR = (S - PRE) // NP
WOP = (H * E // 2) // NP
KS = D // 2

EPS = 1e-05
SCALE = float(E) ** -0.5
LOG2E = 1.4426950408889634


def _mod17(x):
    return x - 17 * ((x * 241) >> 12)


def _div14(x):
    return (x * 293) >> 12


assert NS == 17 and SEG == 32 and GPI == 14
assert all(_mod17(x) == x % 17 for x in range(128))
assert all(_div14(x) == x // 14 for x in range(256))


def _rb(v):
    return v.astype(BF16).astype(F32)


def _recip(v):
    y = pl.reciprocal(v, approx=True)
    return y * (2.0 - v * y)


def _layernorm_rows(xb, wr8):
    xf = xb.astype(F32)
    mean = jnp.sum(xf, axis=-1, keepdims=True) * (1.0 / D)
    mb = _rb(mean)
    d = xf - mb
    dm = mean - mb
    var = jnp.maximum(jnp.sum(d * d, axis=-1, keepdims=True) * (1.0 / D) - dm * dm, 0.0)
    ve = _rb(_rb(var) + EPS)
    if opt('lnq', 1):
        inv = _recip(_rb(ve * lax.rsqrt(ve)))
    else:
        inv = 1.0 / _rb(jnp.sqrt(ve))
    xw = d * inv
    wr = jnp.concatenate([wr8] * (xb.shape[0] // 8), axis=0)
    r = _rb(jnp.sum(xw * wr, axis=-1, keepdims=True))
    return xw, r


def _scatter_scores(acc, r, g0):
    lane = lax.broadcasted_iota(jnp.int32, acc.shape, 1)
    for j in range(r.shape[0] // 8):
        acc = jnp.where(lane == g0 + j, r[j * 8:(j + 1) * 8, :], acc)
    return acc


def _dot(a, w32):
    return jnp.dot(a, pltpu.bitcast(w32, BF16), preferred_element_type=F32)


def _kernel(x_hbm, mem0_hbm, wq_hbm, wk_hbm, wv_hbm, wo_hbm, wr_hbm, wg_hbm, wu_hbm, wd_hbm,
            out_hbm,
            x_v, xn_v, xp_v, mem0_v, wqkv, wo_v, stage, wc0, wc1, wc2, wg_v, wu_v, wd_v,
            wr_v, fix_v,
            sem_xa, sem_xb, sem_s, sem_st, sem_wo, sem_w, sem_o, *rest):
    w32 = [w.bitcast(U32) for w in (wq_hbm, wk_hbm, wv_hbm)]
    wo32 = wo_hbm.bitcast(U32)
    wcur = (wc0, wc1, wc2)
    nring = (3 if RSPLIT else 1) * RP
    rings, o_vs = rest[:nring], rest[nring:-2]
    fill_v, wr_in = rest[-2:]

    class _Ring:
        def _ix(self, ix, c, pi):
            if RSPLIT:
                return rings[ix[1] * RP + c], (ix[0], pi) + ix[3:]
            return rings[c], (ix[0], ix[1], pi) + ix[3:]

        def __getitem__(self, ix):
            ref, j = self._ix(ix, ix[2] % RP, ix[2] // RP)
            return ref[j]

        def __setitem__(self, ix, v):
            p = ix[2]
            if isinstance(p, int):
                ref, j = self._ix(ix, p % RP, p // RP)
                ref[j] = v
            else:
                for c in range(RP):
                    pi = p if RP == 1 else jnp.where((p & (RP - 1)) == c, p >> (RP // 2), NP // RP)
                    ref, j = self._ix(ix, c, pi)
                    ref[j] = v

    ring = _Ring()

    def o_ld(c, rows):
        oa, ok = OMAP[c]
        return o_vs[oa][rows, ok * KC:(ok + 1) * KC]

    def xa_copy(c):
        n = XA if c == 0 else PRE + TPS - XA
        return pltpu.make_async_copy(x_hbm.at[pl.ds(c * XA, n)], x_v.at[pl.ds(c * XA, n)],
                                     sem_xa.at[c])

    def xb_copy(i):
        src = pl.multiple_of(PRE + jnp.minimum(i, NP - 1) * XBR, 32)
        dst = pl.multiple_of(PRE + i * XBR, 32)
        return pltpu.make_async_copy(x_hbm.at[pl.ds(src, XBR)], x_v.at[pl.ds(dst, XBR)],
                                     sem_xb.at[i >> 4])

    def st_copy(t, p, slot, k, dp, sem):
        return pltpu.make_async_copy(w32[t].at[:, dp, p, 0, :], stage.at[slot, k, dp], sem)

    def grp_start(g, sems=None):
        slot = g & (NST - 1)
        for k, (t, p) in enumerate(((1, g), (2, g), (0, g + 1))):
            p = jnp.minimum(p, NP - 1)
            for dp in range(2):
                st_copy(t, p, slot, k, dp, sem_st.at[slot] if sems is None else sems[k]).start()

    def st_wait(view, sem):
        pltpu.make_async_copy(view, view, sem).wait()

    def grp_wait(g):
        slot = g & (NST - 1)
        st_wait(stage.at[slot], sem_st.at[slot])

    def wo_copy(i):
        src = pl.multiple_of(jnp.minimum(i, NP - 1) * WOP, 8)
        dst = pl.multiple_of(i * WOP, 8)
        return pltpu.make_async_copy(wo32.at[pl.ds(src, WOP)], wo_v.at[pl.ds(dst, WOP)],
                                     sem_wo.at[i >> 4])

    mem0_copy = pltpu.make_async_copy(mem0_hbm, mem0_v, sem_s.at[0])
    wr_copy = pltpu.make_async_copy(wr_hbm, wr_in, sem_s.at[1])
    first_copies = [st_copy(0, 0, NST, 0, dp, sem_st.at[NST]) for dp in range(2)]
    moe_copies = [pltpu.make_async_copy(src.bitcast(U32), dst, sem_w.at[k])
                  for k, (src, dst) in enumerate(((wg_hbm, wg_v), (wu_hbm, wu_v), (wd_hbm, wd_v)))]

    xa_copy(0).start()
    wr_copy.start()
    for cp in first_copies:
        cp.start()
    xa_copy(1).start()

    row = lax.broadcasted_iota(jnp.int32, (L2, L2), 0)
    col = lax.broadcasted_iota(jnp.int32, (L2, L2), 1)
    rl = jnp.where(row >= L1, row - L1, row)
    cl = jnp.where(col >= L1, col - L1, col)
    same = (row >= L1) == (col >= L1)
    keep = (rl < M) | (rl >= cl)
    fill_v[...] = jnp.where(same, jnp.where(keep, 0.0, -1000000000.0 / (SCALE if opt('sm', 2) == 2 else 1.0)), -jnp.inf).astype(F32)

    def ln_rows(r0, n, racc):
        LR = opt('lnr', 32)
        for j in range(n // LR):
            r = r0 + j * LR
            rs = pl.ds(r if isinstance(r, int) else pl.multiple_of(r, LR), LR)
            xw, sc = _layernorm_rows(x_v[rs, :], wr_v[...])
            r2 = r // 2 if isinstance(r, int) else pl.multiple_of(r >> 1, LR // 2)
            xn_v[rs, :] = xw.astype(BF16)
            xp_v[pl.ds(r2, LR // 2), :] = pltpu.bitcast(xn_v[rs, :], U32)
            racc = _scatter_scores(racc, sc, r // 8 if isinstance(r, int) else r >> 3)
        return racc

    def ln_step(i, racc):
        ic = jnp.minimum(i, NSEG - 1)
        r0 = pl.multiple_of(PRE + ic * TPS, 8)
        xw, r = _layernorm_rows(x_v[pl.ds(r0, TPS), :], wr_v[...])
        xn_v[pl.ds(r0, TPS), :] = xw.astype(BF16)
        return _scatter_scores(racc, r, PRE // 8 + ic * (TPS // 8))

    with scope('ln0'):
        wr_copy.wait()
        wrf = wr_in[...].astype(F32)
        wr_v[...] = jnp.broadcast_to(
            jnp.concatenate([wrf[k:k + 1, :] for k in range(D // E)], axis=1), (8, D))
        xa_copy(0).wait()
        grp_start(0, (sem_st.at[0], sem_st.at[0], sem_st.at[NST + 1]))
        LB = opt('lnb', 256)
        racc = jnp.zeros((8, S // 8), F32)
        if LB == XA:
            racc = ln_rows(0, XA, racc)
        else:
            racc = lax.fori_loop(0, XA // LB, lambda i, ra: ln_rows(i * LB, LB, ra), racc)

    def relayout(slot, k, c, dst):
        for j in range(D // 2 // 64):
            a = stage[slot, k, 0, j * 64:(j + 1) * 64, :]
            b = stage[slot, k, 1, j * 64:(j + 1) * 64, :]
            ev = (a & jnp.uint32(0xFFFF)) | (b << 16)
            od = (a >> 16) | (b & jnp.uint32(0xFFFF0000))
            dst[j * 64:(j + 1) * 64, 0:E] = ev
            dst[j * 64:(j + 1) * 64, E:2 * E] = od
            wqkv[c, j * 64:(j + 1) * 64, 0:E] = ev
            wqkv[c, j * 64:(j + 1) * 64, E:2 * E] = od

    MB = opt('promb', 256)

    def pro_dots(t, p):
        for rb in range(PRE // MB):
            if opt('xpn', 1):
                a = pltpu.bitcast(xp_v[rb * MB // 2:(rb + 1) * MB // 2, :], BF16)
            else:
                a = xp_v[rb * MB:(rb + 1) * MB, :]
            y = _dot(a, wcur[t][...]).astype(BF16)
            for sg in range(MB // SEG):
                for hh in range(2):
                    ring[rb * (MB // SEG) + sg, t, p, hh * L1 + M:(hh + 1) * L1, :] = (
                        y[sg * SEG:(sg + 1) * SEG, hh * E:(hh + 1) * E])

    with scope('blkB'):
        st_wait(stage.at[NST, 0], sem_st.at[NST])
        xa_copy(1).wait()
        mem0_copy.start()
        grp_start(1)
        relayout(NST, 0, 0, wc0)
        racc = ln_rows(XA, PRE - XA, racc)
        pro_dots(0, 0)
        racc = ln_step(0, racc)
    with scope('blkC'):
        st_wait(stage.at[0, pl.ds(0, 2)], sem_st.at[0])
        grp_start(2)
        relayout(0, 0, 1, wc1)
        relayout(0, 1, 2, wc2)
        pro_dots(1, 0)
    with scope('blkD'):
        st_wait(stage.at[0, 2], sem_st.at[NST + 1])
        for i in range(3):
            wo_copy(i).start()
            xb_copy(i).start()
        relayout(0, 2, 3, wc0)
        pro_dots(2, 0)

    def pro(p, carry):
        grp_wait(p)
        slot = p & (NST - 1)
        for t in range(3):
            relayout(slot, t, 3 * p + t + 1, wcur[(t + 1) % 3])
            pro_dots(t, p)

        grp_start(p + 2)
        wo_copy(p + 2).start()
        xb_copy(p + 2).start()
        return carry

    with scope('pro'):
        lax.fori_loop(1, NP, pro, 0)

    st_wait(x_v.at[pl.ds(PRE, S - PRE)], sem_xb.at[0])
    mem0_copy.wait()
    st_wait(wo_v.at[pl.ds(0, NP * WOP)], sem_wo.at[0])

    def step(it, u, carry):
        racc, mem = carry
        s = it * U + u
        slot = _mod17(s)
        t0 = pl.multiple_of(PRE + s * TPS, 8)
        top = xn_v[pl.ds(t0, 8), :].astype(F32)
        bot = xn_v[pl.ds(t0 + 8, 16), :]
        lhs = jnp.concatenate([jnp.concatenate([mem, top], axis=0).astype(BF16), bot], axis=0)
        part = [_dot(lhs[:, :KS], wqkv[t, 0:KS // 2, :]) for t in range(3)]
        qdst = []
        for j in range(TPS // 8):
            tj = t0 + 8 * j
            qdst.append((_mod17(tj >> 5), M + (tj & (SEG - 1))))
        odst = []
        for j in range(SEG // 8):
            g = (SEG // 8) * s + j
            gi = _div14(g)
            gr = g - GPI * gi
            r_ring = (gi & (NREC - 1)) * REC + (gr + 1 + sum((gr >= WGS[k]).astype(jnp.int32) for k in range(1, U))) * 8
            r_epi = OEPI + (g - (S - EPI) // 8) * 8
            odst.append(pl.multiple_of(jnp.where(g < (S - EPI) // 8, r_ring, r_epi), 8))
        orow = pl.multiple_of((it & (NREC - 1)) * REC + (WGS[u] + u) * 8, 16)
        nw = WG[u] * 8
        if opt('fake', 0) & 1:
            slot = u
            qdst = [(4 + u, 8 + 8 * j) for j in range(3)]
        if opt('fake', 0) & 2:
            odst = [REC + 8 + 8 * j + 40 * u for j in range(4)]
        if opt('fake', 0) & 4:
            orow = (WGS[u] + u) * 8

        def qkv(p, t):
            if p == 0:
                y = _dot(lhs[:, KS:], wqkv[t, KS // 2:, :]) + part[t]
            elif opt('n128', 0):
                y = jnp.concatenate([_dot(lhs, wqkv[3 * p + t, :, hh * E:(hh + 1) * E])
                                     for hh in range(2)], axis=1)
            else:
                y = _dot(lhs, wqkv[3 * p + t])
            y = y.astype(BF16)
            for hh in range(2):
                yc = y[:, hh * E:(hh + 1) * E]
                ring[slot, t, p, hh * L1:hh * L1 + M, :] = yc[0:M]
                for j in range(TPS // 8):
                    qs, qr = qdst[j]
                    ring[qs, t, p, pl.ds(hh * L1 + qr if isinstance(qr, int) else pl.multiple_of(hh * L1 + qr, 8), 8), :] = (
                        yc[M + 8 * j:M + 8 * j + 8])

        def attn_a(q, k):
            sc = lax.dot_general(q, k, (((1,), (1,)), ((), ())), preferred_element_type=F32)
            fill = fill_v[...]
            if opt('sm', 2) == 0:
                sc = jnp.where(fill == 0.0, sc * SCALE, fill)
                e = jnp.exp(sc - jnp.max(sc, axis=-1, keepdims=True))
            elif opt('sm', 2) == 1:
                sc = jnp.where(fill == 0.0, sc * (SCALE * LOG2E), fill * LOG2E)
                e = jnp.exp2(sc - jnp.max(sc, axis=-1, keepdims=True))
            else:
                sc = jnp.where(fill == 0.0, sc, fill)
                e = jnp.exp2((sc - jnp.max(sc, axis=-1, keepdims=True)) * (SCALE * LOG2E))
            den = jnp.sum(e, axis=-1, keepdims=True)
            return (e * pl.reciprocal(den, approx=True)).astype(BF16)

        def attn_b(p, pr, v):
            o = jnp.dot(pr, v, preferred_element_type=F32).astype(BF16)
            oa, ok = OMAP[p // PPC]
            oc = o_vs[oa]
            for hh in range(2):
                cs = ok * KC + (2 * (p % PPC) + hh) * E
                oc[pl.ds(orow, M), cs:cs + E] = o[hh * L1:hh * L1 + M]
                for j in range(SEG // 8):
                    r = hh * L1 + M + 8 * j
                    oc[pl.ds(odst[j], 8), cs:cs + E] = o[r:r + 8]

        def wo_chunk(c, c1):
            a = jnp.concatenate([o_ld(i, pl.ds(orow, M + nw)) for i in range(c, c1)], axis=1)
            return _dot(a, wo_v[c * KC // 2:c1 * KC // 2, :])

        wl = OPT.get('wl', '0.1.2.3.4.5.6-7').split('.')
        nslot = 3 * NP + len(wl)
        ev = {n: [] for n in range(nslot + 1)}
        lq, aa, lv, bb = opt('lq', 2), opt('a', 4), opt('lv', 6), opt('b', 8)
        ta = [int(x) for x in OPT.get('ta', '50').split('.')]
        tb = [int(x) for x in OPT.get('tb', '50.53').split('.')]
        for p in range(NP):
            pa_ = 3 * p + aa if p < NP - len(ta) else ta[p - (NP - len(ta))]
            pb_ = 3 * p + bb if p < NP - len(tb) else tb[p - (NP - len(tb))]
            ql, vl = min(3 * p + lq, pa_), min(3 * p + lv, pb_)
            if 'ga' in OPT:
                G = opt('G', 4)
                pa_ = [int(x) for x in OPT['ga'].split('.')][p // G]
                pb_ = [int(x) for x in OPT['gb'].split('.')][p // G]
                ql = max(3 * p + 2, pa_ - opt('gl', 2))
                vl = max(3 * p + 3, pb_ - opt('gl', 2))
            assert pa_ <= pb_ <= nslot
            ev[ql].append((0, 'Q', p))
            ev[vl].append((1, 'V', p))
            ev[pa_].append((3, 'A', p))
            ev[pb_].append((2, 'B', p))
        pe, qk, vv = {}, {}, {}
        acc = None
        r0 = pl.multiple_of((it * GPI + WGS[u]) * 8, 8)
        for n in range(nslot + 1):
            for _, kind, p in sorted(ev[n]):
                if kind == 'Q':
                    qk[p] = (ring[slot, 0, p], ring[slot, 1, p])
                elif kind == 'V':
                    vv[p] = ring[slot, 2, p]
                elif kind == 'A':
                    pe[p] = attn_a(*qk.pop(p))
                else:
                    attn_b(p, pe.pop(p), vv.pop(p))
            if n == opt('lnpos', 99):
                base = x_v[pl.ds(r0, nw), :].astype(F32) + xn_v[pl.ds(r0, nw), :].astype(F32)
                racc = ln_step(s + 1, racc)
            if n < 3 * NP:
                qkv(n // 3, [int(c) for c in OPT.get('mo', '012')][n % 3])
            elif n < nslot:
                tk = wl[n - 3 * NP].split('-')
                y = wo_chunk(int(tk[0]), int(tk[-1]) + 1)
                acc = y if acc is None else y + acc
        if opt('lnpos', 99) > nslot:
            base = x_v[pl.ds(r0, nw), :].astype(F32) + xn_v[pl.ds(r0, nw), :].astype(F32)
        if opt('lnpos', 99) > nslot:
            racc = ln_step(s + 1, racc)
        x_v[pl.ds(r0, nw), :] = (base + acc[M:]).astype(BF16)
        return racc, acc[0:M]

    def steps(it, carry):
        def start_moe(_, c):
            for cp in moe_copies:
                cp.start()
            return c

        lax.fori_loop(0, (it == 1).astype(jnp.int32), start_moe, 0)

        with scope('it'):
            for u in range(U):
                carry = step(it, u, carry)
        return carry

    with scope('main'):
        racc, _ = lax.fori_loop(0, NSEG // U, steps, (racc, mem0_v[...].astype(F32)))

    def out_copy(r0, n, k):
        return pltpu.make_async_copy(x_v.at[pl.ds(r0, n)], out_hbm.at[pl.ds(r0, n)], sem_o.at[k])

    for cp in moe_copies:
        cp.wait()
    grp_wait(NP)
    grp_wait(NP + 1)
    st_wait(x_v.at[pl.ds(S, 2 * XBR)], sem_xb.at[1])
    st_wait(wo_v.at[pl.ds(NP * WOP, 2 * WOP)], sem_wo.at[1])
    out_copy(0, S - EPI, 0).start()

    idx = (lax.broadcasted_iota(jnp.int32, racc.shape, 1) * 8
           + lax.broadcasted_iota(jnp.int32, racc.shape, 0)).astype(F32)

    def allred(fn, v):
        return fn(fn(v, axis=1, keepdims=True), axis=0, keepdims=True)

    m1 = allred(jnp.max, racc)
    i1 = allred(jnp.min, jnp.where(racc == m1, idx, float(S - 1)))
    r2 = jnp.where(idx == i1, -jnp.inf, racc)
    m2 = allred(jnp.max, r2)
    i2 = allred(jnp.min, jnp.where((r2 == m2) & (idx != i1), idx, float(S - 1)))
    sel = [jnp.clip(jnp.max(iv).astype(jnp.int32), 0, S - 1) for iv in (i1, i2)]
    grp = [pl.multiple_of((i >> 3) << 3, 8) for i in sel]
    row8 = lax.broadcasted_iota(jnp.int32, (8, D), 0)
    rows = [jnp.sum(jnp.where(row8 == (i & 7), xn_v[pl.ds(g, 8), :].astype(F32), 0.0),
                    axis=0, keepdims=True) for i, g in zip(sel, grp)]
    row16 = lax.broadcasted_iota(jnp.int32, (16, D), 0)
    xs = jnp.where(row16 == 0, rows[0], jnp.where(row16 == 1, rows[1], 0.0)).astype(BF16)

    hs, ys, gps = {}, {}, {}

    def moe_gate(j):
        gps[j] = _rb(_dot(xs, wg_v[:, j * E:(j + 1) * E]))

    def moe_up(j):
        up = _rb(_dot(xs, wu_v[:, j * E:(j + 1) * E]))
        gp = gps.pop(j)
        g = _rb(gp * (1.0 / (1.0 + jnp.exp(-gp))))
        hs[j] = (g * up).astype(BF16)

    def moe_down(kc, nq):
        hk = jnp.concatenate([hs[4 * kc + i] for i in range(4)], axis=1)
        d = _dot(hk, wd_v[kc * 256:(kc + 1) * 256, nq * 256:(nq + 1) * 256])
        ys[nq] = d + ys[nq] if nq in ys else d

    def moe_apply():
        y = _rb(jnp.concatenate([ys[nq] for nq in range(4)], axis=1))
        upd = [_rb(y[n:n + 1, :] * _rb(1.0 / (1.0 + jnp.exp(-mv)))) for n, mv in enumerate((m1, m2))]
        for n in range(2):
            blk = x_v[pl.ds(grp[n], 8), :].astype(F32)
            for k in range(2):
                blk = blk + jnp.where(row8 + grp[n] == sel[k], upd[k], 0.0)
            fix_v[n] = blk.astype(BF16)
        for n in range(2):
            g = pl.multiple_of(jnp.maximum(grp[n], S - MOE_LATE), 8)
            x_v[pl.ds(g, 8), :] = (x_v[pl.ds(g, 8), :].astype(F32)
                                   + jnp.where(row8 + g == sel[n], upd[n], 0.0)).astype(BF16)

    waves = []
    for j in range(FF // E):
        waves += [functools.partial(moe_gate, j), functools.partial(moe_up, j)]
    for kc in range(FF // 512):
        waves += [functools.partial(moe_down, kc, nq) for nq in range(4)]
    waves = [None] * opt('mlead', 10) + waves + [None] * opt('mgap', 1) + [moe_apply]
    NM = opt('nm', 6)
    MOE_LATE = EPI

    def finish(rs, cs, acc):
        x_v[rs, cs] = (x_v[rs, cs].astype(F32) + xn_v[rs, cs].astype(F32) + acc).astype(BF16)

    with scope('epi0'):
        for blk in range(EPI // 128):
            ar = OEPI + blk * 128
            r0 = S - EPI + blk * 128
            for n in range(NM):
                acc = None
                for kc in range(NOC):
                    d = _dot(o_ld(kc, slice(ar, ar + 128)),
                             wo_v[kc * KC // 2:(kc + 1) * KC // 2, n * E:(n + 1) * E])
                    acc = d if acc is None else d + acc
                    if kc == NOC - 1:
                        finish(slice(r0, r0 + 128), slice(n * E, (n + 1) * E), acc)
                    if waves:
                        wv = waves.pop(0)
                        if wv is not None:
                            wv()
        for wv in waves:
            if wv is not None:
                wv()

    fixes = [pltpu.make_async_copy(fix_v.at[n], out_hbm.at[pl.ds(grp[n], 8)], sem_o.at[3 + n])
             for n in range(2)]
    need = [sel[0] < S - EPI, jnp.logical_and(sel[1] < S - EPI, grp[1] != grp[0])]
    out_copy(0, S - EPI, 0).wait()
    for n in range(2):
        @pl.when(need[n])
        def _():
            fixes[n].start()

    def epi(blk, carry):
        ar = pl.ds(pl.multiple_of(OEPI + blk * 128, 16), 128)
        a = jnp.concatenate([o_ld(c, ar) for c in range(NOC)], axis=1)
        r0 = pl.multiple_of(S - EPI + blk * 128, 128)
        finish(pl.ds(r0, 128), slice(NM * E, D), _dot(a, wo_v[0:NP * WOP, NM * E:]))
        out_copy(r0, 128, 1 + blk).start()
        return carry

    with scope('epi'):
        lax.fori_loop(0, EPI // 128, epi, 0)

    with scope('fin'):
        for n in range(2):
            @pl.when(need[n])
            def _():
                fixes[n].wait()
        for blk in range(EPI // 128):
            out_copy(S - EPI + blk * 128, 128, 1 + blk).wait()


@jax.jit
def pallas_parallel_sum__memory_aug_recurrent_mem_tr__moe_arch_mod__prompt_kernel(
    A_x: jax.Array,
    A_mem0: jax.Array,
    A_Wq: jax.Array,
    A_Wk: jax.Array,
    A_Wv: jax.Array,
    A_Wo: jax.Array,
    A_seg_len: jax.Array,
    B_x: jax.Array,
    B_w_r: jax.Array,
    B_w_gate: jax.Array,
    B_w_up: jax.Array,
    B_w_down: jax.Array,
):
    del A_seg_len, B_x
    assert A_x.shape == (1, S, D) and A_Wq.shape == (D, H, E) and A_mem0.shape == (1, M, D)
    wshape = (D // 2, 2, NP, 2, E)
    any_spec = pl.BlockSpec(memory_space=pl.ANY)
    out = pl.pallas_call(
        _kernel,
        out_shape=jax.ShapeDtypeStruct((S, D), BF16),
        in_specs=[any_spec] * 10,
        out_specs=any_spec,
        scratch_shapes=[
            pltpu.VMEM((S + 2 * XBR, D), BF16),
            pltpu.VMEM((S, D), BF16),
            pltpu.VMEM((PRE // 2, D), U32) if opt('xpn', 1) else pltpu.VMEM((PRE, D), BF16),
            pltpu.VMEM((M, D), BF16),
            pltpu.VMEM((NCH + 1, D // 2, 2 * E), U32),
            pltpu.VMEM(((NP + 2) * WOP, D), U32),
            pltpu.VMEM((NST + 1, 3, 2, D // 2, E), U32),
            pltpu.VMEM((D // 2, 2 * E), U32),
            pltpu.VMEM((D // 2, 2 * E), U32),
            pltpu.VMEM((D // 2, 2 * E), U32),
            pltpu.VMEM((D // 2, FF), U32),
            pltpu.VMEM((D // 2, FF), U32),
            pltpu.VMEM((FF // 2, D), U32),
            pltpu.VMEM((8, D), F32),
            pltpu.VMEM((2, 8, D), BF16),
            pltpu.SemaphoreType.DMA((2,)),
            pltpu.SemaphoreType.DMA((2,)),
            pltpu.SemaphoreType.DMA((2,)),
            pltpu.SemaphoreType.DMA((NST + 2,)),
            pltpu.SemaphoreType.DMA((2,)),
            pltpu.SemaphoreType.DMA((3,)),
            pltpu.SemaphoreType.DMA((5,)),
            *([pltpu.VMEM((NS, NPR + RPAD, L2, E), BF16)] * (3 * RP) if RSPLIT
              else [pltpu.VMEM((NS, 3, NPR + RPAD, L2, E), BF16)] * RP),
            *[pltpu.VMEM((OEPI + EPI, n * KC), BF16) for n in OGR],
            pltpu.VMEM((L2, L2), F32),
            pltpu.VMEM((D // E, E), BF16),
        ],
        compiler_params=pltpu.CompilerParams(vmem_limit_bytes=120 * 1024 * 1024,
                                             disable_bounds_checks=True),
    )(
        A_x.reshape(S, D),
        A_mem0.reshape(M, D),
        A_Wq.reshape(wshape),
        A_Wk.reshape(wshape),
        A_Wv.reshape(wshape),
        A_Wo.reshape(H * E, D),
        B_w_r.reshape(D // E, E),
        B_w_gate,
        B_w_up,
        B_w_down,
    )
    return out.reshape(1, S, D)
```

```python
import functools
import os

import jax
import jax.numpy as jnp
from jax import lax
import jax.experimental.pallas as pl
import jax.experimental.pallas.tpu as pltpu

OPT = dict(kv.split('=') for kv in os.environ.get('KOPT', '').split(',') if kv)


def opt(k, d):
    return int(OPT.get(k, d))


class _NoScope:
    def __enter__(self):
        return self

    def __exit__(self, *a):
        return False


def scope(name):
    return jax.named_scope(name) if opt('scopes', 0) else _NoScope()


F32 = jnp.float32
BF16 = jnp.bfloat16
U32 = jnp.uint32

S = 2048
D = 1024
H = 32
E = 128
M = 8
SEG = 32
NSEG = S // SEG
FF = 3584
NP = H // 2
L1 = M + SEG
L2 = 2 * L1

PRE = 512
TPS = 24
NS = 17
U = 4
WG = tuple(int(c) for c in OPT.get('wg', '3353'))
WGS = tuple(sum(WG[:u]) for u in range(U))
GPI = sum(WG)
REC = (GPI + U) * 8
NREC = 4
EPI = S - (NSEG // U) * GPI * 8
OEPI = NREC * REC
NST = 4
NCH = 3 * NP
NOC = 8
KC = H * E // NOC
PPC = NP // NOC
OGR = [int(c) for c in OPT.get('ogr', '11111111')]
OMAP = [(a, k) for a, n in enumerate(OGR) for k in range(n)]
RSPLIT = opt('rsplit', 1)
RP = opt('rp', 1)
NPR = NP // RP + (RP > 1)
RPAD = (-NPR) % 4
XA = PRE // 2
XBR = (S - PRE) // NP
WOP = (H * E // 2) // NP
KS = D // 2

EPS = 1e-05
SCALE = float(E) ** -0.5
LOG2E = 1.4426950408889634


def _mod17(x):
    return x - 17 * ((x * 241) >> 12)


def _div14(x):
    return (x * 293) >> 12


assert NS == 17 and SEG == 32 and GPI == 14
assert all(_mod17(x) == x % 17 for x in range(128))
assert all(_div14(x) == x // 14 for x in range(256))


def _rb(v):
    return v.astype(BF16).astype(F32)


def _recip(v):
    y = pl.reciprocal(v, approx=True)
    return y * (2.0 - v * y)


def _layernorm_rows(xb, wr8):
    xf = xb.astype(F32)
    mean = jnp.sum(xf, axis=-1, keepdims=True) * (1.0 / D)
    mb = _rb(mean)
    d = xf - mb
    dm = mean - mb
    var = jnp.maximum(jnp.sum(d * d, axis=-1, keepdims=True) * (1.0 / D) - dm * dm, 0.0)
    ve = _rb(_rb(var) + EPS)
    if opt('lnq', 1):
        inv = _recip(_rb(ve * lax.rsqrt(ve)))
    else:
        inv = 1.0 / _rb(jnp.sqrt(ve))
    xw = d * inv
    wr = jnp.concatenate([wr8] * (xb.shape[0] // 8), axis=0)
    r = _rb(jnp.sum(xw * wr, axis=-1, keepdims=True))
    return xw, r


def _scatter_scores(acc, r, g0):
    lane = lax.broadcasted_iota(jnp.int32, acc.shape, 1)
    for j in range(r.shape[0] // 8):
        acc = jnp.where(lane == g0 + j, r[j * 8:(j + 1) * 8, :], acc)
    return acc


def _dot(a, w32):
    return jnp.dot(a, pltpu.bitcast(w32, BF16), preferred_element_type=F32)


def _kernel(x_hbm, mem0_hbm, wq_hbm, wk_hbm, wv_hbm, wo_hbm, wr_hbm, wg_hbm, wu_hbm, wd_hbm,
            out_hbm,
            x_v, xn_v, xp_v, mem0_v, wqkv, wo_v, stage, wc0, wc1, wc2, wg_v, wu_v, wd_v,
            wr_v, fix_v,
            sem_xa, sem_xb, sem_s, sem_st, sem_wo, sem_w, sem_o, *rest):
    w32 = [w.bitcast(U32) for w in (wq_hbm, wk_hbm, wv_hbm)]
    wo32 = wo_hbm.bitcast(U32)
    wcur = (wc0, wc1, wc2)
    nring = (3 if RSPLIT else 1) * RP
    rings, o_vs = rest[:nring], rest[nring:-2]
    fill_v, wr_in = rest[-2:]

    class _Ring:
        def _ix(self, ix, c, pi):
            if RSPLIT:
                return rings[ix[1] * RP + c], (ix[0], pi) + ix[3:]
            return rings[c], (ix[0], ix[1], pi) + ix[3:]

        def __getitem__(self, ix):
            ref, j = self._ix(ix, ix[2] % RP, ix[2] // RP)
            return ref[j]

        def __setitem__(self, ix, v):
            p = ix[2]
            if isinstance(p, int):
                ref, j = self._ix(ix, p % RP, p // RP)
                ref[j] = v
            else:
                for c in range(RP):
                    pi = p if RP == 1 else jnp.where((p & (RP - 1)) == c, p >> (RP // 2), NP // RP)
                    ref, j = self._ix(ix, c, pi)
                    ref[j] = v

    ring = _Ring()

    def o_ld(c, rows):
        oa, ok = OMAP[c]
        return o_vs[oa][rows, ok * KC:(ok + 1) * KC]

    def xa_copy(c):
        n = XA if c == 0 else PRE + TPS - XA
        return pltpu.make_async_copy(x_hbm.at[pl.ds(c * XA, n)], x_v.at[pl.ds(c * XA, n)],
                                     sem_xa.at[c])

    def xb_copy(i):
        src = pl.multiple_of(PRE + jnp.minimum(i, NP - 1) * XBR, 32)
        dst = pl.multiple_of(PRE + i * XBR, 32)
        return pltpu.make_async_copy(x_hbm.at[pl.ds(src, XBR)], x_v.at[pl.ds(dst, XBR)],
                                     sem_xb.at[i >> 4])

    def st_copy(t, p, slot, k, dp, sem):
        return pltpu.make_async_copy(w32[t].at[:, dp, p, 0, :], stage.at[slot, k, dp], sem)

    def grp_start(g, sems=None):
        slot = g & (NST - 1)
        for k, (t, p) in enumerate(((1, g), (2, g), (0, g + 1))):
            p = jnp.minimum(p, NP - 1)
            for dp in range(2):
                st_copy(t, p, slot, k, dp, sem_st.at[slot] if sems is None else sems[k]).start()

    def st_wait(view, sem):
        pltpu.make_async_copy(view, view, sem).wait()

    def grp_wait(g):
        slot = g & (NST - 1)
        st_wait(stage.at[slot], sem_st.at[slot])

    def wo_copy(i):
        src = pl.multiple_of(jnp.minimum(i, NP - 1) * WOP, 8)
        dst = pl.multiple_of(i * WOP, 8)
        return pltpu.make_async_copy(wo32.at[pl.ds(src, WOP)], wo_v.at[pl.ds(dst, WOP)],
                                     sem_wo.at[i >> 4])

    mem0_copy = pltpu.make_async_copy(mem0_hbm, mem0_v, sem_s.at[0])
    wr_copy = pltpu.make_async_copy(wr_hbm, wr_in, sem_s.at[1])
    first_copies = [st_copy(0, 0, NST, 0, dp, sem_st.at[NST]) for dp in range(2)]
    moe_copies = [pltpu.make_async_copy(src.bitcast(U32), dst, sem_w.at[k])
                  for k, (src, dst) in enumerate(((wg_hbm, wg_v), (wu_hbm, wu_v), (wd_hbm, wd_v)))]

    xa_copy(0).start()
    wr_copy.start()
    for cp in first_copies:
        cp.start()
    xa_copy(1).start()

    row = lax.broadcasted_iota(jnp.int32, (L2, L2), 0)
    col = lax.broadcasted_iota(jnp.int32, (L2, L2), 1)
    rl = jnp.where(row >= L1, row - L1, row)
    cl = jnp.where(col >= L1, col - L1, col)
    same = (row >= L1) == (col >= L1)
    keep = (rl < M) | (rl >= cl)
    fill_v[...] = jnp.where(same, jnp.where(keep, 0.0, -1000000000.0 / (SCALE if opt('sm', 2) == 2 else 1.0)), -jnp.inf).astype(F32)

    def ln_rows(r0, n, racc):
        LR = opt('lnr', 32)
        for j in range(n // LR):
            r = r0 + j * LR
            rs = pl.ds(r if isinstance(r, int) else pl.multiple_of(r, LR), LR)
            xw, sc = _layernorm_rows(x_v[rs, :], wr_v[...])
            r2 = r // 2 if isinstance(r, int) else pl.multiple_of(r >> 1, LR // 2)
            xn_v[rs, :] = xw.astype(BF16)
            xp_v[pl.ds(r2, LR // 2), :] = pltpu.bitcast(xn_v[rs, :], U32)
            racc = _scatter_scores(racc, sc, r // 8 if isinstance(r, int) else r >> 3)
        return racc

    def ln_step(i, racc):
        ic = jnp.minimum(i, NSEG - 1)
        r0 = pl.multiple_of(PRE + ic * TPS, 8)
        xw, r = _layernorm_rows(x_v[pl.ds(r0, TPS), :], wr_v[...])
        xn_v[pl.ds(r0, TPS), :] = xw.astype(BF16)
        return _scatter_scores(racc, r, PRE // 8 + ic * (TPS // 8))

    with scope('ln0'):
        wr_copy.wait()
        wrf = wr_in[...].astype(F32)
        wr_v[...] = jnp.broadcast_to(
            jnp.concatenate([wrf[k:k + 1, :] for k in range(D // E)], axis=1), (8, D))
        xa_copy(0).wait()
        grp_start(0, (sem_st.at[0], sem_st.at[0], sem_st.at[NST + 1]))
        LB = opt('lnb', 256)
        racc = jnp.zeros((8, S // 8), F32)
        if LB == XA:
            racc = ln_rows(0, XA, racc)
        else:
            racc = lax.fori_loop(0, XA // LB, lambda i, ra: ln_rows(i * LB, LB, ra), racc)

    def relayout(slot, k, c, dst):
        for j in range(D // 2 // 64):
            a = stage[slot, k, 0, j * 64:(j + 1) * 64, :]
            b = stage[slot, k, 1, j * 64:(j + 1) * 64, :]
            ev = (a & jnp.uint32(0xFFFF)) | (b << 16)
            od = (a >> 16) | (b & jnp.uint32(0xFFFF0000))
            dst[j * 64:(j + 1) * 64, 0:E] = ev
            dst[j * 64:(j + 1) * 64, E:2 * E] = od
            wqkv[c, j * 64:(j + 1) * 64, 0:E] = ev
            wqkv[c, j * 64:(j + 1) * 64, E:2 * E] = od

    MB = opt('promb', 256)

    def pro_dots(t, p):
        for rb in range(PRE // MB):
            if opt('xpn', 1):
                a = pltpu.bitcast(xp_v[rb * MB // 2:(rb + 1) * MB // 2, :], BF16)
            else:
                a = xp_v[rb * MB:(rb + 1) * MB, :]
            y = _dot(a, wcur[t][...]).astype(BF16)
            for sg in range(MB // SEG):
                for hh in range(2):
                    ring[rb * (MB // SEG) + sg, t, p, hh * L1 + M:(hh + 1) * L1, :] = (
                        y[sg * SEG:(sg + 1) * SEG, hh * E:(hh + 1) * E])

    with scope('blkB'):
        st_wait(stage.at[NST, 0], sem_st.at[NST])
        xa_copy(1).wait()
        mem0_copy.start()
        grp_start(1)
        relayout(NST, 0, 0, wc0)
        racc = ln_rows(XA, PRE - XA, racc)
        pro_dots(0, 0)
        racc = ln_step(0, racc)
    with scope('blkC'):
        st_wait(stage.at[0, pl.ds(0, 2)], sem_st.at[0])
        grp_start(2)
        relayout(0, 0, 1, wc1)
        relayout(0, 1, 2, wc2)
        pro_dots(1, 0)
    with scope('blkD'):
        st_wait(stage.at[0, 2], sem_st.at[NST + 1])
        for i in range(3):
            wo_copy(i).start()
            xb_copy(i).start()
        relayout(0, 2, 3, wc0)
        pro_dots(2, 0)

    def pro(p, carry):
        grp_wait(p)
        slot = p & (NST - 1)
        for t in range(3):
            relayout(slot, t, 3 * p + t + 1, wcur[(t + 1) % 3])
            pro_dots(t, p)

        grp_start(p + 2)
        wo_copy(p + 2).start()
        xb_copy(p + 2).start()
        return carry

    with scope('pro'):
        lax.fori_loop(1, NP, pro, 0)

    st_wait(x_v.at[pl.ds(PRE, S - PRE)], sem_xb.at[0])
    mem0_copy.wait()
    st_wait(wo_v.at[pl.ds(0, NP * WOP)], sem_wo.at[0])

    def step(it, u, carry):
        racc, mem = carry
        s = it * U + u
        slot = _mod17(s)
        t0 = pl.multiple_of(PRE + s * TPS, 8)
        top = xn_v[pl.ds(t0, 8), :].astype(F32)
        bot = xn_v[pl.ds(t0 + 8, 16), :]
        lhs = jnp.concatenate([jnp.concatenate([mem, top], axis=0).astype(BF16), bot], axis=0)
        part = [_dot(lhs[:, :KS], wqkv[t, 0:KS // 2, :]) for t in range(3)]
        qdst = []
        for j in range(TPS // 8):
            tj = t0 + 8 * j
            qdst.append((_mod17(tj >> 5), M + (tj & (SEG - 1))))
        odst = []
        for j in range(SEG // 8):
            g = (SEG // 8) * s + j
            gi = _div14(g)
            gr = g - GPI * gi
            r_ring = (gi & (NREC - 1)) * REC + (gr + 1 + sum((gr >= WGS[k]).astype(jnp.int32) for k in range(1, U))) * 8
            r_epi = OEPI + (g - (S - EPI) // 8) * 8
            odst.append(pl.multiple_of(jnp.where(g < (S - EPI) // 8, r_ring, r_epi), 8))
        orow = pl.multiple_of((it & (NREC - 1)) * REC + (WGS[u] + u) * 8, 16)
        nw = WG[u] * 8
        if opt('fake', 0) & 1:
            slot = u
            qdst = [(4 + u, 8 + 8 * j) for j in range(3)]
        if opt('fake', 0) & 2:
            odst = [REC + 8 + 8 * j + 40 * u for j in range(4)]
        if opt('fake', 0) & 4:
            orow = (WGS[u] + u) * 8

        def qkv(p, t):
            if p == 0:
                y = _dot(lhs[:, KS:], wqkv[t, KS // 2:, :]) + part[t]
            elif opt('n128', 0):
                y = jnp.concatenate([_dot(lhs, wqkv[3 * p + t, :, hh * E:(hh + 1) * E])
                                     for hh in range(2)], axis=1)
            else:
                y = _dot(lhs, wqkv[3 * p + t])
            y = y.astype(BF16)
            for hh in range(2):
                yc = y[:, hh * E:(hh + 1) * E]
                ring[slot, t, p, hh * L1:hh * L1 + M, :] = yc[0:M]
                for j in range(TPS // 8):
                    qs, qr = qdst[j]
                    ring[qs, t, p, pl.ds(hh * L1 + qr if isinstance(qr, int) else pl.multiple_of(hh * L1 + qr, 8), 8), :] = (
                        yc[M + 8 * j:M + 8 * j + 8])

        def attn_a(q, k):
            sc = lax.dot_general(q, k, (((1,), (1,)), ((), ())), preferred_element_type=F32)
            fill = fill_v[...]
            if opt('sm', 2) == 0:
                sc = jnp.where(fill == 0.0, sc * SCALE, fill)
                e = jnp.exp(sc - jnp.max(sc, axis=-1, keepdims=True))
            elif opt('sm', 2) == 1:
                sc = jnp.where(fill == 0.0, sc * (SCALE * LOG2E), fill * LOG2E)
                e = jnp.exp2(sc - jnp.max(sc, axis=-1, keepdims=True))
            else:
                sc = jnp.where(fill == 0.0, sc, fill)
                e = jnp.exp2((sc - jnp.max(sc, axis=-1, keepdims=True)) * (SCALE * LOG2E))
            den = jnp.sum(e, axis=-1, keepdims=True)
            return (e * pl.reciprocal(den, approx=True)).astype(BF16)

        def attn_b(p, pr, v):
            o = jnp.dot(pr, v, preferred_element_type=F32).astype(BF16)
            oa, ok = OMAP[p // PPC]
            oc = o_vs[oa]
            for hh in range(2):
                cs = ok * KC + (2 * (p % PPC) + hh) * E
                oc[pl.ds(orow, M), cs:cs + E] = o[hh * L1:hh * L1 + M]
                for j in range(SEG // 8):
                    r = hh * L1 + M + 8 * j
                    oc[pl.ds(odst[j], 8), cs:cs + E] = o[r:r + 8]

        def wo_chunk(c, c1):
            a = jnp.concatenate([o_ld(i, pl.ds(orow, M + nw)) for i in range(c, c1)], axis=1)
            return _dot(a, wo_v[c * KC // 2:c1 * KC // 2, :])

        wl = OPT.get('wl', '0.1.2.3.4.5.6-7').split('.')
        nslot = 3 * NP + len(wl)
        ev = {n: [] for n in range(nslot + 1)}
        lq, aa, lv, bb = opt('lq', 2), opt('a', 4), opt('lv', 6), opt('b', 8)
        ta = [int(x) for x in OPT.get('ta', '50').split('.')]
        tb = [int(x) for x in OPT.get('tb', '50.53').split('.')]
        for p in range(NP):
            pa_ = 3 * p + aa if p < NP - len(ta) else ta[p - (NP - len(ta))]
            pb_ = 3 * p + bb if p < NP - len(tb) else tb[p - (NP - len(tb))]
            ql, vl = min(3 * p + lq, pa_), min(3 * p + lv, pb_)
            if 'ga' in OPT:
                G = opt('G', 4)
                pa_ = [int(x) for x in OPT['ga'].split('.')][p // G]
                pb_ = [int(x) for x in OPT['gb'].split('.')][p // G]
                ql = max(3 * p + 2, pa_ - opt('gl', 2))
                vl = max(3 * p + 3, pb_ - opt('gl', 2))
            assert pa_ <= pb_ <= nslot
            ev[ql].append((0, 'Q', p))
            ev[vl].append((1, 'V', p))
            ev[pa_].append((3, 'A', p))
            ev[pb_].append((2, 'B', p))
        pe, qk, vv = {}, {}, {}
        acc = None
        r0 = pl.multiple_of((it * GPI + WGS[u]) * 8, 8)
        for n in range(nslot + 1):
            for _, kind, p in sorted(ev[n]):
                if kind == 'Q':
                    qk[p] = (ring[slot, 0, p], ring[slot, 1, p])
                elif kind == 'V':
                    vv[p] = ring[slot, 2, p]
                elif kind == 'A':
                    pe[p] = attn_a(*qk.pop(p))
                else:
                    attn_b(p, pe.pop(p), vv.pop(p))
            if n == opt('lnpos', 99):
                base = x_v[pl.ds(r0, nw), :].astype(F32) + xn_v[pl.ds(r0, nw), :].astype(F32)
                racc = ln_step(s + 1, racc)
            if n < 3 * NP:
                qkv(n // 3, [int(c) for c in OPT.get('mo', '012')][n % 3])
            elif n < nslot:
                tk = wl[n - 3 * NP].split('-')
                y = wo_chunk(int(tk[0]), int(tk[-1]) + 1)
                acc = y if acc is None else y + acc
        if opt('lnpos', 99) > nslot:
            base = x_v[pl.ds(r0, nw), :].astype(F32) + xn_v[pl.ds(r0, nw), :].astype(F32)
        if opt('lnpos', 99) > nslot:
            racc = ln_step(s + 1, racc)
        x_v[pl.ds(r0, nw), :] = (base + acc[M:]).astype(BF16)
        return racc, acc[0:M]

    def steps(it, carry):
        def start_moe(_, c):
            for cp in moe_copies:
                cp.start()
            return c

        lax.fori_loop(0, (it == 1).astype(jnp.int32), start_moe, 0)

        with scope('it'):
            for u in range(U):
                carry = step(it, u, carry)
        return carry

    with scope('main'):
        racc, _ = lax.fori_loop(0, NSEG // U, steps, (racc, mem0_v[...].astype(F32)))

    def out_copy(r0, n, k):
        return pltpu.make_async_copy(x_v.at[pl.ds(r0, n)], out_hbm.at[pl.ds(r0, n)], sem_o.at[k])

    for cp in moe_copies:
        cp.wait()
    grp_wait(NP)
    grp_wait(NP + 1)
    st_wait(x_v.at[pl.ds(S, 2 * XBR)], sem_xb.at[1])
    st_wait(wo_v.at[pl.ds(NP * WOP, 2 * WOP)], sem_wo.at[1])
    out_copy(0, S - EPI, 0).start()

    idx = (lax.broadcasted_iota(jnp.int32, racc.shape, 1) * 8
           + lax.broadcasted_iota(jnp.int32, racc.shape, 0)).astype(F32)

    def allred(fn, v):
        return fn(fn(v, axis=1, keepdims=True), axis=0, keepdims=True)

    m1 = allred(jnp.max, racc)
    i1 = allred(jnp.min, jnp.where(racc == m1, idx, float(S - 1)))
    r2 = jnp.where(idx == i1, -jnp.inf, racc)
    m2 = allred(jnp.max, r2)
    i2 = allred(jnp.min, jnp.where((r2 == m2) & (idx != i1), idx, float(S - 1)))
    sel = [jnp.clip(jnp.max(iv).astype(jnp.int32), 0, S - 1) for iv in (i1, i2)]
    grp = [pl.multiple_of((i >> 3) << 3, 8) for i in sel]
    row8 = lax.broadcasted_iota(jnp.int32, (8, D), 0)
    rows = [jnp.sum(jnp.where(row8 == (i & 7), xn_v[pl.ds(g, 8), :].astype(F32), 0.0),
                    axis=0, keepdims=True) for i, g in zip(sel, grp)]
    row16 = lax.broadcasted_iota(jnp.int32, (16, D), 0)
    xs = jnp.where(row16 == 0, rows[0], jnp.where(row16 == 1, rows[1], 0.0)).astype(BF16)

    hs, ys, gps = {}, {}, {}

    def moe_gate(j):
        gps[j] = _rb(_dot(xs, wg_v[:, j * E:(j + 1) * E]))

    def moe_up(j):
        up = _rb(_dot(xs, wu_v[:, j * E:(j + 1) * E]))
        gp = gps.pop(j)
        g = _rb(gp * (1.0 / (1.0 + jnp.exp(-gp))))
        hs[j] = (g * up).astype(BF16)

    def moe_down(kc, nq):
        hk = jnp.concatenate([hs[4 * kc + i] for i in range(4)], axis=1)
        d = _dot(hk, wd_v[kc * 256:(kc + 1) * 256, nq * 256:(nq + 1) * 256])
        ys[nq] = d + ys[nq] if nq in ys else d

    def moe_apply():
        y = _rb(jnp.concatenate([ys[nq] for nq in range(4)], axis=1))
        upd = [_rb(y[n:n + 1, :] * _rb(1.0 / (1.0 + jnp.exp(-mv)))) for n, mv in enumerate((m1, m2))]
        for n in range(2):
            blk = x_v[pl.ds(grp[n], 8), :].astype(F32)
            for k in range(2):
                blk = blk + jnp.where(row8 + grp[n] == sel[k], upd[k], 0.0)
            fix_v[n] = blk.astype(BF16)
        for n in range(2):
            g = pl.multiple_of(jnp.maximum(grp[n], S - MOE_LATE), 8)
            x_v[pl.ds(g, 8), :] = (x_v[pl.ds(g, 8), :].astype(F32)
                                   + jnp.where(row8 + g == sel[n], upd[n], 0.0)).astype(BF16)

    waves = []
    for j in range(FF // E):
        waves += [functools.partial(moe_gate, j), functools.partial(moe_up, j)]
    for kc in range(FF // 512):
        waves += [functools.partial(moe_down, kc, nq) for nq in range(4)]
    waves = [None] * opt('mlead', 10) + waves + [None] * opt('mgap', 1) + [moe_apply]
    NM = opt('nm', 6)
    MOE_LATE = EPI

    def finish(rs, cs, acc):
        x_v[rs, cs] = (x_v[rs, cs].astype(F32) + xn_v[rs, cs].astype(F32) + acc).astype(BF16)

    NT = D // E
    with scope('epi0'):
        for blk, n in [(0, n) for n in range(NT)] + [(1, n) for n in range(2 * NM - NT)]:
            ar = OEPI + blk * 128
            r0 = S - EPI + blk * 128
            acc = None
            for kc in range(NOC):
                d = _dot(o_ld(kc, slice(ar, ar + 128)),
                         wo_v[kc * KC // 2:(kc + 1) * KC // 2, n * E:(n + 1) * E])
                acc = d if acc is None else d + acc
                if kc == NOC - 1:
                    finish(slice(r0, r0 + 128), slice(n * E, (n + 1) * E), acc)
                if waves:
                    wv = waves.pop(0)
                    if wv is not None:
                        wv()
        for wv in waves:
            if wv is not None:
                wv()

    fixes = [pltpu.make_async_copy(fix_v.at[n], out_hbm.at[pl.ds(grp[n], 8)], sem_o.at[4 + n])
             for n in range(2)]
    need = [sel[0] < S - EPI, jnp.logical_and(sel[1] < S - EPI, grp[1] != grp[0])]
    out_copy(S - EPI, 128, 1).start()
    out_copy(0, S - EPI, 0).wait()
    for n in range(2):
        @pl.when(need[n])
        def _():
            fixes[n].start()

    c0 = (2 * NM - NT) * E

    def epi(i, carry):
        ar = pl.ds(pl.multiple_of(OEPI + 128 + i * 64, 16), 64)
        a = jnp.concatenate([o_ld(c, ar) for c in range(NOC)], axis=1)
        r0 = pl.multiple_of(S - 128 + i * 64, 64)
        finish(pl.ds(r0, 64), slice(c0, D), _dot(a, wo_v[0:NP * WOP, c0:]))
        out_copy(r0, 64, 2 + i).start()
        return carry

    with scope('epi'):
        lax.fori_loop(0, 2, epi, 0)

    with scope('fin'):
        for n in range(2):
            @pl.when(need[n])
            def _():
                fixes[n].wait()
        out_copy(S - EPI, 128, 1).wait()
        for i in range(2):
            out_copy(S - 128 + i * 64, 64, 2 + i).wait()


@jax.jit
def pallas_parallel_sum__memory_aug_recurrent_mem_tr__moe_arch_mod__prompt_kernel(
    A_x: jax.Array,
    A_mem0: jax.Array,
    A_Wq: jax.Array,
    A_Wk: jax.Array,
    A_Wv: jax.Array,
    A_Wo: jax.Array,
    A_seg_len: jax.Array,
    B_x: jax.Array,
    B_w_r: jax.Array,
    B_w_gate: jax.Array,
    B_w_up: jax.Array,
    B_w_down: jax.Array,
):
    del A_seg_len, B_x
    assert A_x.shape == (1, S, D) and A_Wq.shape == (D, H, E) and A_mem0.shape == (1, M, D)
    wshape = (D // 2, 2, NP, 2, E)
    any_spec = pl.BlockSpec(memory_space=pl.ANY)
    out = pl.pallas_call(
        _kernel,
        out_shape=jax.ShapeDtypeStruct((S, D), BF16),
        in_specs=[any_spec] * 10,
        out_specs=any_spec,
        scratch_shapes=[
            pltpu.VMEM((S + 2 * XBR, D), BF16),
            pltpu.VMEM((S, D), BF16),
            pltpu.VMEM((PRE // 2, D), U32) if opt('xpn', 1) else pltpu.VMEM((PRE, D), BF16),
            pltpu.VMEM((M, D), BF16),
            pltpu.VMEM((NCH + 1, D // 2, 2 * E), U32),
            pltpu.VMEM(((NP + 2) * WOP, D), U32),
            pltpu.VMEM((NST + 1, 3, 2, D // 2, E), U32),
            pltpu.VMEM((D // 2, 2 * E), U32),
            pltpu.VMEM((D // 2, 2 * E), U32),
            pltpu.VMEM((D // 2, 2 * E), U32),
            pltpu.VMEM((D // 2, FF), U32),
            pltpu.VMEM((D // 2, FF), U32),
            pltpu.VMEM((FF // 2, D), U32),
            pltpu.VMEM((8, D), F32),
            pltpu.VMEM((2, 8, D), BF16),
            pltpu.SemaphoreType.DMA((2,)),
            pltpu.SemaphoreType.DMA((2,)),
            pltpu.SemaphoreType.DMA((2,)),
            pltpu.SemaphoreType.DMA((NST + 2,)),
            pltpu.SemaphoreType.DMA((2,)),
            pltpu.SemaphoreType.DMA((3,)),
            pltpu.SemaphoreType.DMA((6,)),
            *([pltpu.VMEM((NS, NPR + RPAD, L2, E), BF16)] * (3 * RP) if RSPLIT
              else [pltpu.VMEM((NS, 3, NPR + RPAD, L2, E), BF16)] * RP),
            *[pltpu.VMEM((OEPI + EPI, n * KC), BF16) for n in OGR],
            pltpu.VMEM((L2, L2), F32),
            pltpu.VMEM((D // E, E), BF16),
        ],
        compiler_params=pltpu.CompilerParams(vmem_limit_bytes=120 * 1024 * 1024,
                                             disable_bounds_checks=True),
    )(
        A_x.reshape(S, D),
        A_mem0.reshape(M, D),
        A_Wq.reshape(wshape),
        A_Wk.reshape(wshape),
        A_Wv.reshape(wshape),
        A_Wo.reshape(H * E, D),
        B_w_r.reshape(D // E, E),
        B_w_gate,
        B_w_up,
        B_w_down,
    )
    return out.reshape(1, S, D)
```

```python
import functools

import jax
import jax.numpy as jnp
from jax import lax
import jax.experimental.pallas as pl
import jax.experimental.pallas.tpu as pltpu

F32 = jnp.float32
BF16 = jnp.bfloat16
U32 = jnp.uint32

S = 2048
D = 1024
H = 32
E = 128
M = 8
SEG = 32
NSEG = S // SEG
FF = 3584
NP = H // 2
L1 = M + SEG
L2 = 2 * L1

PRE = 512
TPS = 24
NS = 17
U = 4
WG = (3, 3, 5, 3)
WGS = (0, 3, 6, 11)
GPI = sum(WG)
REC = (GPI + U) * 8
NREC = 4
EPI = S - (NSEG // U) * GPI * 8
OEPI = NREC * REC
NST = 4
NCH = 3 * NP
NOC = 8
KC = H * E // NOC
PPC = NP // NOC
XA = PRE // 2
XBR = (S - PRE) // NP
WOP = (H * E // 2) // NP
KS = D // 2
MB = 256
LR = 32

WO_CHUNKS = ((0, 1), (1, 2), (2, 3), (3, 4), (4, 5), (5, 6), (6, 8))
LAG_QK, LAG_S, LAG_V, LAG_PV = 2, 4, 6, 8
LATE_S = {15: 50}
LATE_PV = {14: 50, 15: 53}
MOE_LEAD, MOE_GAP = 10, 1
EPI_TILES = 4

EPS = 1e-05
SCALE = float(E) ** -0.5
LOG2E = 1.4426950408889634


def _mod17(x):
    return x - 17 * ((x * 241) >> 12)


def _div14(x):
    return (x * 293) >> 12


assert NS == 17 and SEG == 32 and GPI == 14 and NP == 16
assert all(_mod17(x) == x % 17 for x in range(128))
assert all(_div14(x) == x // 14 for x in range(256))


def _rb(v):
    return v.astype(BF16).astype(F32)


def _recip(v):
    y = pl.reciprocal(v, approx=True)
    return y * (2.0 - v * y)


def _layernorm_rows(xb, wr8):
    xf = xb.astype(F32)
    mean = jnp.sum(xf, axis=-1, keepdims=True) * (1.0 / D)
    mb = _rb(mean)
    d = xf - mb
    dm = mean - mb
    var = jnp.maximum(jnp.sum(d * d, axis=-1, keepdims=True) * (1.0 / D) - dm * dm, 0.0)
    ve = _rb(_rb(var) + EPS)
    inv = _recip(_rb(ve * lax.rsqrt(ve)))
    xw = d * inv
    wr = jnp.concatenate([wr8] * (xb.shape[0] // 8), axis=0)
    r = _rb(jnp.sum(xw * wr, axis=-1, keepdims=True))
    return xw, r


def _scatter_scores(acc, r, g0):
    lane = lax.broadcasted_iota(jnp.int32, acc.shape, 1)
    for j in range(r.shape[0] // 8):
        acc = jnp.where(lane == g0 + j, r[j * 8:(j + 1) * 8, :], acc)
    return acc


def _dot(a, w32):
    return jnp.dot(a, pltpu.bitcast(w32, BF16), preferred_element_type=F32)


def _kernel(x_hbm, mem0_hbm, wq_hbm, wk_hbm, wv_hbm, wo_hbm, wr_hbm, wg_hbm, wu_hbm, wd_hbm,
            out_hbm,
            x_v, xn_v, xp_v, mem0_v, wqkv, wo_v, stage, wc0, wc1, wc2, wg_v, wu_v, wd_v,
            wr_v, fix_v,
            sem_xa, sem_xb, sem_s, sem_st, sem_wo, sem_w, sem_o, *rest):
    w32 = [w.bitcast(U32) for w in (wq_hbm, wk_hbm, wv_hbm)]
    wo32 = wo_hbm.bitcast(U32)
    wcur = (wc0, wc1, wc2)
    ring, o_vs = rest[:3], rest[3:3 + NOC]
    fill_v, wr_in = rest[3 + NOC:]

    def xa_copy(c):
        n = XA if c == 0 else PRE + TPS - XA
        return pltpu.make_async_copy(x_hbm.at[pl.ds(c * XA, n)], x_v.at[pl.ds(c * XA, n)],
                                     sem_xa.at[c])

    def xb_copy(i):
        src = pl.multiple_of(PRE + jnp.minimum(i, NP - 1) * XBR, 32)
        dst = pl.multiple_of(PRE + i * XBR, 32)
        return pltpu.make_async_copy(x_hbm.at[pl.ds(src, XBR)], x_v.at[pl.ds(dst, XBR)],
                                     sem_xb.at[i >> 4])

    def st_copy(t, p, slot, k, dp, sem):
        return pltpu.make_async_copy(w32[t].at[:, dp, p, 0, :], stage.at[slot, k, dp], sem)

    def grp_start(g, sems=None):
        slot = g & (NST - 1)
        for k, (t, p) in enumerate(((1, g), (2, g), (0, g + 1))):
            p = jnp.minimum(p, NP - 1)
            for dp in range(2):
                st_copy(t, p, slot, k, dp, sem_st.at[slot] if sems is None else sems[k]).start()

    def wait_all(view, sem):
        pltpu.make_async_copy(view, view, sem).wait()

    def grp_wait(g):
        slot = g & (NST - 1)
        wait_all(stage.at[slot], sem_st.at[slot])

    def wo_copy(i):
        src = pl.multiple_of(jnp.minimum(i, NP - 1) * WOP, 8)
        dst = pl.multiple_of(i * WOP, 8)
        return pltpu.make_async_copy(wo32.at[pl.ds(src, WOP)], wo_v.at[pl.ds(dst, WOP)],
                                     sem_wo.at[i >> 4])

    mem0_copy = pltpu.make_async_copy(mem0_hbm, mem0_v, sem_s.at[0])
    wr_copy = pltpu.make_async_copy(wr_hbm, wr_in, sem_s.at[1])
    moe_copies = [pltpu.make_async_copy(src.bitcast(U32), dst, sem_w.at[k])
                  for k, (src, dst) in enumerate(((wg_hbm, wg_v), (wu_hbm, wu_v), (wd_hbm, wd_v)))]

    xa_copy(0).start()
    wr_copy.start()
    for dp in range(2):
        st_copy(0, 0, NST, 0, dp, sem_st.at[NST]).start()
    xa_copy(1).start()

    row = lax.broadcasted_iota(jnp.int32, (L2, L2), 0)
    col = lax.broadcasted_iota(jnp.int32, (L2, L2), 1)
    rl = jnp.where(row >= L1, row - L1, row)
    cl = jnp.where(col >= L1, col - L1, col)
    same = (row >= L1) == (col >= L1)
    keep = (rl < M) | (rl >= cl)
    fill_v[...] = jnp.where(same, jnp.where(keep, 0.0, -1000000000.0 / SCALE), -jnp.inf).astype(F32)

    def ln_rows(r0, n, racc):
        for r in range(r0, r0 + n, LR):
            xw, sc = _layernorm_rows(x_v[pl.ds(r, LR), :], wr_v[...])
            xn_v[pl.ds(r, LR), :] = xw.astype(BF16)
            xp_v[pl.ds(r // 2, LR // 2), :] = pltpu.bitcast(xn_v[pl.ds(r, LR), :], U32)
            racc = _scatter_scores(racc, sc, r // 8)
        return racc

    def ln_step(i, racc):
        ic = jnp.minimum(i, NSEG - 1)
        r0 = pl.multiple_of(PRE + ic * TPS, 8)
        xw, r = _layernorm_rows(x_v[pl.ds(r0, TPS), :], wr_v[...])
        xn_v[pl.ds(r0, TPS), :] = xw.astype(BF16)
        return _scatter_scores(racc, r, PRE // 8 + ic * (TPS // 8))

    wr_copy.wait()
    wrf = wr_in[...].astype(F32)
    wr_v[...] = jnp.broadcast_to(
        jnp.concatenate([wrf[k:k + 1, :] for k in range(D // E)], axis=1), (8, D))
    xa_copy(0).wait()
    grp_start(0, (sem_st.at[0], sem_st.at[0], sem_st.at[NST + 1]))
    racc = ln_rows(0, XA, jnp.zeros((8, S // 8), F32))

    def relayout(slot, k, c, dst):
        for j in range(D // 2 // 64):
            a = stage[slot, k, 0, j * 64:(j + 1) * 64, :]
            b = stage[slot, k, 1, j * 64:(j + 1) * 64, :]
            ev = (a & jnp.uint32(0xFFFF)) | (b << 16)
            od = (a >> 16) | (b & jnp.uint32(0xFFFF0000))
            dst[j * 64:(j + 1) * 64, 0:E] = ev
            dst[j * 64:(j + 1) * 64, E:2 * E] = od
            wqkv[c, j * 64:(j + 1) * 64, 0:E] = ev
            wqkv[c, j * 64:(j + 1) * 64, E:2 * E] = od

    def pro_dots(t, p):
        for rb in range(PRE // MB):
            a = pltpu.bitcast(xp_v[rb * MB // 2:(rb + 1) * MB // 2, :], BF16)
            y = _dot(a, wcur[t][...]).astype(BF16)
            for sg in range(MB // SEG):
                for hh in range(2):
                    ring[t][rb * (MB // SEG) + sg, p, hh * L1 + M:(hh + 1) * L1, :] = (
                        y[sg * SEG:(sg + 1) * SEG, hh * E:(hh + 1) * E])

    wait_all(stage.at[NST, 0], sem_st.at[NST])
    xa_copy(1).wait()
    mem0_copy.start()
    grp_start(1)
    relayout(NST, 0, 0, wc0)
    racc = ln_rows(XA, PRE - XA, racc)
    pro_dots(0, 0)
    racc = ln_step(0, racc)

    wait_all(stage.at[0, pl.ds(0, 2)], sem_st.at[0])
    grp_start(2)
    relayout(0, 0, 1, wc1)
    relayout(0, 1, 2, wc2)
    pro_dots(1, 0)

    wait_all(stage.at[0, 2], sem_st.at[NST + 1])
    for i in range(3):
        wo_copy(i).start()
        xb_copy(i).start()
    relayout(0, 2, 3, wc0)
    pro_dots(2, 0)

    def pro(p, carry):
        grp_wait(p)
        slot = p & (NST - 1)
        for t in range(3):
            relayout(slot, t, 3 * p + t + 1, wcur[(t + 1) % 3])
            pro_dots(t, p)

        grp_start(p + 2)
        wo_copy(p + 2).start()
        xb_copy(p + 2).start()
        return carry

    lax.fori_loop(1, NP, pro, 0)

    wait_all(x_v.at[pl.ds(PRE, S - PRE)], sem_xb.at[0])
    mem0_copy.wait()
    wait_all(wo_v.at[pl.ds(0, NP * WOP)], sem_wo.at[0])

    def step(it, u, carry):
        racc, mem = carry
        s = it * U + u
        slot = _mod17(s)
        t0 = pl.multiple_of(PRE + s * TPS, 8)
        top = xn_v[pl.ds(t0, 8), :].astype(F32)
        bot = xn_v[pl.ds(t0 + 8, 16), :]
        lhs = jnp.concatenate([jnp.concatenate([mem, top], axis=0).astype(BF16), bot], axis=0)
        part = [_dot(lhs[:, :KS], wqkv[t, 0:KS // 2, :]) for t in range(3)]
        qdst = []
        for j in range(TPS // 8):
            tj = t0 + 8 * j
            qdst.append((_mod17(tj >> 5), M + (tj & (SEG - 1))))
        odst = []
        for j in range(SEG // 8):
            g = (SEG // 8) * s + j
            gi = _div14(g)
            gr = g - GPI * gi
            r_ring = (gi & (NREC - 1)) * REC + (
                gr + 1 + sum((gr >= WGS[k]).astype(jnp.int32) for k in range(1, U))) * 8
            r_epi = OEPI + (g - (S - EPI) // 8) * 8
            odst.append(pl.multiple_of(jnp.where(g < (S - EPI) // 8, r_ring, r_epi), 8))
        orow = pl.multiple_of((it & (NREC - 1)) * REC + (WGS[u] + u) * 8, 16)
        nw = WG[u] * 8

        def qkv(p, t):
            if p == 0:
                y = _dot(lhs[:, KS:], wqkv[t, KS // 2:, :]) + part[t]
            else:
                y = _dot(lhs, wqkv[3 * p + t])
            y = y.astype(BF16)
            for hh in range(2):
                yc = y[:, hh * E:(hh + 1) * E]
                ring[t][slot, p, hh * L1:hh * L1 + M, :] = yc[0:M]
                for j in range(TPS // 8):
                    qs, qr = qdst[j]
                    ring[t][qs, p, pl.ds(pl.multiple_of(hh * L1 + qr, 8), 8), :] = (
                        yc[M + 8 * j:M + 8 * j + 8])

        def attn_probs(q, k):
            sc = lax.dot_general(q, k, (((1,), (1,)), ((), ())), preferred_element_type=F32)
            fill = fill_v[...]
            sc = jnp.where(fill == 0.0, sc, fill)
            e = jnp.exp2((sc - jnp.max(sc, axis=-1, keepdims=True)) * (SCALE * LOG2E))
            den = jnp.sum(e, axis=-1, keepdims=True)
            return (e * pl.reciprocal(den, approx=True)).astype(BF16)

        def attn_out(p, pr, v):
            o = jnp.dot(pr, v, preferred_element_type=F32).astype(BF16)
            oc = o_vs[p // PPC]
            for hh in range(2):
                cs = (2 * (p % PPC) + hh) * E
                oc[pl.ds(orow, M), cs:cs + E] = o[hh * L1:hh * L1 + M]
                for j in range(SEG // 8):
                    r = hh * L1 + M + 8 * j
                    oc[pl.ds(odst[j], 8), cs:cs + E] = o[r:r + 8]

        def wo_chunk(c, c1):
            a = jnp.concatenate([o_vs[i][pl.ds(orow, M + nw), :] for i in range(c, c1)], axis=1)
            return _dot(a, wo_v[c * KC // 2:c1 * KC // 2, :])

        nslot = 3 * NP + len(WO_CHUNKS)
        ev = {n: [] for n in range(nslot)}
        for p in range(NP):
            at_s = LATE_S.get(p, 3 * p + LAG_S)
            at_pv = LATE_PV.get(p, 3 * p + LAG_PV)
            ev[min(3 * p + LAG_QK, at_s)].append((0, p))
            ev[min(3 * p + LAG_V, at_pv)].append((1, p))
            ev[at_pv].append((2, p))
            ev[at_s].append((3, p))
        pr, qk, vv = {}, {}, {}
        acc = None
        r0 = pl.multiple_of((it * GPI + WGS[u]) * 8, 8)
        for n in range(nslot):
            for kind, p in sorted(ev[n]):
                if kind == 0:
                    qk[p] = (ring[0][slot, p], ring[1][slot, p])
                elif kind == 1:
                    vv[p] = ring[2][slot, p]
                elif kind == 2:
                    attn_out(p, pr.pop(p), vv.pop(p))
                else:
                    pr[p] = attn_probs(*qk.pop(p))
            if n < 3 * NP:
                qkv(n // 3, n % 3)
            else:
                y = wo_chunk(*WO_CHUNKS[n - 3 * NP])
                acc = y if acc is None else y + acc
        base = x_v[pl.ds(r0, nw), :].astype(F32) + xn_v[pl.ds(r0, nw), :].astype(F32)
        racc = ln_step(s + 1, racc)
        x_v[pl.ds(r0, nw), :] = (base + acc[M:]).astype(BF16)
        return racc, acc[0:M]

    def steps(it, carry):
        def start_moe(_, c):
            for cp in moe_copies:
                cp.start()
            return c

        lax.fori_loop(0, (it == 1).astype(jnp.int32), start_moe, 0)

        for u in range(U):
            carry = step(it, u, carry)
        return carry

    racc, _ = lax.fori_loop(0, NSEG // U, steps, (racc, mem0_v[...].astype(F32)))

    def out_copy(r0, n, k):
        return pltpu.make_async_copy(x_v.at[pl.ds(r0, n)], out_hbm.at[pl.ds(r0, n)], sem_o.at[k])

    for cp in moe_copies:
        cp.wait()
    grp_wait(NP)
    grp_wait(NP + 1)
    wait_all(x_v.at[pl.ds(S, 2 * XBR)], sem_xb.at[1])
    wait_all(wo_v.at[pl.ds(NP * WOP, 2 * WOP)], sem_wo.at[1])
    out_copy(0, S - EPI, 0).start()

    idx = (lax.broadcasted_iota(jnp.int32, racc.shape, 1) * 8
           + lax.broadcasted_iota(jnp.int32, racc.shape, 0)).astype(F32)

    def allred(fn, v):
        return fn(fn(v, axis=1, keepdims=True), axis=0, keepdims=True)

    m1 = allred(jnp.max, racc)
    i1 = allred(jnp.min, jnp.where(racc == m1, idx, float(S - 1)))
    r2 = jnp.where(idx == i1, -jnp.inf, racc)
    m2 = allred(jnp.max, r2)
    i2 = allred(jnp.min, jnp.where((r2 == m2) & (idx != i1), idx, float(S - 1)))
    sel = [jnp.clip(jnp.max(iv).astype(jnp.int32), 0, S - 1) for iv in (i1, i2)]
    grp = [pl.multiple_of((i >> 3) << 3, 8) for i in sel]
    row8 = lax.broadcasted_iota(jnp.int32, (8, D), 0)
    rows = [jnp.sum(jnp.where(row8 == (i & 7), xn_v[pl.ds(g, 8), :].astype(F32), 0.0),
                    axis=0, keepdims=True) for i, g in zip(sel, grp)]
    row16 = lax.broadcasted_iota(jnp.int32, (16, D), 0)
    xs = jnp.where(row16 == 0, rows[0], jnp.where(row16 == 1, rows[1], 0.0)).astype(BF16)

    hs, ys, gps = {}, {}, {}

    def moe_gate(j):
        gps[j] = _rb(_dot(xs, wg_v[:, j * E:(j + 1) * E]))

    def moe_up(j):
        up = _rb(_dot(xs, wu_v[:, j * E:(j + 1) * E]))
        gp = gps.pop(j)
        g = _rb(gp * (1.0 / (1.0 + jnp.exp(-gp))))
        hs[j] = (g * up).astype(BF16)

    def moe_down(kc, nq):
        hk = jnp.concatenate([hs[4 * kc + i] for i in range(4)], axis=1)
        d = _dot(hk, wd_v[kc * 256:(kc + 1) * 256, nq * 256:(nq + 1) * 256])
        ys[nq] = d + ys[nq] if nq in ys else d

    def moe_apply():
        y = _rb(jnp.concatenate([ys[nq] for nq in range(4)], axis=1))
        upd = [_rb(y[n:n + 1, :] * _rb(1.0 / (1.0 + jnp.exp(-mv)))) for n, mv in enumerate((m1, m2))]
        for n in range(2):
            blk = x_v[pl.ds(grp[n], 8), :].astype(F32)
            for k in range(2):
                blk = blk + jnp.where(row8 + grp[n] == sel[k], upd[k], 0.0)
            fix_v[n] = blk.astype(BF16)
        for n in range(2):
            g = pl.multiple_of(jnp.maximum(grp[n], S - EPI), 8)
            x_v[pl.ds(g, 8), :] = (x_v[pl.ds(g, 8), :].astype(F32)
                                   + jnp.where(row8 + g == sel[n], upd[n], 0.0)).astype(BF16)

    waves = []
    for j in range(FF // E):
        waves += [functools.partial(moe_gate, j), functools.partial(moe_up, j)]
    for kc in range(FF // 512):
        waves += [functools.partial(moe_down, kc, nq) for nq in range(4)]
    waves = [None] * MOE_LEAD + waves + [None] * MOE_GAP + [moe_apply]

    def finish(rs, cs, acc):
        x_v[rs, cs] = (x_v[rs, cs].astype(F32) + xn_v[rs, cs].astype(F32) + acc).astype(BF16)

    for blk, n in [(0, n) for n in range(D // E)] + [(1, n) for n in range(EPI_TILES)]:
        ar = OEPI + blk * 128
        r0 = S - EPI + blk * 128
        acc = None
        for kc in range(NOC):
            d = _dot(o_vs[kc][ar:ar + 128, :],
                     wo_v[kc * KC // 2:(kc + 1) * KC // 2, n * E:(n + 1) * E])
            acc = d if acc is None else d + acc
            if kc == NOC - 1:
                finish(slice(r0, r0 + 128), slice(n * E, (n + 1) * E), acc)
            wv = waves.pop(0) if waves else None
            if wv is not None:
                wv()
    assert not waves

    fixes = [pltpu.make_async_copy(fix_v.at[n], out_hbm.at[pl.ds(grp[n], 8)], sem_o.at[4 + n])
             for n in range(2)]
    need = [sel[0] < S - EPI, jnp.logical_and(sel[1] < S - EPI, grp[1] != grp[0])]
    out_copy(S - EPI, 128, 1).start()
    out_copy(0, S - EPI, 0).wait()
    for n in range(2):
        @pl.when(need[n])
        def _():
            fixes[n].start()

    c0 = EPI_TILES * E

    def epi(i, carry):
        ar = pl.ds(pl.multiple_of(OEPI + 128 + i * 64, 16), 64)
        a = jnp.concatenate([oc[ar, :] for oc in o_vs], axis=1)
        r0 = pl.multiple_of(S - 128 + i * 64, 64)
        finish(pl.ds(r0, 64), slice(c0, D), _dot(a, wo_v[0:NP * WOP, c0:]))
        out_copy(r0, 64, 2 + i).start()
        return carry

    lax.fori_loop(0, 2, epi, 0)

    for n in range(2):
        @pl.when(need[n])
        def _():
            fixes[n].wait()
    out_copy(S - EPI, 128, 1).wait()
    for i in range(2):
        out_copy(S - 128 + i * 64, 64, 2 + i).wait()


@jax.jit
def pallas_parallel_sum__memory_aug_recurrent_mem_tr__moe_arch_mod__prompt_kernel(
    A_x: jax.Array,
    A_mem0: jax.Array,
    A_Wq: jax.Array,
    A_Wk: jax.Array,
    A_Wv: jax.Array,
    A_Wo: jax.Array,
    A_seg_len: jax.Array,
    B_x: jax.Array,
    B_w_r: jax.Array,
    B_w_gate: jax.Array,
    B_w_up: jax.Array,
    B_w_down: jax.Array,
):
    del A_seg_len, B_x
    assert A_x.shape == (1, S, D) and A_Wq.shape == (D, H, E) and A_mem0.shape == (1, M, D)
    assert B_w_gate.shape == (D, FF)
    wshape = (D // 2, 2, NP, 2, E)
    any_spec = pl.BlockSpec(memory_space=pl.ANY)
    out = pl.pallas_call(
        _kernel,
        out_shape=jax.ShapeDtypeStruct((S, D), BF16),
        in_specs=[any_spec] * 10,
        out_specs=any_spec,
        scratch_shapes=[
            pltpu.VMEM((S + 2 * XBR, D), BF16),
            pltpu.VMEM((S, D), BF16),
            pltpu.VMEM((PRE // 2, D), U32),
            pltpu.VMEM((M, D), BF16),
            pltpu.VMEM((NCH + 1, D // 2, 2 * E), U32),
            pltpu.VMEM(((NP + 2) * WOP, D), U32),
            pltpu.VMEM((NST + 1, 3, 2, D // 2, E), U32),
            pltpu.VMEM((D // 2, 2 * E), U32),
            pltpu.VMEM((D // 2, 2 * E), U32),
            pltpu.VMEM((D // 2, 2 * E), U32),
            pltpu.VMEM((D // 2, FF), U32),
            pltpu.VMEM((D // 2, FF), U32),
            pltpu.VMEM((FF // 2, D), U32),
            pltpu.VMEM((8, D), F32),
            pltpu.VMEM((2, 8, D), BF16),
            pltpu.SemaphoreType.DMA((2,)),
            pltpu.SemaphoreType.DMA((2,)),
            pltpu.SemaphoreType.DMA((2,)),
            pltpu.SemaphoreType.DMA((NST + 2,)),
            pltpu.SemaphoreType.DMA((2,)),
            pltpu.SemaphoreType.DMA((3,)),
            pltpu.SemaphoreType.DMA((6,)),
            *[pltpu.VMEM((NS, NP, L2, E), BF16)] * 3,
            *[pltpu.VMEM((OEPI + EPI, KC), BF16)] * NOC,
            pltpu.VMEM((L2, L2), F32),
            pltpu.VMEM((D // E, E), BF16),
        ],
        compiler_params=pltpu.CompilerParams(vmem_limit_bytes=120 * 1024 * 1024,
                                             disable_bounds_checks=True),
    )(
        A_x.reshape(S, D),
        A_mem0.reshape(M, D),
        A_Wq.reshape(wshape),
        A_Wk.reshape(wshape),
        A_Wv.reshape(wshape),
        A_Wo.reshape(H * E, D),
        B_w_r.reshape(D // E, E),
        B_w_gate,
        B_w_up,
        B_w_down,
    )
    return out.reshape(1, S, D)
```

```python
import functools

import jax
import jax.numpy as jnp
from jax import lax
import jax.experimental.pallas as pl
import jax.experimental.pallas.tpu as pltpu

F32 = jnp.float32
BF16 = jnp.bfloat16
U32 = jnp.uint32

S = 2048
D = 1024
H = 32
E = 128
M = 8
SEG = 32
NSEG = S // SEG
FF = 3584
NP = H // 2
L1 = M + SEG
L2 = 2 * L1

PRE = 512
TPS = 24
NS = 17
U = 4
WG = (3, 3, 5, 3)
WGS = (0, 3, 6, 11)
GPI = sum(WG)
REC = (GPI + U) * 8
NREC = 4
EPI = S - (NSEG // U) * GPI * 8
OEPI = NREC * REC
NST = 4
NCH = 3 * NP
NOC = 8
KC = H * E // NOC
PPC = NP // NOC
XA = PRE // 2
XBR = (S - PRE) // NP
WOP = (H * E // 2) // NP
KS = D // 2
MB = 256
LR = 32

WO_CHUNKS = ((0, 1), (1, 2), (2, 3), (3, 4), (4, 5), (5, 6), (6, 8))
LAG_QK, LAG_S, LAG_V, LAG_PV = 2, 4, 6, 8
LATE_S = {15: 50}
LATE_PV = {14: 50, 15: 53}
MOE_LEAD, MOE_GAP = 10, 1
EPI_TILES = 4

EPS = 1e-05
SCALE = float(E) ** -0.5
LOG2E = 1.4426950408889634


def _mod17(x):
    return x - 17 * ((x * 241) >> 12)


def _div14(x):
    return (x * 293) >> 12


assert NS == 17 and SEG == 32 and GPI == 14 and NP == 16
assert all(_mod17(x) == x % 17 for x in range(128))
assert all(_div14(x) == x // 14 for x in range(256))


def _rb(v):
    return v.astype(BF16).astype(F32)


def _recip(v):
    y = pl.reciprocal(v, approx=True)
    return y * (2.0 - v * y)


def _layernorm_rows(xb, wr8):
    xf = xb.astype(F32)
    mean = jnp.sum(xf, axis=-1, keepdims=True) * (1.0 / D)
    mb = _rb(mean)
    d = xf - mb
    dm = mean - mb
    var = jnp.maximum(jnp.sum(d * d, axis=-1, keepdims=True) * (1.0 / D) - dm * dm, 0.0)
    ve = _rb(_rb(var) + EPS)
    inv = _recip(_rb(ve * lax.rsqrt(ve)))
    xw = d * inv
    wr = jnp.concatenate([wr8] * (xb.shape[0] // 8), axis=0)
    r = _rb(jnp.sum(xw * wr, axis=-1, keepdims=True))
    return xw, r


def _scatter_scores(acc, r, g0):
    lane = lax.broadcasted_iota(jnp.int32, acc.shape, 1)
    for j in range(r.shape[0] // 8):
        acc = jnp.where(lane == g0 + j, r[j * 8:(j + 1) * 8, :], acc)
    return acc


def _dot(a, w32):
    return jnp.dot(a, pltpu.bitcast(w32, BF16), preferred_element_type=F32)


def _kernel(x_hbm, mem0_hbm, wq_hbm, wk_hbm, wv_hbm, wo_hbm, wr_hbm, wg_hbm, wu_hbm, wd_hbm,
            out_hbm,
            x_v, xn_v, xp_v, mem0_v, wqkv, wo_v, stage, wc0, wc1, wc2, wg_v, wu_v, wd_v,
            wr_v, fix_v,
            sem_xa, sem_xb, sem_s, sem_st, sem_wo, sem_w, sem_o, *rest):
    w32 = [w.bitcast(U32) for w in (wq_hbm, wk_hbm, wv_hbm)]
    wo32 = wo_hbm.bitcast(U32)
    wcur = (wc0, wc1, wc2)
    ring, o_vs = rest[:3], rest[3:3 + NOC]
    fill_v, wr_in = rest[3 + NOC:]

    def xa_copy(c):
        n = XA if c == 0 else PRE + TPS - XA
        return pltpu.make_async_copy(x_hbm.at[pl.ds(c * XA, n)], x_v.at[pl.ds(c * XA, n)],
                                     sem_xa.at[c])

    def xb_copy(i):
        src = pl.multiple_of(PRE + jnp.minimum(i, NP - 1) * XBR, 32)
        dst = pl.multiple_of(PRE + i * XBR, 32)
        return pltpu.make_async_copy(x_hbm.at[pl.ds(src, XBR)], x_v.at[pl.ds(dst, XBR)],
                                     sem_xb.at[i >> 4])

    def st_copy(t, p, slot, k, dp, sem):
        return pltpu.make_async_copy(w32[t].at[:, dp, p, 0, :], stage.at[slot, k, dp], sem)

    def grp_start(g, sems=None):
        slot = g & (NST - 1)
        for k, (t, p) in enumerate(((1, g), (2, g), (0, g + 1))):
            p = jnp.minimum(p, NP - 1)
            for dp in range(2):
                st_copy(t, p, slot, k, dp, sem_st.at[slot] if sems is None else sems[k]).start()

    def wait_all(view, sem):
        pltpu.make_async_copy(view, view, sem).wait()

    def grp_wait(g):
        slot = g & (NST - 1)
        wait_all(stage.at[slot], sem_st.at[slot])

    def wo_copy(i):
        src = pl.multiple_of(jnp.minimum(i, NP - 1) * WOP, 8)
        dst = pl.multiple_of(i * WOP, 8)
        return pltpu.make_async_copy(wo32.at[pl.ds(src, WOP)], wo_v.at[pl.ds(dst, WOP)],
                                     sem_wo.at[i >> 4])

    mem0_copy = pltpu.make_async_copy(mem0_hbm, mem0_v, sem_s.at[0])
    wr_copy = pltpu.make_async_copy(wr_hbm, wr_in, sem_s.at[1])
    moe_copies = [pltpu.make_async_copy(src.bitcast(U32), dst, sem_w.at[k])
                  for k, (src, dst) in enumerate(((wg_hbm, wg_v), (wu_hbm, wu_v), (wd_hbm, wd_v)))]

    xa_copy(0).start()
    wr_copy.start()
    for dp in range(2):
        st_copy(0, 0, NST, 0, dp, sem_st.at[NST]).start()
    xa_copy(1).start()

    row = lax.broadcasted_iota(jnp.int32, (L2, L2), 0)
    col = lax.broadcasted_iota(jnp.int32, (L2, L2), 1)
    rl = jnp.where(row >= L1, row - L1, row)
    cl = jnp.where(col >= L1, col - L1, col)
    same = (row >= L1) == (col >= L1)
    keep = (rl < M) | (rl >= cl)
    fill_v[...] = jnp.where(same, jnp.where(keep, 0.0, -1000000000.0 / SCALE), -jnp.inf).astype(F32)

    def ln_rows(r0, n, racc):
        for r in range(r0, r0 + n, LR):
            xw, sc = _layernorm_rows(x_v[pl.ds(r, LR), :], wr_v[...])
            xn_v[pl.ds(r, LR), :] = xw.astype(BF16)
            xp_v[pl.ds(r // 2, LR // 2), :] = pltpu.bitcast(xn_v[pl.ds(r, LR), :], U32)
            racc = _scatter_scores(racc, sc, r // 8)
        return racc

    def ln_step(i, racc):
        ic = jnp.minimum(i, NSEG - 1)
        r0 = pl.multiple_of(PRE + ic * TPS, 8)
        xw, r = _layernorm_rows(x_v[pl.ds(r0, TPS), :], wr_v[...])
        xn_v[pl.ds(r0, TPS), :] = xw.astype(BF16)
        return _scatter_scores(racc, r, PRE // 8 + ic * (TPS // 8))

    wr_copy.wait()
    wrf = wr_in[...].astype(F32)
    wr_v[...] = jnp.broadcast_to(
        jnp.concatenate([wrf[k:k + 1, :] for k in range(D // E)], axis=1), (8, D))
    xa_copy(0).wait()
    grp_start(0, (sem_st.at[0], sem_st.at[0], sem_st.at[NST + 1]))
    racc = ln_rows(0, XA, jnp.zeros((8, S // 8), F32))

    def relayout(slot, k, c, dst):
        for j in range(D // 2 // 64):
            a = stage[slot, k, 0, j * 64:(j + 1) * 64, :]
            b = stage[slot, k, 1, j * 64:(j + 1) * 64, :]
            ev = (a & jnp.uint32(0xFFFF)) | (b << 16)
            od = (a >> 16) | (b & jnp.uint32(0xFFFF0000))
            dst[j * 64:(j + 1) * 64, 0:E] = ev
            dst[j * 64:(j + 1) * 64, E:2 * E] = od
            wqkv[c, j * 64:(j + 1) * 64, 0:E] = ev
            wqkv[c, j * 64:(j + 1) * 64, E:2 * E] = od

    def pro_dots(t, p):
        for rb in range(PRE // MB):
            a = pltpu.bitcast(xp_v[rb * MB // 2:(rb + 1) * MB // 2, :], BF16)
            y = _dot(a, wcur[t][...]).astype(BF16)
            for sg in range(MB // SEG):
                for hh in range(2):
                    ring[t][rb * (MB // SEG) + sg, p, hh * L1 + M:(hh + 1) * L1, :] = (
                        y[sg * SEG:(sg + 1) * SEG, hh * E:(hh + 1) * E])

    wait_all(stage.at[NST, 0], sem_st.at[NST])
    xa_copy(1).wait()
    mem0_copy.start()
    grp_start(1)
    relayout(NST, 0, 0, wc0)
    racc = ln_rows(XA, PRE - XA, racc)
    pro_dots(0, 0)
    racc = ln_step(0, racc)

    wait_all(stage.at[0, pl.ds(0, 2)], sem_st.at[0])
    grp_start(2)
    relayout(0, 0, 1, wc1)
    relayout(0, 1, 2, wc2)
    pro_dots(1, 0)

    wait_all(stage.at[0, 2], sem_st.at[NST + 1])
    for i in range(3):
        wo_copy(i).start()
        xb_copy(i).start()
    relayout(0, 2, 3, wc0)
    pro_dots(2, 0)

    def pro(p, carry):
        grp_wait(p)
        slot = p & (NST - 1)
        for t in range(3):
            relayout(slot, t, 3 * p + t + 1, wcur[(t + 1) % 3])
            pro_dots(t, p)

        grp_start(p + 2)
        wo_copy(p + 2).start()
        xb_copy(p + 2).start()
        return carry

    lax.fori_loop(1, NP, pro, 0)

    wait_all(x_v.at[pl.ds(PRE, S - PRE)], sem_xb.at[0])
    mem0_copy.wait()
    wait_all(wo_v.at[pl.ds(0, NP * WOP)], sem_wo.at[0])
    for cp in moe_copies:
        cp.start()

    def step(it, u, carry):
        racc, mem = carry
        s = it * U + u
        slot = _mod17(s)
        t0 = pl.multiple_of(PRE + s * TPS, 8)
        top = xn_v[pl.ds(t0, 8), :].astype(F32)
        bot = xn_v[pl.ds(t0 + 8, 16), :]
        lhs = jnp.concatenate([jnp.concatenate([mem, top], axis=0).astype(BF16), bot], axis=0)
        part = [_dot(lhs[:, :KS], wqkv[t, 0:KS // 2, :]) for t in range(3)]
        qdst = []
        for j in range(TPS // 8):
            tj = t0 + 8 * j
            qdst.append((_mod17(tj >> 5), M + (tj & (SEG - 1))))
        odst = []
        for j in range(SEG // 8):
            g = (SEG // 8) * s + j
            gi = _div14(g)
            gr = g - GPI * gi
            r_ring = (gi & (NREC - 1)) * REC + (
                gr + 1 + sum((gr >= WGS[k]).astype(jnp.int32) for k in range(1, U))) * 8
            r_epi = OEPI + (g - (S - EPI) // 8) * 8
            odst.append(pl.multiple_of(jnp.where(g < (S - EPI) // 8, r_ring, r_epi), 8))
        orow = pl.multiple_of((it & (NREC - 1)) * REC + (WGS[u] + u) * 8, 16)
        nw = WG[u] * 8

        def qkv(p, t):
            if p == 0:
                y = _dot(lhs[:, KS:], wqkv[t, KS // 2:, :]) + part[t]
            else:
                y = _dot(lhs, wqkv[3 * p + t])
            y = y.astype(BF16)
            for hh in range(2):
                yc = y[:, hh * E:(hh + 1) * E]
                ring[t][slot, p, hh * L1:hh * L1 + M, :] = yc[0:M]
                for j in range(TPS // 8):
                    qs, qr = qdst[j]
                    ring[t][qs, p, pl.ds(pl.multiple_of(hh * L1 + qr, 8), 8), :] = (
                        yc[M + 8 * j:M + 8 * j + 8])

        def attn_probs(q, k):
            sc = lax.dot_general(q, k, (((1,), (1,)), ((), ())), preferred_element_type=F32)
            fill = fill_v[...]
            sc = jnp.where(fill == 0.0, sc, fill)
            e = jnp.exp2((sc - jnp.max(sc, axis=-1, keepdims=True)) * (SCALE * LOG2E))
            den = jnp.sum(e, axis=-1, keepdims=True)
            return (e * pl.reciprocal(den, approx=True)).astype(BF16)

        def attn_out(p, pr, v):
            o = jnp.dot(pr, v, preferred_element_type=F32).astype(BF16)
            oc = o_vs[p // PPC]
            for hh in range(2):
                cs = (2 * (p % PPC) + hh) * E
                oc[pl.ds(orow, M), cs:cs + E] = o[hh * L1:hh * L1 + M]
                for j in range(SEG // 8):
                    r = hh * L1 + M + 8 * j
                    oc[pl.ds(odst[j], 8), cs:cs + E] = o[r:r + 8]

        def wo_chunk(c, c1):
            a = jnp.concatenate([o_vs[i][pl.ds(orow, M + nw), :] for i in range(c, c1)], axis=1)
            return _dot(a, wo_v[c * KC // 2:c1 * KC // 2, :])

        nslot = 3 * NP + len(WO_CHUNKS)
        ev = {n: [] for n in range(nslot)}
        for p in range(NP):
            at_s = LATE_S.get(p, 3 * p + LAG_S)
            at_pv = LATE_PV.get(p, 3 * p + LAG_PV)
            ev[min(3 * p + LAG_QK, at_s)].append((0, p))
            ev[min(3 * p + LAG_V, at_pv)].append((1, p))
            ev[at_pv].append((2, p))
            ev[at_s].append((3, p))
        pr, qk, vv = {}, {}, {}
        acc = None
        r0 = pl.multiple_of((it * GPI + WGS[u]) * 8, 8)
        for n in range(nslot):
            for kind, p in sorted(ev[n]):
                if kind == 0:
                    qk[p] = (ring[0][slot, p], ring[1][slot, p])
                elif kind == 1:
                    vv[p] = ring[2][slot, p]
                elif kind == 2:
                    attn_out(p, pr.pop(p), vv.pop(p))
                else:
                    pr[p] = attn_probs(*qk.pop(p))
            if n < 3 * NP:
                qkv(n // 3, n % 3)
            else:
                y = wo_chunk(*WO_CHUNKS[n - 3 * NP])
                acc = y if acc is None else y + acc
        base = x_v[pl.ds(r0, nw), :].astype(F32) + xn_v[pl.ds(r0, nw), :].astype(F32)
        racc = ln_step(s + 1, racc)
        x_v[pl.ds(r0, nw), :] = (base + acc[M:]).astype(BF16)
        return racc, acc[0:M]

    def steps(it, carry):
        for u in range(U):
            carry = step(it, u, carry)
        return carry

    racc, _ = lax.fori_loop(0, NSEG // U, steps, (racc, mem0_v[...].astype(F32)))

    def out_copy(r0, n, k):
        return pltpu.make_async_copy(x_v.at[pl.ds(r0, n)], out_hbm.at[pl.ds(r0, n)], sem_o.at[k])

    for cp in moe_copies:
        cp.wait()
    grp_wait(NP)
    grp_wait(NP + 1)
    wait_all(x_v.at[pl.ds(S, 2 * XBR)], sem_xb.at[1])
    wait_all(wo_v.at[pl.ds(NP * WOP, 2 * WOP)], sem_wo.at[1])
    out_copy(0, S - EPI, 0).start()

    idx = (lax.broadcasted_iota(jnp.int32, racc.shape, 1) * 8
           + lax.broadcasted_iota(jnp.int32, racc.shape, 0)).astype(F32)

    def allred(fn, v):
        return fn(fn(v, axis=1, keepdims=True), axis=0, keepdims=True)

    m1 = allred(jnp.max, racc)
    i1 = allred(jnp.min, jnp.where(racc == m1, idx, float(S - 1)))
    r2 = jnp.where(idx == i1, -jnp.inf, racc)
    m2 = allred(jnp.max, r2)
    i2 = allred(jnp.min, jnp.where((r2 == m2) & (idx != i1), idx, float(S - 1)))
    sel = [jnp.clip(jnp.max(iv).astype(jnp.int32), 0, S - 1) for iv in (i1, i2)]
    grp = [pl.multiple_of((i >> 3) << 3, 8) for i in sel]
    row8 = lax.broadcasted_iota(jnp.int32, (8, D), 0)
    rows = [jnp.sum(jnp.where(row8 == (i & 7), xn_v[pl.ds(g, 8), :].astype(F32), 0.0),
                    axis=0, keepdims=True) for i, g in zip(sel, grp)]
    row16 = lax.broadcasted_iota(jnp.int32, (16, D), 0)
    xs = jnp.where(row16 == 0, rows[0], jnp.where(row16 == 1, rows[1], 0.0)).astype(BF16)

    hs, ys, gps = {}, {}, {}

    def moe_gate(j):
        gps[j] = _rb(_dot(xs, wg_v[:, j * E:(j + 1) * E]))

    def moe_up(j):
        up = _rb(_dot(xs, wu_v[:, j * E:(j + 1) * E]))
        gp = gps.pop(j)
        g = _rb(gp * (1.0 / (1.0 + jnp.exp(-gp))))
        hs[j] = (g * up).astype(BF16)

    def moe_down(kc, nq):
        hk = jnp.concatenate([hs[4 * kc + i] for i in range(4)], axis=1)
        d = _dot(hk, wd_v[kc * 256:(kc + 1) * 256, nq * 256:(nq + 1) * 256])
        ys[nq] = d + ys[nq] if nq in ys else d

    def moe_apply():
        y = _rb(jnp.concatenate([ys[nq] for nq in range(4)], axis=1))
        upd = [_rb(y[n:n + 1, :] * _rb(1.0 / (1.0 + jnp.exp(-mv)))) for n, mv in enumerate((m1, m2))]
        for n in range(2):
            blk = x_v[pl.ds(grp[n], 8), :].astype(F32)
            for k in range(2):
                blk = blk + jnp.where(row8 + grp[n] == sel[k], upd[k], 0.0)
            fix_v[n] = blk.astype(BF16)
        for n in range(2):
            g = pl.multiple_of(jnp.maximum(grp[n], S - EPI), 8)
            x_v[pl.ds(g, 8), :] = (x_v[pl.ds(g, 8), :].astype(F32)
                                   + jnp.where(row8 + g == sel[n], upd[n], 0.0)).astype(BF16)

    waves = []
    for j in range(FF // E):
        waves += [functools.partial(moe_gate, j), functools.partial(moe_up, j)]
    for kc in range(FF // 512):
        waves += [functools.partial(moe_down, kc, nq) for nq in range(4)]
    waves = [None] * MOE_LEAD + waves + [None] * MOE_GAP + [moe_apply]

    def finish(rs, cs, acc):
        x_v[rs, cs] = (x_v[rs, cs].astype(F32) + xn_v[rs, cs].astype(F32) + acc).astype(BF16)

    for blk, n in [(0, n) for n in range(D // E)] + [(1, n) for n in range(EPI_TILES)]:
        ar = OEPI + blk * 128
        r0 = S - EPI + blk * 128
        acc = None
        for kc in range(NOC):
            d = _dot(o_vs[kc][ar:ar + 128, :],
                     wo_v[kc * KC // 2:(kc + 1) * KC // 2, n * E:(n + 1) * E])
            acc = d if acc is None else d + acc
            if kc == NOC - 1:
                finish(slice(r0, r0 + 128), slice(n * E, (n + 1) * E), acc)
            wv = waves.pop(0) if waves else None
            if wv is not None:
                wv()
    assert not waves

    fixes = [pltpu.make_async_copy(fix_v.at[n], out_hbm.at[pl.ds(grp[n], 8)], sem_o.at[4 + n])
             for n in range(2)]
    need = [sel[0] < S - EPI, jnp.logical_and(sel[1] < S - EPI, grp[1] != grp[0])]
    out_copy(S - EPI, 128, 1).start()
    out_copy(0, S - EPI, 0).wait()
    for n in range(2):
        @pl.when(need[n])
        def _():
            fixes[n].start()

    c0 = EPI_TILES * E

    def epi(i, carry):
        ar = pl.ds(pl.multiple_of(OEPI + 128 + i * 64, 16), 64)
        a = jnp.concatenate([oc[ar, :] for oc in o_vs], axis=1)
        r0 = pl.multiple_of(S - 128 + i * 64, 64)
        finish(pl.ds(r0, 64), slice(c0, D), _dot(a, wo_v[0:NP * WOP, c0:]))
        out_copy(r0, 64, 2 + i).start()
        return carry

    lax.fori_loop(0, 2, epi, 0)

    for n in range(2):
        @pl.when(need[n])
        def _():
            fixes[n].wait()
    out_copy(S - EPI, 128, 1).wait()
    for i in range(2):
        out_copy(S - 128 + i * 64, 64, 2 + i).wait()


@jax.jit
def pallas_parallel_sum__memory_aug_recurrent_mem_tr__moe_arch_mod__prompt_kernel(
    A_x: jax.Array,
    A_mem0: jax.Array,
    A_Wq: jax.Array,
    A_Wk: jax.Array,
    A_Wv: jax.Array,
    A_Wo: jax.Array,
    A_seg_len: jax.Array,
    B_x: jax.Array,
    B_w_r: jax.Array,
    B_w_gate: jax.Array,
    B_w_up: jax.Array,
    B_w_down: jax.Array,
):
    del A_seg_len, B_x
    assert A_x.shape == (1, S, D) and A_Wq.shape == (D, H, E) and A_mem0.shape == (1, M, D)
    assert B_w_gate.shape == (D, FF)
    wshape = (D // 2, 2, NP, 2, E)
    any_spec = pl.BlockSpec(memory_space=pl.ANY)
    out = pl.pallas_call(
        _kernel,
        out_shape=jax.ShapeDtypeStruct((S, D), BF16),
        in_specs=[any_spec] * 10,
        out_specs=any_spec,
        scratch_shapes=[
            pltpu.VMEM((S + 2 * XBR, D), BF16),
            pltpu.VMEM((S, D), BF16),
            pltpu.VMEM((PRE // 2, D), U32),
            pltpu.VMEM((M, D), BF16),
            pltpu.VMEM((NCH + 1, D // 2, 2 * E), U32),
            pltpu.VMEM(((NP + 2) * WOP, D), U32),
            pltpu.VMEM((NST + 1, 3, 2, D // 2, E), U32),
            pltpu.VMEM((D // 2, 2 * E), U32),
            pltpu.VMEM((D // 2, 2 * E), U32),
            pltpu.VMEM((D // 2, 2 * E), U32),
            pltpu.VMEM((D // 2, FF), U32),
            pltpu.VMEM((D // 2, FF), U32),
            pltpu.VMEM((FF // 2, D), U32),
            pltpu.VMEM((8, D), F32),
            pltpu.VMEM((2, 8, D), BF16),
            pltpu.SemaphoreType.DMA((2,)),
            pltpu.SemaphoreType.DMA((2,)),
            pltpu.SemaphoreType.DMA((2,)),
            pltpu.SemaphoreType.DMA((NST + 2,)),
            pltpu.SemaphoreType.DMA((2,)),
            pltpu.SemaphoreType.DMA((3,)),
            pltpu.SemaphoreType.DMA((6,)),
            *[pltpu.VMEM((NS, NP, L2, E), BF16)] * 3,
            *[pltpu.VMEM((OEPI + EPI, KC), BF16)] * NOC,
            pltpu.VMEM((L2, L2), F32),
            pltpu.VMEM((D // E, E), BF16),
        ],
        compiler_params=pltpu.CompilerParams(vmem_limit_bytes=120 * 1024 * 1024,
                                             disable_bounds_checks=True),
    )(
        A_x.reshape(S, D),
        A_mem0.reshape(M, D),
        A_Wq.reshape(wshape),
        A_Wk.reshape(wshape),
        A_Wv.reshape(wshape),
        A_Wo.reshape(H * E, D),
        B_w_r.reshape(D // E, E),
        B_w_gate,
        B_w_up,
        B_w_down,
    )
    return out.reshape(1, S, D)
```

```python
import functools

import jax
import jax.numpy as jnp
from jax import lax
import jax.experimental.pallas as pl
import jax.experimental.pallas.tpu as pltpu

F32 = jnp.float32
BF16 = jnp.bfloat16
U32 = jnp.uint32

S = 2048
D = 1024
H = 32
E = 128
M = 8
SEG = 32
NSEG = S // SEG
FF = 3584
NP = H // 2
L1 = M + SEG
L2 = 2 * L1

PRE = 512
TPS = 24
NS = 17
U = 4
WG = (3, 3, 5, 3)
WGS = (0, 3, 6, 11)
GPI = sum(WG)
REC = (GPI + U) * 8
NREC = 4
EPI = S - (NSEG // U) * GPI * 8
OEPI = NREC * REC
NST = 4
NCH = 3 * NP
NOC = 8
KC = H * E // NOC
PPC = NP // NOC
XA = PRE // 2
XBR = (S - PRE) // NP
WOP = (H * E // 2) // NP
KS = D // 2
MB = 256
LR = 32

WO_CHUNKS = ((0, 1), (1, 2), (2, 3), (3, 4), (4, 5), (5, 6), (6, 8))
LAG_QK, LAG_S, LAG_V, LAG_PV = 2, 4, 6, 8
LATE_S = {15: 50}
LATE_PV = {14: 50, 15: 53}
MOE_LEAD, MOE_GAP = 10, 1
EPI_TILES = 4

EPS = 1e-05
SCALE = float(E) ** -0.5
LOG2E = 1.4426950408889634


def _mod17(x):
    return x - 17 * ((x * 241) >> 12)


def _div14(x):
    return (x * 293) >> 12


assert NS == 17 and SEG == 32 and GPI == 14 and NP == 16
assert all(_mod17(x) == x % 17 for x in range(128))
assert all(_div14(x) == x // 14 for x in range(256))


def _rb(v):
    return v.astype(BF16).astype(F32)


def _recip(v):
    y = pl.reciprocal(v, approx=True)
    return y * (2.0 - v * y)


def _layernorm_rows(xb, wr8):
    xf = xb.astype(F32)
    mean = jnp.sum(xf, axis=-1, keepdims=True) * (1.0 / D)
    mb = _rb(mean)
    d = xf - mb
    dm = mean - mb
    var = jnp.maximum(jnp.sum(d * d, axis=-1, keepdims=True) * (1.0 / D) - dm * dm, 0.0)
    ve = _rb(_rb(var) + EPS)
    inv = _recip(_rb(ve * lax.rsqrt(ve)))
    xw = d * inv
    wr = jnp.concatenate([wr8] * (xb.shape[0] // 8), axis=0)
    r = _rb(jnp.sum(xw * wr, axis=-1, keepdims=True))
    return xw, r


def _scatter_scores(acc, r, g0):
    lane = lax.broadcasted_iota(jnp.int32, acc.shape, 1)
    for j in range(r.shape[0] // 8):
        acc = jnp.where(lane == g0 + j, r[j * 8:(j + 1) * 8, :], acc)
    return acc


def _dot(a, w32):
    return jnp.dot(a, pltpu.bitcast(w32, BF16), preferred_element_type=F32)


def _kernel(x_hbm, mem0_hbm, wq_hbm, wk_hbm, wv_hbm, wo_hbm, wr_hbm, wg_hbm, wu_hbm, wd_hbm,
            out_hbm,
            x_v, xn_v, xp_v, mem0_v, wqkv, wo_v, stage, wc0, wc1, wc2, wg_v, wu_v, wd_v,
            wr_v, fix_v,
            sem_xa, sem_xb, sem_s, sem_st, sem_wo, sem_w, sem_o, *rest):
    w32 = [w.bitcast(U32) for w in (wq_hbm, wk_hbm, wv_hbm)]
    wo32 = wo_hbm.bitcast(U32)
    wcur = (wc0, wc1, wc2)
    ring, o_vs = rest[:3], rest[3:3 + NOC]
    fill_v, wr_in = rest[3 + NOC:]

    def xa_copy(c):
        n = XA if c == 0 else PRE + TPS - XA
        return pltpu.make_async_copy(x_hbm.at[pl.ds(c * XA, n)], x_v.at[pl.ds(c * XA, n)],
                                     sem_xa.at[c])

    def xb_copy(i):
        src = pl.multiple_of(PRE + jnp.minimum(i, NP - 1) * XBR, 32)
        dst = pl.multiple_of(PRE + i * XBR, 32)
        return pltpu.make_async_copy(x_hbm.at[pl.ds(src, XBR)], x_v.at[pl.ds(dst, XBR)],
                                     sem_xb.at[i >> 4])

    def st_copy(t, p, slot, k, dp, sem):
        return pltpu.make_async_copy(w32[t].at[:, dp, p, 0, :], stage.at[slot, k, dp], sem)

    def grp_start(g, sems=None):
        slot = g & (NST - 1)
        for k, (t, p) in enumerate(((1, g), (2, g), (0, g + 1))):
            p = jnp.minimum(p, NP - 1)
            for dp in range(2):
                st_copy(t, p, slot, k, dp, sem_st.at[slot] if sems is None else sems[k]).start()

    def wait_all(view, sem):
        pltpu.make_async_copy(view, view, sem).wait()

    def grp_wait(g):
        slot = g & (NST - 1)
        wait_all(stage.at[slot], sem_st.at[slot])

    def wo_copy(i):
        src = pl.multiple_of(jnp.minimum(i, NP - 1) * WOP, 8)
        dst = pl.multiple_of(i * WOP, 8)
        return pltpu.make_async_copy(wo32.at[pl.ds(src, WOP)], wo_v.at[pl.ds(dst, WOP)],
                                     sem_wo.at[i >> 4])

    mem0_copy = pltpu.make_async_copy(mem0_hbm, mem0_v, sem_s.at[0])
    wr_copy = pltpu.make_async_copy(wr_hbm, wr_in, sem_s.at[1])
    moe_copies = [pltpu.make_async_copy(src.bitcast(U32), dst, sem_w.at[k])
                  for k, (src, dst) in enumerate(((wg_hbm, wg_v), (wu_hbm, wu_v), (wd_hbm, wd_v)))]

    xa_copy(0).start()
    wr_copy.start()
    for dp in range(2):
        st_copy(0, 0, NST, 0, dp, sem_st.at[NST]).start()
    xa_copy(1).start()

    row = lax.broadcasted_iota(jnp.int32, (L2, L2), 0)
    col = lax.broadcasted_iota(jnp.int32, (L2, L2), 1)
    rl = jnp.where(row >= L1, row - L1, row)
    cl = jnp.where(col >= L1, col - L1, col)
    same = (row >= L1) == (col >= L1)
    keep = (rl < M) | (rl >= cl)
    fill_v[...] = jnp.where(same, jnp.where(keep, 0.0, -1000000000.0 / SCALE), -jnp.inf).astype(F32)

    def ln_rows(r0, n, racc):
        for r in range(r0, r0 + n, LR):
            xw, sc = _layernorm_rows(x_v[pl.ds(r, LR), :], wr_v[...])
            xn_v[pl.ds(r, LR), :] = xw.astype(BF16)
            xp_v[pl.ds(r // 2, LR // 2), :] = pltpu.bitcast(xn_v[pl.ds(r, LR), :], U32)
            racc = _scatter_scores(racc, sc, r // 8)
        return racc

    def ln_step(i, racc):
        ic = jnp.minimum(i, NSEG - 1)
        r0 = pl.multiple_of(PRE + ic * TPS, 8)
        xw, r = _layernorm_rows(x_v[pl.ds(r0, TPS), :], wr_v[...])
        xn_v[pl.ds(r0, TPS), :] = xw.astype(BF16)
        return _scatter_scores(racc, r, PRE // 8 + ic * (TPS // 8))

    wr_copy.wait()
    wrf = wr_in[...].astype(F32)
    wr_v[...] = jnp.broadcast_to(
        jnp.concatenate([wrf[k:k + 1, :] for k in range(D // E)], axis=1), (8, D))
    xa_copy(0).wait()
    grp_start(0, (sem_st.at[0], sem_st.at[0], sem_st.at[NST + 1]))
    racc = ln_rows(0, XA, jnp.zeros((8, S // 8), F32))

    def relayout(slot, k, c, dst):
        for j in range(D // 2 // 64):
            a = stage[slot, k, 0, j * 64:(j + 1) * 64, :]
            b = stage[slot, k, 1, j * 64:(j + 1) * 64, :]
            ev = (a & jnp.uint32(0xFFFF)) | (b << 16)
            od = (a >> 16) | (b & jnp.uint32(0xFFFF0000))
            dst[j * 64:(j + 1) * 64, 0:E] = ev
            dst[j * 64:(j + 1) * 64, E:2 * E] = od
            wqkv[c, j * 64:(j + 1) * 64, 0:E] = ev
            wqkv[c, j * 64:(j + 1) * 64, E:2 * E] = od

    def pro_dots(t, p):
        for rb in range(PRE // MB):
            a = pltpu.bitcast(xp_v[rb * MB // 2:(rb + 1) * MB // 2, :], BF16)
            y = _dot(a, wcur[t][...]).astype(BF16)
            for sg in range(MB // SEG):
                for hh in range(2):
                    ring[t][rb * (MB // SEG) + sg, p, hh * L1 + M:(hh + 1) * L1, :] = (
                        y[sg * SEG:(sg + 1) * SEG, hh * E:(hh + 1) * E])

    wait_all(stage.at[NST, 0], sem_st.at[NST])
    xa_copy(1).wait()
    mem0_copy.start()
    grp_start(1)
    relayout(NST, 0, 0, wc0)
    racc = ln_rows(XA, PRE - XA, racc)
    pro_dots(0, 0)
    racc = ln_step(0, racc)

    wait_all(stage.at[0, pl.ds(0, 2)], sem_st.at[0])
    grp_start(2)
    relayout(0, 0, 1, wc1)
    relayout(0, 1, 2, wc2)
    pro_dots(1, 0)

    wait_all(stage.at[0, 2], sem_st.at[NST + 1])
    for i in range(3):
        wo_copy(i).start()
        xb_copy(i).start()
    relayout(0, 2, 3, wc0)
    pro_dots(2, 0)

    def pro(p, carry):
        grp_wait(p)
        slot = p & (NST - 1)
        for t in range(3):
            relayout(slot, t, 3 * p + t + 1, wcur[(t + 1) % 3])
            pro_dots(t, p)

        grp_start(p + 2)
        wo_copy(p + 2).start()
        xb_copy(p + 2).start()
        return carry

    lax.fori_loop(1, NP, pro, 0)

    wait_all(x_v.at[pl.ds(PRE, S - PRE)], sem_xb.at[0])
    mem0_copy.wait()
    wait_all(wo_v.at[pl.ds(0, NP * WOP)], sem_wo.at[0])
    for cp in moe_copies:
        cp.start()

    def step(it, u, carry):
        racc, mem = carry
        s = it * U + u
        slot = _mod17(s)
        t0 = pl.multiple_of(PRE + s * TPS, 8)
        top = xn_v[pl.ds(t0, 8), :].astype(F32)
        bot = xn_v[pl.ds(t0 + 8, 16), :]
        lhs = jnp.concatenate([jnp.concatenate([mem, top], axis=0).astype(BF16), bot], axis=0)
        part = [_dot(lhs[:, :KS], wqkv[t, 0:KS // 2, :]) for t in range(3)]
        qdst = []
        for j in range(TPS // 8):
            tj = t0 + 8 * j
            qdst.append((_mod17(tj >> 5), M + (tj & (SEG - 1))))
        odst = []
        for j in range(SEG // 8):
            g = (SEG // 8) * s + j
            gi = _div14(g)
            gr = g - GPI * gi
            r_ring = (gi & (NREC - 1)) * REC + (
                gr + 1 + sum((gr >= WGS[k]).astype(jnp.int32) for k in range(1, U))) * 8
            r_epi = OEPI + (g - (S - EPI) // 8) * 8
            odst.append(pl.multiple_of(jnp.where(g < (S - EPI) // 8, r_ring, r_epi), 8))
        orow = pl.multiple_of((it & (NREC - 1)) * REC + (WGS[u] + u) * 8, 16)
        nw = WG[u] * 8

        def qkv(p, t):
            if p == 0:
                y = _dot(lhs[:, KS:], wqkv[t, KS // 2:, :]) + part[t]
            else:
                y = _dot(lhs, wqkv[3 * p + t])
            y = y.astype(BF16)
            for hh in range(2):
                yc = y[:, hh * E:(hh + 1) * E]
                ring[t][slot, p, hh * L1:hh * L1 + M, :] = yc[0:M]
                for j in range(TPS // 8):
                    qs, qr = qdst[j]
                    ring[t][qs, p, pl.ds(pl.multiple_of(hh * L1 + qr, 8), 8), :] = (
                        yc[M + 8 * j:M + 8 * j + 8])

        def attn_probs(q, k):
            sc = lax.dot_general(q, k, (((1,), (1,)), ((), ())), preferred_element_type=F32)
            fill = fill_v[...]
            sc = jnp.where(fill == 0.0, sc, fill)
            e = jnp.exp2((sc - jnp.max(sc, axis=-1, keepdims=True)) * (SCALE * LOG2E))
            den = jnp.sum(e, axis=-1, keepdims=True)
            return (e * pl.reciprocal(den, approx=True)).astype(BF16)

        def attn_out(p, pr, v):
            o = jnp.dot(pr, v, preferred_element_type=F32).astype(BF16)
            oc = o_vs[p // PPC]
            for hh in range(2):
                cs = (2 * (p % PPC) + hh) * E
                oc[pl.ds(orow, M), cs:cs + E] = o[hh * L1:hh * L1 + M]
                for j in range(SEG // 8):
                    r = hh * L1 + M + 8 * j
                    oc[pl.ds(odst[j], 8), cs:cs + E] = o[r:r + 8]

        def wo_chunk(c, c1):
            a = jnp.concatenate([o_vs[i][pl.ds(orow, M + nw), :] for i in range(c, c1)], axis=1)
            return _dot(a, wo_v[c * KC // 2:c1 * KC // 2, :])

        nslot = 3 * NP + len(WO_CHUNKS)
        ev = {n: [] for n in range(nslot)}
        for p in range(NP):
            at_s = LATE_S.get(p, 3 * p + LAG_S)
            at_pv = LATE_PV.get(p, 3 * p + LAG_PV)
            ev[min(3 * p + LAG_QK, at_s)].append((0, p))
            ev[min(3 * p + LAG_V, at_pv)].append((1, p))
            ev[at_pv].append((2, p))
            ev[at_s].append((3, p))
        pr, qk, vv = {}, {}, {}
        acc = None
        r0 = pl.multiple_of((it * GPI + WGS[u]) * 8, 8)
        for n in range(nslot):
            for kind, p in sorted(ev[n]):
                if kind == 0:
                    qk[p] = (ring[0][slot, p], ring[1][slot, p])
                elif kind == 1:
                    vv[p] = ring[2][slot, p]
                elif kind == 2:
                    attn_out(p, pr.pop(p), vv.pop(p))
                else:
                    pr[p] = attn_probs(*qk.pop(p))
            if n < 3 * NP:
                qkv(n // 3, n % 3)
            else:
                y = wo_chunk(*WO_CHUNKS[n - 3 * NP])
                acc = y if acc is None else y + acc
        base = x_v[pl.ds(r0, nw), :].astype(F32) + xn_v[pl.ds(r0, nw), :].astype(F32)
        racc = ln_step(s + 1, racc)
        x_v[pl.ds(r0, nw), :] = (base + acc[M:]).astype(BF16)
        return racc, acc[0:M]

    def steps(it, carry):
        for u in range(U):
            carry = step(it, u, carry)
        return carry

    racc, _ = lax.fori_loop(0, NSEG // U, steps, (racc, mem0_v[...].astype(F32)))

    def out_copy(r0, n, k):
        return pltpu.make_async_copy(x_v.at[pl.ds(r0, n)], out_hbm.at[pl.ds(r0, n)], sem_o.at[k])

    for cp in moe_copies:
        cp.wait()
    grp_wait(NP)
    grp_wait(NP + 1)
    wait_all(x_v.at[pl.ds(S, 2 * XBR)], sem_xb.at[1])
    wait_all(wo_v.at[pl.ds(NP * WOP, 2 * WOP)], sem_wo.at[1])
    out_copy(0, S - EPI, 0).start()

    idx = (lax.broadcasted_iota(jnp.int32, racc.shape, 1) * 8
           + lax.broadcasted_iota(jnp.int32, racc.shape, 0)).astype(F32)

    def allred(fn, v):
        return fn(fn(v, axis=1, keepdims=True), axis=0, keepdims=True)

    m1 = allred(jnp.max, racc)
    i1 = allred(jnp.min, jnp.where(racc == m1, idx, float(S - 1)))
    r2 = jnp.where(idx == i1, -jnp.inf, racc)
    m2 = allred(jnp.max, r2)
    i2 = allred(jnp.min, jnp.where((r2 == m2) & (idx != i1), idx, float(S - 1)))
    sel = [jnp.clip(jnp.max(iv).astype(jnp.int32), 0, S - 1) for iv in (i1, i2)]
    grp = [pl.multiple_of((i >> 3) << 3, 8) for i in sel]
    sent = [pl.multiple_of(jnp.minimum(g, S - EPI - 8), 8) for g in grp]
    row8 = lax.broadcasted_iota(jnp.int32, (8, D), 0)
    rows = [jnp.sum(jnp.where(row8 == (i & 7), xn_v[pl.ds(g, 8), :].astype(F32), 0.0),
                    axis=0, keepdims=True) for i, g in zip(sel, grp)]
    row16 = lax.broadcasted_iota(jnp.int32, (16, D), 0)
    xs = jnp.where(row16 == 0, rows[0], jnp.where(row16 == 1, rows[1], 0.0)).astype(BF16)

    hs, ys, gps = {}, {}, {}

    def moe_gate(j):
        gps[j] = _rb(_dot(xs, wg_v[:, j * E:(j + 1) * E]))

    def moe_up(j):
        up = _rb(_dot(xs, wu_v[:, j * E:(j + 1) * E]))
        gp = gps.pop(j)
        g = _rb(gp * (1.0 / (1.0 + jnp.exp(-gp))))
        hs[j] = (g * up).astype(BF16)

    def moe_down(kc, nq):
        hk = jnp.concatenate([hs[4 * kc + i] for i in range(4)], axis=1)
        d = _dot(hk, wd_v[kc * 256:(kc + 1) * 256, nq * 256:(nq + 1) * 256])
        ys[nq] = d + ys[nq] if nq in ys else d

    def moe_apply():
        y = _rb(jnp.concatenate([ys[nq] for nq in range(4)], axis=1))
        upd = [_rb(y[n:n + 1, :] * _rb(1.0 / (1.0 + jnp.exp(-mv)))) for n, mv in enumerate((m1, m2))]
        for n in range(2):
            blk = x_v[pl.ds(sent[n], 8), :].astype(F32)
            for k in range(2):
                blk = blk + jnp.where(row8 + sent[n] == sel[k], upd[k], 0.0)
            fix_v[n] = blk.astype(BF16)
        for n in range(2):
            g = pl.multiple_of(jnp.maximum(grp[n], S - EPI), 8)
            x_v[pl.ds(g, 8), :] = (x_v[pl.ds(g, 8), :].astype(F32)
                                   + jnp.where(row8 + g == sel[n], upd[n], 0.0)).astype(BF16)

    waves = []
    for j in range(FF // E):
        waves += [functools.partial(moe_gate, j), functools.partial(moe_up, j)]
    for kc in range(FF // 512):
        waves += [functools.partial(moe_down, kc, nq) for nq in range(4)]
    waves = [None] * MOE_LEAD + waves + [None] * MOE_GAP + [moe_apply]

    def finish(rs, cs, acc):
        x_v[rs, cs] = (x_v[rs, cs].astype(F32) + xn_v[rs, cs].astype(F32) + acc).astype(BF16)

    for blk, n in [(0, n) for n in range(D // E)] + [(1, n) for n in range(EPI_TILES)]:
        ar = OEPI + blk * 128
        r0 = S - EPI + blk * 128
        acc = None
        for kc in range(NOC):
            d = _dot(o_vs[kc][ar:ar + 128, :],
                     wo_v[kc * KC // 2:(kc + 1) * KC // 2, n * E:(n + 1) * E])
            acc = d if acc is None else d + acc
            if kc == NOC - 1:
                finish(slice(r0, r0 + 128), slice(n * E, (n + 1) * E), acc)
            wv = waves.pop(0) if waves else None
            if wv is not None:
                wv()
    assert not waves

    fixes = [pltpu.make_async_copy(fix_v.at[n], out_hbm.at[pl.ds(sent[n], 8)], sem_o.at[4 + n])
             for n in range(2)]
    out_copy(S - EPI, 128, 1).start()
    out_copy(0, S - EPI, 0).wait()
    fixes[0].start()

    c0 = EPI_TILES * E

    def epi(i, carry):
        ar = pl.ds(pl.multiple_of(OEPI + 128 + i * 64, 16), 64)
        a = jnp.concatenate([oc[ar, :] for oc in o_vs], axis=1)
        r0 = pl.multiple_of(S - 128 + i * 64, 64)
        finish(pl.ds(r0, 64), slice(c0, D), _dot(a, wo_v[0:NP * WOP, c0:]))
        out_copy(r0, 64, 2 + i).start()

        @pl.when(i == 0)
        def _():
            fixes[0].wait()
            fixes[1].start()

        return carry

    lax.fori_loop(0, 2, epi, 0)

    fixes[1].wait()
    out_copy(S - EPI, 128, 1).wait()
    for i in range(2):
        out_copy(S - 128 + i * 64, 64, 2 + i).wait()


@jax.jit
def pallas_parallel_sum__memory_aug_recurrent_mem_tr__moe_arch_mod__prompt_kernel(
    A_x: jax.Array,
    A_mem0: jax.Array,
    A_Wq: jax.Array,
    A_Wk: jax.Array,
    A_Wv: jax.Array,
    A_Wo: jax.Array,
    A_seg_len: jax.Array,
    B_x: jax.Array,
    B_w_r: jax.Array,
    B_w_gate: jax.Array,
    B_w_up: jax.Array,
    B_w_down: jax.Array,
):
    del A_seg_len, B_x
    assert A_x.shape == (1, S, D) and A_Wq.shape == (D, H, E) and A_mem0.shape == (1, M, D)
    assert B_w_gate.shape == (D, FF)
    wshape = (D // 2, 2, NP, 2, E)
    any_spec = pl.BlockSpec(memory_space=pl.ANY)
    out = pl.pallas_call(
        _kernel,
        out_shape=jax.ShapeDtypeStruct((S, D), BF16),
        in_specs=[any_spec] * 10,
        out_specs=any_spec,
        scratch_shapes=[
            pltpu.VMEM((S + 2 * XBR, D), BF16),
            pltpu.VMEM((S, D), BF16),
            pltpu.VMEM((PRE // 2, D), U32),
            pltpu.VMEM((M, D), BF16),
            pltpu.VMEM((NCH + 1, D // 2, 2 * E), U32),
            pltpu.VMEM(((NP + 2) * WOP, D), U32),
            pltpu.VMEM((NST + 1, 3, 2, D // 2, E), U32),
            pltpu.VMEM((D // 2, 2 * E), U32),
            pltpu.VMEM((D // 2, 2 * E), U32),
            pltpu.VMEM((D // 2, 2 * E), U32),
            pltpu.VMEM((D // 2, FF), U32),
            pltpu.VMEM((D // 2, FF), U32),
            pltpu.VMEM((FF // 2, D), U32),
            pltpu.VMEM((8, D), F32),
            pltpu.VMEM((2, 8, D), BF16),
            pltpu.SemaphoreType.DMA((2,)),
            pltpu.SemaphoreType.DMA((2,)),
            pltpu.SemaphoreType.DMA((2,)),
            pltpu.SemaphoreType.DMA((NST + 2,)),
            pltpu.SemaphoreType.DMA((2,)),
            pltpu.SemaphoreType.DMA((3,)),
            pltpu.SemaphoreType.DMA((6,)),
            *[pltpu.VMEM((NS, NP, L2, E), BF16)] * 3,
            *[pltpu.VMEM((OEPI + EPI, KC), BF16)] * NOC,
            pltpu.VMEM((L2, L2), F32),
            pltpu.VMEM((D // E, E), BF16),
        ],
        compiler_params=pltpu.CompilerParams(vmem_limit_bytes=120 * 1024 * 1024,
                                             disable_bounds_checks=True),
    )(
        A_x.reshape(S, D),
        A_mem0.reshape(M, D),
        A_Wq.reshape(wshape),
        A_Wk.reshape(wshape),
        A_Wv.reshape(wshape),
        A_Wo.reshape(H * E, D),
        B_w_r.reshape(D // E, E),
        B_w_gate,
        B_w_up,
        B_w_down,
    )
    return out.reshape(1, S, D)
```

```python
import functools

import jax
import jax.numpy as jnp
from jax import lax
import jax.experimental.pallas as pl
import jax.experimental.pallas.tpu as pltpu

F32 = jnp.float32
BF16 = jnp.bfloat16
U32 = jnp.uint32

S = 2048
D = 1024
H = 32
E = 128
M = 8
SEG = 32
NSEG = S // SEG
FF = 3584
NP = H // 2
L1 = M + SEG
L2 = 2 * L1

PRE = 512
TPS = 24
NS = 17
U = 4
WG = (3, 3, 5, 3)
WGS = (0, 3, 6, 11)
GPI = sum(WG)
REC = (GPI + U) * 8
NREC = 4
EPI = S - (NSEG // U) * GPI * 8
OEPI = NREC * REC
NST = 4
NCH = 3 * NP
NOC = 8
KC = H * E // NOC
PPC = NP // NOC
XA = PRE // 2
XBR = (S - PRE) // NP
WOP = (H * E // 2) // NP
KS = D // 2
MB = 256
LR = 32

WO_CHUNKS = ((0, 1), (1, 2), (2, 3), (3, 4), (4, 5), (5, 6), (6, 8))
LAG_QK, LAG_S, LAG_V, LAG_PV = 2, 4, 6, 8
LATE_S = {15: 50}
LATE_PV = {14: 50, 15: 53}
MOE_LEAD, MOE_GAP = 10, 1
EPI_TILES = 4

EPS = 1e-05
SCALE = float(E) ** -0.5
LOG2E = 1.4426950408889634


def _mod17(x):
    return x - 17 * ((x * 241) >> 12)


def _div14(x):
    return (x * 293) >> 12


assert NS == 17 and GPI == 14 and NP == 16 and (U * TPS) % SEG == 0
assert all(_mod17(x) == x % 17 for x in range(128))
assert all(_div14(x) == x // 14 for x in range(256))


def _rb(v):
    return v.astype(BF16).astype(F32)


def _recip(v):
    y = pl.reciprocal(v, approx=True)
    return y * (2.0 - v * y)


def _layernorm_rows(xb, wr8):
    xf = xb.astype(F32)
    mean = jnp.sum(xf, axis=-1, keepdims=True) * (1.0 / D)
    mb = _rb(mean)
    d = xf - mb
    dm = mean - mb
    var = jnp.maximum(jnp.sum(d * d, axis=-1, keepdims=True) * (1.0 / D) - dm * dm, 0.0)
    ve = _rb(_rb(var) + EPS)
    inv = _recip(_rb(ve * lax.rsqrt(ve)))
    xw = d * inv
    wr = jnp.concatenate([wr8] * (xb.shape[0] // 8), axis=0)
    r = _rb(jnp.sum(xw * wr, axis=-1, keepdims=True))
    return xw, r


def _scatter_scores(acc, r, g0):
    lane = lax.broadcasted_iota(jnp.int32, acc.shape, 1)
    for j in range(r.shape[0] // 8):
        acc = jnp.where(lane == g0 + j, r[j * 8:(j + 1) * 8, :], acc)
    return acc


def _dot(a, w32):
    return jnp.dot(a, pltpu.bitcast(w32, BF16), preferred_element_type=F32)


def _kernel(x_hbm, mem0_hbm, wq_hbm, wk_hbm, wv_hbm, wo_hbm, wr_hbm, wg_hbm, wu_hbm, wd_hbm,
            out_hbm,
            x_v, xn_v, xp_v, mem0_v, wqkv, wo_v, stage, wc0, wc1, wc2, wg_v, wu_v, wd_v,
            wr_v, fix_v,
            sem_xa, sem_xb, sem_s, sem_st, sem_wo, sem_w, sem_o, *rest):
    w32 = [w.bitcast(U32) for w in (wq_hbm, wk_hbm, wv_hbm)]
    wo32 = wo_hbm.bitcast(U32)
    wcur = (wc0, wc1, wc2)
    ring, o_vs = rest[:3], rest[3:3 + NOC]
    fill_v, wr_in = rest[3 + NOC:]

    def xa_copy(c):
        n = XA if c == 0 else PRE + TPS - XA
        return pltpu.make_async_copy(x_hbm.at[pl.ds(c * XA, n)], x_v.at[pl.ds(c * XA, n)],
                                     sem_xa.at[c])

    def xb_copy(i):
        src = pl.multiple_of(PRE + jnp.minimum(i, NP - 1) * XBR, 32)
        dst = pl.multiple_of(PRE + i * XBR, 32)
        return pltpu.make_async_copy(x_hbm.at[pl.ds(src, XBR)], x_v.at[pl.ds(dst, XBR)],
                                     sem_xb.at[i >> 4])

    def st_copy(t, p, slot, k, dp, sem):
        return pltpu.make_async_copy(w32[t].at[:, dp, p, 0, :], stage.at[slot, k, dp], sem)

    def grp_start(g, sems=None):
        slot = g & (NST - 1)
        for k, (t, p) in enumerate(((1, g), (2, g), (0, g + 1))):
            p = jnp.minimum(p, NP - 1)
            for dp in range(2):
                st_copy(t, p, slot, k, dp, sem_st.at[slot] if sems is None else sems[k]).start()

    def wait_all(view, sem):
        pltpu.make_async_copy(view, view, sem).wait()

    def grp_wait(g):
        slot = g & (NST - 1)
        wait_all(stage.at[slot], sem_st.at[slot])

    def wo_copy(i):
        src = pl.multiple_of(jnp.minimum(i, NP - 1) * WOP, 8)
        dst = pl.multiple_of(i * WOP, 8)
        return pltpu.make_async_copy(wo32.at[pl.ds(src, WOP)], wo_v.at[pl.ds(dst, WOP)],
                                     sem_wo.at[i >> 4])

    mem0_copy = pltpu.make_async_copy(mem0_hbm, mem0_v, sem_s.at[0])
    wr_copy = pltpu.make_async_copy(wr_hbm, wr_in, sem_s.at[1])
    moe_copies = [pltpu.make_async_copy(src.bitcast(U32), dst, sem_w.at[k])
                  for k, (src, dst) in enumerate(((wg_hbm, wg_v), (wu_hbm, wu_v), (wd_hbm, wd_v)))]

    xa_copy(0).start()
    wr_copy.start()
    for dp in range(2):
        st_copy(0, 0, NST, 0, dp, sem_st.at[NST]).start()
    xa_copy(1).start()

    row = lax.broadcasted_iota(jnp.int32, (L2, L2), 0)
    col = lax.broadcasted_iota(jnp.int32, (L2, L2), 1)
    rl = jnp.where(row >= L1, row - L1, row)
    cl = jnp.where(col >= L1, col - L1, col)
    same = (row >= L1) == (col >= L1)
    keep = (rl < M) | (rl >= cl)
    fill_v[...] = jnp.where(same, jnp.where(keep, 0.0, -1000000000.0 / SCALE), -jnp.inf).astype(F32)

    def ln_rows(r0, n, racc):
        for r in range(r0, r0 + n, LR):
            xw, sc = _layernorm_rows(x_v[pl.ds(r, LR), :], wr_v[...])
            xn_v[pl.ds(r, LR), :] = xw.astype(BF16)
            xp_v[pl.ds(r // 2, LR // 2), :] = pltpu.bitcast(xn_v[pl.ds(r, LR), :], U32)
            racc = _scatter_scores(racc, sc, r // 8)
        return racc

    def ln_step(i, racc):
        ic = jnp.minimum(i, NSEG - 1)
        r0 = pl.multiple_of(PRE + ic * TPS, 8)
        xw, r = _layernorm_rows(x_v[pl.ds(r0, TPS), :], wr_v[...])
        xn_v[pl.ds(r0, TPS), :] = xw.astype(BF16)
        return _scatter_scores(racc, r, PRE // 8 + ic * (TPS // 8))

    wr_copy.wait()
    wrf = wr_in[...].astype(F32)
    wr_v[...] = jnp.broadcast_to(
        jnp.concatenate([wrf[k:k + 1, :] for k in range(D // E)], axis=1), (8, D))
    xa_copy(0).wait()
    grp_start(0, (sem_st.at[0], sem_st.at[0], sem_st.at[NST + 1]))
    racc = ln_rows(0, XA, jnp.zeros((8, S // 8), F32))

    def relayout(slot, k, c, dst):
        for j in range(D // 2 // 64):
            a = stage[slot, k, 0, j * 64:(j + 1) * 64, :]
            b = stage[slot, k, 1, j * 64:(j + 1) * 64, :]
            ev = (a & jnp.uint32(0xFFFF)) | (b << 16)
            od = (a >> 16) | (b & jnp.uint32(0xFFFF0000))
            dst[j * 64:(j + 1) * 64, 0:E] = ev
            dst[j * 64:(j + 1) * 64, E:2 * E] = od
            wqkv[c, j * 64:(j + 1) * 64, 0:E] = ev
            wqkv[c, j * 64:(j + 1) * 64, E:2 * E] = od

    def pro_dots(t, p):
        for rb in range(PRE // MB):
            a = pltpu.bitcast(xp_v[rb * MB // 2:(rb + 1) * MB // 2, :], BF16)
            y = _dot(a, wcur[t][...]).astype(BF16)
            for sg in range(MB // SEG):
                for hh in range(2):
                    ring[t][rb * (MB // SEG) + sg, p, hh * L1 + M:(hh + 1) * L1, :] = (
                        y[sg * SEG:(sg + 1) * SEG, hh * E:(hh + 1) * E])

    wait_all(stage.at[NST, 0], sem_st.at[NST])
    xa_copy(1).wait()
    mem0_copy.start()
    grp_start(1)
    relayout(NST, 0, 0, wc0)
    racc = ln_rows(XA, PRE - XA, racc)
    pro_dots(0, 0)
    racc = ln_step(0, racc)

    wait_all(stage.at[0, pl.ds(0, 2)], sem_st.at[0])
    grp_start(2)
    relayout(0, 0, 1, wc1)
    relayout(0, 1, 2, wc2)
    pro_dots(1, 0)

    wait_all(stage.at[0, 2], sem_st.at[NST + 1])
    for i in range(3):
        wo_copy(i).start()
        xb_copy(i).start()
    relayout(0, 2, 3, wc0)
    pro_dots(2, 0)

    def pro(p, carry):
        grp_wait(p)
        slot = p & (NST - 1)
        for t in range(3):
            relayout(slot, t, 3 * p + t + 1, wcur[(t + 1) % 3])
            pro_dots(t, p)

        grp_start(p + 2)
        wo_copy(p + 2).start()
        xb_copy(p + 2).start()
        return carry

    lax.fori_loop(1, NP, pro, 0)

    wait_all(x_v.at[pl.ds(PRE, S - PRE)], sem_xb.at[0])
    mem0_copy.wait()
    wait_all(wo_v.at[pl.ds(0, NP * WOP)], sem_wo.at[0])
    for cp in moe_copies:
        cp.start()

    def step(it, u, carry):
        racc, mem = carry
        s = it * U + u
        slot = _mod17(s)
        t0 = pl.multiple_of(PRE + s * TPS, 8)
        top = xn_v[pl.ds(t0, 8), :].astype(F32)
        bot = xn_v[pl.ds(t0 + 8, 16), :]
        lhs = jnp.concatenate([jnp.concatenate([mem, top], axis=0).astype(BF16), bot], axis=0)
        part = [_dot(lhs[:, :KS], wqkv[t, 0:KS // 2, :]) for t in range(3)]
        qdst = []
        for j in range(TPS // 8):
            m, gq = divmod(u * (TPS // 8) + j, SEG // 8)
            if qdst and qdst[-1][0] == m:
                qdst[-1][3] += 1
            else:
                qdst.append([m, M + 8 * gq, j, 1])
        qdst = [(_mod17(PRE // SEG + (U * TPS // SEG) * it + m), r, j, n) for m, r, j, n in qdst]
        odst = []
        for j in range(SEG // 8):
            g = (SEG // 8) * s + j
            gi = _div14(g)
            gr = g - GPI * gi
            r_ring = (gi & (NREC - 1)) * REC + (
                gr + 1 + sum((gr >= WGS[k]).astype(jnp.int32) for k in range(1, U))) * 8
            r_epi = OEPI + (g - (S - EPI) // 8) * 8
            odst.append(pl.multiple_of(jnp.where(g < (S - EPI) // 8, r_ring, r_epi), 8))
        orow = pl.multiple_of((it & (NREC - 1)) * REC + (WGS[u] + u) * 8, 16)
        nw = WG[u] * 8

        def qkv(p, t):
            if p == 0:
                y = _dot(lhs[:, KS:], wqkv[t, KS // 2:, :]) + part[t]
            else:
                y = _dot(lhs, wqkv[3 * p + t])
            y = y.astype(BF16)
            for hh in range(2):
                yc = y[:, hh * E:(hh + 1) * E]
                ring[t][slot, p, hh * L1:hh * L1 + M, :] = yc[0:M]
                for qs, qr, j, n in qdst:
                    ring[t][qs, p, hh * L1 + qr:hh * L1 + qr + 8 * n, :] = (
                        yc[M + 8 * j:M + 8 * (j + n)])

        def attn_probs(q, k):
            sc = lax.dot_general(q, k, (((1,), (1,)), ((), ())), preferred_element_type=F32)
            fill = fill_v[...]
            sc = jnp.where(fill == 0.0, sc, fill)
            e = jnp.exp2((sc - jnp.max(sc, axis=-1, keepdims=True)) * (SCALE * LOG2E))
            den = jnp.sum(e, axis=-1, keepdims=True)
            return (e * pl.reciprocal(den, approx=True)).astype(BF16)

        def attn_out(p, pr, v):
            o = jnp.dot(pr, v, preferred_element_type=F32).astype(BF16)
            oc = o_vs[p // PPC]
            for hh in range(2):
                cs = (2 * (p % PPC) + hh) * E
                oc[pl.ds(orow, M), cs:cs + E] = o[hh * L1:hh * L1 + M]
                for j in range(SEG // 8):
                    r = hh * L1 + M + 8 * j
                    oc[pl.ds(odst[j], 8), cs:cs + E] = o[r:r + 8]

        def wo_chunk(c, c1):
            a = jnp.concatenate([o_vs[i][pl.ds(orow, M + nw), :] for i in range(c, c1)], axis=1)
            return _dot(a, wo_v[c * KC // 2:c1 * KC // 2, :])

        nslot = 3 * NP + len(WO_CHUNKS)
        ev = {n: [] for n in range(nslot)}
        for p in range(NP):
            at_s = LATE_S.get(p, 3 * p + LAG_S)
            at_pv = LATE_PV.get(p, 3 * p + LAG_PV)
            ev[min(3 * p + LAG_QK, at_s)].append((0, p))
            ev[min(3 * p + LAG_V, at_pv)].append((1, p))
            ev[at_pv].append((2, p))
            ev[at_s].append((3, p))
        pr, qk, vv = {}, {}, {}
        acc = None
        r0 = pl.multiple_of((it * GPI + WGS[u]) * 8, 8)
        for n in range(nslot):
            for kind, p in sorted(ev[n]):
                if kind == 0:
                    qk[p] = (ring[0][slot, p], ring[1][slot, p])
                elif kind == 1:
                    vv[p] = ring[2][slot, p]
                elif kind == 2:
                    attn_out(p, pr.pop(p), vv.pop(p))
                else:
                    pr[p] = attn_probs(*qk.pop(p))
            if n < 3 * NP:
                qkv(n // 3, n % 3)
            else:
                y = wo_chunk(*WO_CHUNKS[n - 3 * NP])
                acc = y if acc is None else y + acc
        base = x_v[pl.ds(r0, nw), :].astype(F32) + xn_v[pl.ds(r0, nw), :].astype(F32)
        racc = ln_step(s + 1, racc)
        x_v[pl.ds(r0, nw), :] = (base + acc[M:]).astype(BF16)
        return racc, acc[0:M]

    def steps(it, carry):
        for u in range(U):
            carry = step(it, u, carry)
        return carry

    racc, _ = lax.fori_loop(0, NSEG // U, steps, (racc, mem0_v[...].astype(F32)))

    def out_copy(r0, n, k):
        return pltpu.make_async_copy(x_v.at[pl.ds(r0, n)], out_hbm.at[pl.ds(r0, n)], sem_o.at[k])

    for cp in moe_copies:
        cp.wait()
    grp_wait(NP)
    grp_wait(NP + 1)
    wait_all(x_v.at[pl.ds(S, 2 * XBR)], sem_xb.at[1])
    wait_all(wo_v.at[pl.ds(NP * WOP, 2 * WOP)], sem_wo.at[1])
    out_copy(0, S - EPI, 0).start()

    idx = (lax.broadcasted_iota(jnp.int32, racc.shape, 1) * 8
           + lax.broadcasted_iota(jnp.int32, racc.shape, 0)).astype(F32)

    def allred(fn, v):
        return fn(fn(v, axis=1, keepdims=True), axis=0, keepdims=True)

    m1 = allred(jnp.max, racc)
    i1 = allred(jnp.min, jnp.where(racc == m1, idx, float(S - 1)))
    r2 = jnp.where(idx == i1, -jnp.inf, racc)
    m2 = allred(jnp.max, r2)
    i2 = allred(jnp.min, jnp.where((r2 == m2) & (idx != i1), idx, float(S - 1)))
    sel = [jnp.clip(jnp.max(iv).astype(jnp.int32), 0, S - 1) for iv in (i1, i2)]
    grp = [pl.multiple_of((i >> 3) << 3, 8) for i in sel]
    sent = [pl.multiple_of(jnp.minimum(g, S - EPI - 8), 8) for g in grp]
    row8 = lax.broadcasted_iota(jnp.int32, (8, D), 0)
    rows = [jnp.sum(jnp.where(row8 == (i & 7), xn_v[pl.ds(g, 8), :].astype(F32), 0.0),
                    axis=0, keepdims=True) for i, g in zip(sel, grp)]
    row16 = lax.broadcasted_iota(jnp.int32, (16, D), 0)
    xs = jnp.where(row16 == 0, rows[0], jnp.where(row16 == 1, rows[1], 0.0)).astype(BF16)

    hs, ys, gps = {}, {}, {}

    def moe_gate(j):
        gps[j] = _rb(_dot(xs, wg_v[:, j * E:(j + 1) * E]))

    def moe_up(j):
        up = _rb(_dot(xs, wu_v[:, j * E:(j + 1) * E]))
        gp = gps.pop(j)
        g = _rb(gp * (1.0 / (1.0 + jnp.exp(-gp))))
        hs[j] = (g * up).astype(BF16)

    def moe_down(kc, nq):
        hk = jnp.concatenate([hs[4 * kc + i] for i in range(4)], axis=1)
        d = _dot(hk, wd_v[kc * 256:(kc + 1) * 256, nq * 256:(nq + 1) * 256])
        ys[nq] = d + ys[nq] if nq in ys else d

    def moe_apply():
        y = _rb(jnp.concatenate([ys[nq] for nq in range(4)], axis=1))
        upd = [_rb(y[n:n + 1, :] * _rb(1.0 / (1.0 + jnp.exp(-mv)))) for n, mv in enumerate((m1, m2))]
        for n in range(2):
            blk = x_v[pl.ds(sent[n], 8), :].astype(F32)
            for k in range(2):
                blk = blk + jnp.where(row8 + sent[n] == sel[k], upd[k], 0.0)
            fix_v[n] = blk.astype(BF16)
        for n in range(2):
            g = pl.multiple_of(jnp.maximum(grp[n], S - EPI), 8)
            x_v[pl.ds(g, 8), :] = (x_v[pl.ds(g, 8), :].astype(F32)
                                   + jnp.where(row8 + g == sel[n], upd[n], 0.0)).astype(BF16)

    waves = []
    for j in range(FF // E):
        waves += [functools.partial(moe_gate, j), functools.partial(moe_up, j)]
    for kc in range(FF // 512):
        waves += [functools.partial(moe_down, kc, nq) for nq in range(4)]
    waves = [None] * MOE_LEAD + waves + [None] * MOE_GAP + [moe_apply]

    def finish(rs, cs, acc):
        x_v[rs, cs] = (x_v[rs, cs].astype(F32) + xn_v[rs, cs].astype(F32) + acc).astype(BF16)

    for blk, n in [(0, n) for n in range(D // E)] + [(1, n) for n in range(EPI_TILES)]:
        ar = OEPI + blk * 128
        r0 = S - EPI + blk * 128
        acc = None
        for kc in range(NOC):
            d = _dot(o_vs[kc][ar:ar + 128, :],
                     wo_v[kc * KC // 2:(kc + 1) * KC // 2, n * E:(n + 1) * E])
            acc = d if acc is None else d + acc
            if kc == NOC - 1:
                finish(slice(r0, r0 + 128), slice(n * E, (n + 1) * E), acc)
            wv = waves.pop(0) if waves else None
            if wv is not None:
                wv()
    assert not waves

    fixes = [pltpu.make_async_copy(fix_v.at[n], out_hbm.at[pl.ds(sent[n], 8)], sem_o.at[4 + n])
             for n in range(2)]
    out_copy(S - EPI, 128, 1).start()
    out_copy(0, S - EPI, 0).wait()
    fixes[0].start()

    c0 = EPI_TILES * E

    def epi(i, carry):
        ar = pl.ds(pl.multiple_of(OEPI + 128 + i * 64, 16), 64)
        a = jnp.concatenate([oc[ar, :] for oc in o_vs], axis=1)
        r0 = pl.multiple_of(S - 128 + i * 64, 64)
        finish(pl.ds(r0, 64), slice(c0, D), _dot(a, wo_v[0:NP * WOP, c0:]))
        out_copy(r0, 64, 2 + i).start()

        @pl.when(i == 0)
        def _():
            fixes[0].wait()
            fixes[1].start()

        return carry

    lax.fori_loop(0, 2, epi, 0)

    fixes[1].wait()
    out_copy(S - EPI, 128, 1).wait()
    for i in range(2):
        out_copy(S - 128 + i * 64, 64, 2 + i).wait()


@jax.jit
def pallas_parallel_sum__memory_aug_recurrent_mem_tr__moe_arch_mod__prompt_kernel(
    A_x: jax.Array,
    A_mem0: jax.Array,
    A_Wq: jax.Array,
    A_Wk: jax.Array,
    A_Wv: jax.Array,
    A_Wo: jax.Array,
    A_seg_len: jax.Array,
    B_x: jax.Array,
    B_w_r: jax.Array,
    B_w_gate: jax.Array,
    B_w_up: jax.Array,
    B_w_down: jax.Array,
):
    del A_seg_len, B_x
    assert A_x.shape == (1, S, D) and A_Wq.shape == (D, H, E) and A_mem0.shape == (1, M, D)
    assert B_w_gate.shape == (D, FF)
    wshape = (D // 2, 2, NP, 2, E)
    any_spec = pl.BlockSpec(memory_space=pl.ANY)
    out = pl.pallas_call(
        _kernel,
        out_shape=jax.ShapeDtypeStruct((S, D), BF16),
        in_specs=[any_spec] * 10,
        out_specs=any_spec,
        scratch_shapes=[
            pltpu.VMEM((S + 2 * XBR, D), BF16),
            pltpu.VMEM((S, D), BF16),
            pltpu.VMEM((PRE // 2, D), U32),
            pltpu.VMEM((M, D), BF16),
            pltpu.VMEM((NCH + 1, D // 2, 2 * E), U32),
            pltpu.VMEM(((NP + 2) * WOP, D), U32),
            pltpu.VMEM((NST + 1, 3, 2, D // 2, E), U32),
            pltpu.VMEM((D // 2, 2 * E), U32),
            pltpu.VMEM((D // 2, 2 * E), U32),
            pltpu.VMEM((D // 2, 2 * E), U32),
            pltpu.VMEM((D // 2, FF), U32),
            pltpu.VMEM((D // 2, FF), U32),
            pltpu.VMEM((FF // 2, D), U32),
            pltpu.VMEM((8, D), F32),
            pltpu.VMEM((2, 8, D), BF16),
            pltpu.SemaphoreType.DMA((2,)),
            pltpu.SemaphoreType.DMA((2,)),
            pltpu.SemaphoreType.DMA((2,)),
            pltpu.SemaphoreType.DMA((NST + 2,)),
            pltpu.SemaphoreType.DMA((2,)),
            pltpu.SemaphoreType.DMA((3,)),
            pltpu.SemaphoreType.DMA((6,)),
            *[pltpu.VMEM((NS, NP, L2, E), BF16)] * 3,
            *[pltpu.VMEM((OEPI + EPI, KC), BF16)] * NOC,
            pltpu.VMEM((L2, L2), F32),
            pltpu.VMEM((D // E, E), BF16),
        ],
        compiler_params=pltpu.CompilerParams(vmem_limit_bytes=120 * 1024 * 1024,
                                             disable_bounds_checks=True),
    )(
        A_x.reshape(S, D),
        A_mem0.reshape(M, D),
        A_Wq.reshape(wshape),
        A_Wk.reshape(wshape),
        A_Wv.reshape(wshape),
        A_Wo.reshape(H * E, D),
        B_w_r.reshape(D // E, E),
        B_w_gate,
        B_w_up,
        B_w_down,
    )
    return out.reshape(1, S, D)
```
